```python
import jax
import jax.numpy as jnp

def _softmax(x, axis=-1):
    return jax.nn.softmax(x, axis=axis)
def _gelu(x):
    return jax.nn.gelu(x, approximate=True)
def _silu(x):
    return jax.nn.silu(x)
def _sigmoid(x):
    return jax.nn.sigmoid(x)
def _layernorm(x, axis=-1, eps=1e-5):
    m = jnp.mean(x, axis=axis, keepdims=True)
    v = jnp.var(x, axis=axis, keepdims=True)
    return (x - m) / jnp.sqrt(v + eps)
def _scatter_add(tgt, idx, src, axis=0):
    return tgt.at[idx].add(src)
def _segment_sum(src, seg, n):
    return jax.ops.segment_sum(src, seg, n)
class _Rng:
    def __init__(self, key):
        self._k = key
    def _next(self):
        self._k, sub = jax.random.split(self._k)
        return sub
    def normal(self, shape):
        return jax.random.normal(self._next(), shape, dtype=jnp.bfloat16)
    def randint(self, lo, hi, shape):
        return jax.random.randint(self._next(), shape, lo, hi, dtype=jnp.int32)
    def uniform(self, shape, lo=0.0, hi=1.0):
        return jax.random.uniform(self._next(), shape, jnp.bfloat16, lo, hi)
    def permutation(self, n):
        return jax.random.permutation(self._next(), n)


kernel_name = 'recurrent_scan__sliding_block_cached__moe_arch_mod__prompt'

def setup_inputs():
    _rng = _Rng(jax.random.key(int.from_bytes(__import__("os").urandom(4), "little")))
    _w = (lambda a: (lambda t: t.astype(jnp.bfloat16) if jnp.issubdtype(t.dtype, jnp.floating) else t)(jnp.asarray(a)))
    def _A_setup():
        B, Sq, D = 1, 2048, 640
        Hq, Hkv, Sk, Dh = 32, 32, 2048, 192
        assert Hq % Hkv == 0, (Hq, Hkv)
        return {
            "x": _w((lambda *s: _rng.normal(s) * 0.05)(B, Sq, D)),
            "k_cache": _w((lambda *s: _rng.normal(s) * 0.05)(B, Hkv, Sk, Dh)),
            "v_cache": _w((lambda *s: _rng.normal(s) * 0.05)(B, Hkv, Sk, Dh)),
            "wq": _w((lambda *s: _rng.normal(s) * 0.05)(D, Hq * Dh) * (D ** -0.5)),
            "wo": _w((lambda *s: _rng.normal(s) * 0.05)(Hq * Dh, D) * ((Hq * Dh) ** -0.5)),
        }
    _A_in = _A_setup()

    def _B_setup():
        B, S, D, F, C = 1, 2048, 640, 1536, 2
        return {
            "x": _w((lambda *s: _rng.normal(s) * 0.05)(B, S, D)),
            "w_r": _w((lambda *s: _rng.normal(s) * 0.05)(D)),
            "w_gate": _w((lambda *s: _rng.normal(s) * 0.05)(D, F)),
            "w_up": _w((lambda *s: _rng.normal(s) * 0.05)(D, F)),
            "w_down": _w((lambda *s: _rng.normal(s) * 0.05)(F, D)),
        }
    _B_in = _B_setup()

    return {
        "A_x": _A_in["x"],
        "A_k_cache": _A_in["k_cache"],
        "A_v_cache": _A_in["v_cache"],
        "A_wq": _A_in["wq"],
        "A_wo": _A_in["wo"],
        "B_x": _B_in["x"],
        "B_w_r": _B_in["w_r"],
        "B_w_gate": _B_in["w_gate"],
        "B_w_up": _B_in["w_up"],
        "B_w_down": _B_in["w_down"],
    }

def reference(A_x, A_k_cache, A_v_cache, A_wq, A_wo, B_x, B_w_r, B_w_gate, B_w_up, B_w_down):
    def _A_ref(x, k_cache, v_cache, wq, wo):
        B, Sq, D = x.shape
        Hq, Dh = 32, 192
        Hkv, Sk = k_cache.shape[1], k_cache.shape[2]
        W = min(4096, max(256, Sk // 4))
        rep = Hq // Hkv
        q = (lambda x, *d: x.transpose(*d))((x @ wq).reshape(B, Sq, Hq, Dh), 0, 2, 1, 3)
        k = jnp.repeat(k_cache[:, :, Sk - W:, :], rep, axis=1)
        v = jnp.repeat(v_cache[:, :, Sk - W:, :], rep, axis=1)
        scores = jnp.einsum("bhqd,bhkd->bhqk", q, k) * (Dh ** -0.5)
        p = _softmax(scores, axis=-1)
        o = jnp.einsum("bhqk,bhkd->bhqd", p, v)
        return (lambda x, *d: x.transpose(*d))(o, 0, 2, 1, 3).reshape(B, Sq, Hq * Dh) @ wo

    def _B_ref(x, w_r, w_gate, w_up, w_down):
        B, S, D = x.shape
        C = 2
        r = x @ w_r
        idx = jnp.argsort(-r, axis=-1)[:, :C]
        idx_e = jnp.repeat(idx.reshape(B, C, 1), D, axis=2)
        x_sel = jnp.take_along_axis(x, idx_e, axis=1)
        g = _silu(x_sel @ w_gate)
        u = x_sel @ w_up
        y = (g * u) @ w_down
        r_sel = _sigmoid(jnp.take_along_axis(r, idx, axis=1))
        y = y * r_sel.reshape(B, C, 1)
        b_off = (jnp.arange(B) * S).reshape(B, 1)
        flat_idx = (idx + b_off).reshape(B * C)
        zero = (x * 0.0).reshape(B * S, D)
        upd = _scatter_add(zero, flat_idx, y.reshape(B * C, D), axis=0)
        return x + upd.reshape(B, S, D)

    x = A_x
    xn = _layernorm(x, axis=-1)
    s = _A_ref(xn, A_k_cache, A_v_cache, A_wq, A_wo)
    g = _silu(_B_ref(xn, B_w_r, B_w_gate, B_w_up, B_w_down))
    return x + s * g
```

```python
import functools
import math

import jax
import jax.numpy as jnp
import jax.experimental.pallas as pl
import jax.experimental.pallas.tpu as pltpu

S, D = 2048, 640
H, DH, W = 32, 192, 512
F = 1536
NP = H // 2
PW = 2 * DH
TQ = 512
NB = S // TQ
NJ = TQ // 128
NIT = NP * NB
KP = 256
NT_DIMS = (((1,), (1,)), ((), ()))
QSCALE = (DH ** -0.5) * math.log2(math.e)
EPS_BF16 = 1.0013580322265625e-05

bf16 = jnp.bfloat16
f32 = jnp.float32
u32 = jnp.uint32


def _rb(t):
    return t.astype(bf16).astype(f32)


def _sigmoid(t):
    return 1.0 / (1.0 + jnp.exp(-t))


def _pack(t):
    return pltpu.bitcast(t, u32)


def _unpack(t):
    return pltpu.bitcast(t, bf16)


def _dot(a, b):
    return jnp.dot(a, b, preferred_element_type=f32)


def _dot_nt(a, b):
    return jax.lax.dot_general(a, b, NT_DIMS, preferred_element_type=f32)


def _kernel(x_hbm, kt_hbm, vt_hbm, wq_hbm, wo_hbm, wr_ref, wg_hbm, wu_hbm, wd_hbm,
            out_hbm,
            x_ref, xn_ref, acc_ref, wq_ref, wo_ref, kt_ref, vt_ref, kb_ref, vb_ref, q_ref, o_ref,
            s_ref, m_ref,
            wg_ref, wu_ref, wd_ref, y_ref, out_ref,
            sem_x, sem_pair, sem_moe, sem_out):
    sk = kt_hbm.shape[-1]

    def x_copy(b):
        rows = pl.ds(b * 512, 512)
        return pltpu.make_async_copy(x_hbm.at[0, rows, :], x_ref.at[rows, :], sem_x.at[b])

    def pair_copies(p):
        cs = [pltpu.make_async_copy(wq_hbm.at[:, pl.ds(p * PW, PW)], wq_ref.at[p], sem_pair.at[p])]
        for h in range(2):
            cs.append(pltpu.make_async_copy(
                kt_hbm.at[0, 2 * p + h, :, pl.ds(sk - W, W)],
                kt_ref.at[2 * p + h, pl.ds(64 * h, DH), :], sem_pair.at[p]))
        for h in range(2):
            cs.append(pltpu.make_async_copy(
                vt_hbm.at[0, 2 * p + h, :, pl.ds(sk - W, W)],
                vt_ref.at[2 * p + h], sem_pair.at[p]))
        cs.append(pltpu.make_async_copy(wo_hbm.at[pl.ds(p * PW, PW), :], wo_ref.at[p], sem_pair.at[p]))
        return cs

    def moe_copies():
        return (pltpu.make_async_copy(wg_hbm, wg_ref, sem_moe.at[0]),
                pltpu.make_async_copy(wu_hbm, wu_ref, sem_moe.at[1]),
                pltpu.make_async_copy(wd_hbm, wd_ref, sem_moe.at[2]))

    for h in range(H):
        kt_ref[h, pl.ds(DH if h % 2 == 0 else 0, 64), :] = jnp.zeros((64, W), bf16)

    for b in range(S // 512):
        x_copy(b).start()
    for c in pair_copies(0):
        c.start()
    for c in pair_copies(1):
        c.start()
    for c in moe_copies():
        c.start()

    LN_ROWS = 256

    def ln_body(i, carry):
        rows = pl.ds(pl.multiple_of(i * LN_ROWS, LN_ROWS), LN_ROWS)
        prow = pl.ds(pl.multiple_of(i * (LN_ROWS // 2), LN_ROWS // 2), LN_ROWS // 2)
        xf = x_ref[rows, :].astype(f32)
        mean = jnp.sum(xf, axis=-1, keepdims=True) / D
        xc = xf - mean
        var = jnp.sum(xc * xc, axis=-1, keepdims=True) / D
        d = _rb(xf - _rb(mean))
        den = _rb(jnp.sqrt(_rb(_rb(var) + EPS_BF16)))
        xn_ref[prow, :] = _pack((d * (1.0 / den)).astype(bf16))
        acc_ref[rows, :] = jnp.zeros((LN_ROWS, D), f32)
        return carry

    for b in range(S // 512):
        x_copy(b).wait()
    jax.lax.fori_loop(0, S // LN_ROWS, ln_body, 0)

    wr8 = jnp.broadcast_to(wr_ref[...].reshape(1, D), (8, D))
    r8 = _dot_nt(wr8, _unpack(xn_ref[...]))
    r = _rb(r8[0:1, :])
    iota = jax.lax.broadcasted_iota(jnp.int32, (1, S), 1)
    m1 = jnp.max(r)
    i1 = jnp.minimum(jnp.min(jnp.where(r == m1, iota, S)), S - 1)
    r2 = jnp.where(iota == i1, -jnp.inf, r)
    m2 = jnp.max(r2)
    i2 = jnp.minimum(jnp.min(jnp.where(r2 == m2, iota, S)), S - 1)

    for c in moe_copies():
        c.wait()
    row16 = jax.lax.broadcasted_iota(jnp.int32, (16, D), 0)
    xs = jnp.zeros((16, D), f32)
    for j, idx in enumerate((i1, i2)):
        base = pl.multiple_of((idx // 16) * 8, 8)
        blk = _unpack(xn_ref[pl.ds(base, 8), :]).astype(f32)
        row = jnp.sum(jnp.where(row16 == idx - 2 * base, blk, 0.0), axis=0, keepdims=True)
        xs = jnp.where(row16 == j, row, xs)
    xs = xs.astype(bf16)
    g = _rb(_dot(xs, wg_ref[...]))
    g = _rb(g * _rb(_sigmoid(g)))
    u = _rb(_dot(xs, wu_ref[...]))
    gu = (g * u).astype(bf16)
    y = _rb(_dot(gu, wd_ref[...]))
    rs = jnp.where(row16 == 0, m1, m2)
    y_ref[...] = _rb(y * _rb(_sigmoid(rs)))

    def q_proj(i):
        p = i // NB
        prow = pl.ds(pl.multiple_of((i % NB) * (TQ // 2), TQ // 2), TQ // 2)
        q = _dot(_unpack(xn_ref[prow, :]), wq_ref[p])
        q_ref[...] = _pack((q * QSCALE).astype(bf16))

    def kv_prep(p, t):
        h = t // 2
        half = t % 2
        cols = pl.ds(pl.multiple_of(half * 256, 256), 256)
        prow = pl.ds(pl.multiple_of(half * 128, 128), 128)
        ku = _pack(kt_ref[2 * p + h, :, cols].T)
        ke = pltpu.unpack_elementwise(ku, index=0, packed_dtype=bf16, unpacked_dtype=f32)
        ko = pltpu.unpack_elementwise(ku, index=1, packed_dtype=bf16, unpacked_dtype=f32)
        kb_ref[p % 2, h, prow, :] = _pack(jnp.concatenate([ke, ko], axis=0).astype(bf16))
        vb_ref[p % 2, h, :, cols] = _pack(vt_ref[2 * p + h, :, cols])

    KSTEP = 4 // NB if NB <= 4 else 0

    for c in pair_copies(0):
        c.wait()
    for t in range(4):
        kv_prep(0, t)
    q_proj(0)


    def s_stage(i):
        slot = (i // NB) % 2
        for j in range(NJ):
            for h in range(2):
                qh = _unpack(q_ref[64 * j:64 * (j + 1), 128 * h:128 * h + 256])
                st = _dot_nt(_unpack(kb_ref[slot, h]), qh)
                s_ref[2 * j + h] = st
                m_ref[2 * j + h] = jnp.max(st.reshape(W // 8, 8, 128), axis=0)

    def c_stage():
        ls = []
        ps = []
        for u in range(2 * NJ):
            m = jnp.max(m_ref[u], axis=0, keepdims=True)
            pt = jnp.exp2(s_ref[u] - m)
            ls.append(jnp.sum(pt, axis=0, keepdims=True))
            ps.append(jnp.concatenate(
                [pltpu.pack_elementwise([pt[256 * c:256 * c + 128], pt[256 * c + 128:256 * c + 256]],
                                        packed_dtype=bf16) for c in range(2)], axis=0))
        return ls, ps

    def p_stage(i, ls, ps):
        slot = (i // NB) % 2
        os_ = []
        for j in range(NJ):
            ots = []
            for h in range(2):
                ot = _dot(_unpack(vb_ref[slot, h]), _unpack(ps[2 * j + h]))
                ots.append(ot * (1.0 / ls[2 * j + h]))
            os_.append(jnp.concatenate(ots, axis=0).T)
        o_ref[...] = _pack(jnp.concatenate(os_, axis=0).astype(bf16))

    def o_stage(i):
        p = i // NB
        rows = pl.ds(pl.multiple_of((i % NB) * TQ, TQ), TQ)
        acc_ref[rows, :] += _dot(_unpack(o_ref[...]), wo_ref[p])

    s_stage(0)
    o_ref[...] = jnp.zeros(o_ref.shape, u32)

    def pair_body(p, carry):
        @pl.when(p + 1 < NP)
        def _():
            for c in pair_copies(p + 1):
                c.wait()

        @pl.when(p + 2 < NP)
        def _():
            for c in pair_copies(p + 2):
                c.start()

        def body(b, carry):
            i = p * NB + b
            nxt = jnp.minimum(i + 1, NIT - 1)
            for t in range(4 // NB):
                kv_prep(jnp.minimum(p + 1, NP - 1), b * (4 // NB) + t)
            ls, ps = c_stage()
            q_proj(nxt)
            o_stage(jnp.maximum(i - 1, 0))
            p_stage(i, ls, ps)
            s_stage(nxt)
            return carry

        jax.lax.fori_loop(0, NB, body, 0, unroll=1)
        return carry

    jax.lax.fori_loop(0, NP, pair_body, 0)
    o_stage(NIT - 1)


    y1 = y_ref[0:1, :]
    y2 = y_ref[1:2, :]
    EP = 256

    def out_copy(t):
        rows = pl.ds(t * EP, EP)
        return pltpu.make_async_copy(out_ref.at[rows, :], out_hbm.at[0, rows, :], sem_out.at[t])

    def ep_body(t, carry):
        start = pl.multiple_of(t * EP, EP)
        rows = pl.ds(start, EP)
        prow = pl.ds(pl.multiple_of(t * (EP // 2), EP // 2), EP // 2)
        s = _rb(acc_ref[rows, :])
        rid = jax.lax.broadcasted_iota(jnp.int32, (EP, D), 0) + start
        upd = jnp.where(rid == i1, y1, jnp.where(rid == i2, y2, 0.0))
        gin = _rb(_unpack(xn_ref[prow, :]).astype(f32) + upd)
        g = _rb(gin * _rb(_sigmoid(gin)))
        out_ref[rows, :] = (x_ref[rows, :].astype(f32) + _rb(s * g)).astype(bf16)
        out_copy(t).start()
        return carry

    jax.lax.fori_loop(0, S // EP, ep_body, 0)
    for t in range(S // EP):
        out_copy(t).wait()


@jax.jit
def pallas_recurrent_scan__sliding_block_cached__moe_arch_mod__prompt_kernel(
    A_x, A_k_cache, A_v_cache, A_wq, A_wo, B_x, B_w_r, B_w_gate, B_w_up, B_w_down,
):
    kt = jnp.swapaxes(A_k_cache, 2, 3)
    vt = jnp.swapaxes(A_v_cache, 2, 3)
    any_spec = pl.BlockSpec(memory_space=pl.ANY)
    return pl.pallas_call(
        _kernel,
        in_specs=[any_spec, any_spec, any_spec, any_spec, any_spec,
                  pl.BlockSpec(memory_space=pltpu.VMEM),
                  any_spec, any_spec, any_spec],
        out_specs=any_spec,
        out_shape=jax.ShapeDtypeStruct(A_x.shape, A_x.dtype),
        scratch_shapes=[
            pltpu.VMEM((S, D), bf16),
            pltpu.VMEM((S // 2, D), u32),
            pltpu.VMEM((S, D), f32),
            pltpu.VMEM((NP, D, PW), bf16),
            pltpu.VMEM((NP, PW, D), bf16),
            pltpu.VMEM((H, KP, W), bf16),
            pltpu.VMEM((H, DH, W), bf16),
            pltpu.VMEM((2, 2, W // 2, KP), u32),
            pltpu.VMEM((2, 2, DH // 2, W), u32),
            pltpu.VMEM((TQ // 2, PW), u32),
            pltpu.VMEM((TQ // 2, PW), u32),
            pltpu.VMEM((2 * NJ, W, 128), f32),
            pltpu.VMEM((2 * NJ, 8, 128), f32),
            pltpu.VMEM((D, F), bf16),
            pltpu.VMEM((D, F), bf16),
            pltpu.VMEM((F, D), bf16),
            pltpu.VMEM((16, D), f32),
            pltpu.VMEM((S, D), bf16),
            pltpu.SemaphoreType.DMA((S // 512,)),
            pltpu.SemaphoreType.DMA((NP,)),
            pltpu.SemaphoreType.DMA((3,)),
            pltpu.SemaphoreType.DMA((S // 256,)),
        ],
        compiler_params=pltpu.CompilerParams(
            vmem_limit_bytes=128 * 1024 * 1024,
            disable_bounds_checks=True,
        ),
    )(A_x, kt, vt, A_wq, A_wo, B_w_r, B_w_gate, B_w_up, B_w_down)
```

```python
import math

import jax
import jax.numpy as jnp
import jax.experimental.pallas as pl
import jax.experimental.pallas.tpu as pltpu

S, D = 2048, 640
H, DH, W = 32, 192, 512
F = 1536
NP = H // 2
PW = 2 * DH
TQ = 512
NB = S // TQ
NJ = TQ // 128
NIT = NP * NB
KP = 256
GR = S // NIT
NT_DIMS = (((1,), (1,)), ((), ()))
QSCALE = (DH ** -0.5) * math.log2(math.e)
LOG2E = math.log2(math.e)
EPS_BF16 = 1.0013580322265625e-05

bf16 = jnp.bfloat16
f32 = jnp.float32
u32 = jnp.uint32
i32 = jnp.int32


def _rb(t):
    return t.astype(bf16).astype(f32)


def _sigmoid(t):
    return 1.0 / (1.0 + jnp.exp(-t))


def _pack(t):
    return pltpu.bitcast(t, u32)


def _unpack(t):
    return pltpu.bitcast(t, bf16)


def _even_odd(u):
    return (pltpu.unpack_elementwise(u, index=0, packed_dtype=bf16, unpacked_dtype=f32),
            pltpu.unpack_elementwise(u, index=1, packed_dtype=bf16, unpacked_dtype=f32))


def _pack2(e, o):
    return pltpu.pack_elementwise([e, o], packed_dtype=bf16)


def _dot(a, b):
    return jnp.dot(a, b, preferred_element_type=f32)


def _dot_nt(a, b):
    return jax.lax.dot_general(a, b, NT_DIMS, preferred_element_type=f32)


def _kernel(x_hbm, kt_hbm, vt_hbm, wq_hbm, wo_hbm, wr_ref, wg_hbm, wu_hbm, wd_hbm,
            out_hbm,
            x_ref, xn_ref, acc_ref, wq_ref, wo_ref, kt_ref, vt_ref, kb_ref, vb_ref,
            q_ref, o_ref, s_ref, m_ref, g_ref, top_ref,
            wg_ref, wu_ref, wd_ref, out_ref,
            sem_x, sem_p0, sem_pair, sem_moe, sem_out):
    sk = kt_hbm.shape[-1]

    def x_copy(b):
        rows = pl.ds(b * TQ, TQ)
        return pltpu.make_async_copy(x_hbm.at[0, rows, :], x_ref.at[rows, :], sem_x.at[b])

    def pair_copies(p, sems=None):
        sem = (lambda j: sem_pair.at[p]) if sems is None else (lambda j: sems.at[j])
        cs = [pltpu.make_async_copy(wq_hbm.at[:, pl.ds(p * PW, PW)], wq_ref.at[p], sem(0))]
        for h in range(2):
            cs.append(pltpu.make_async_copy(
                kt_hbm.at[0, 2 * p + h, :, pl.ds(sk - W, W)],
                kt_ref.at[2 * p + h, pl.ds(64 * h, DH), :], sem(1 + h)))
        for h in range(2):
            cs.append(pltpu.make_async_copy(
                vt_hbm.at[0, 2 * p + h, :, pl.ds(sk - W, W)],
                vt_ref.at[2 * p + h], sem(3 + h)))
        cs.append(pltpu.make_async_copy(wo_hbm.at[pl.ds(p * PW, PW), :], wo_ref.at[p], sem(5)))
        return cs

    def moe_copies():
        return (pltpu.make_async_copy(wg_hbm, wg_ref, sem_moe.at[0]),
                pltpu.make_async_copy(wu_hbm, wu_ref, sem_moe.at[1]),
                pltpu.make_async_copy(wd_hbm, wd_ref, sem_moe.at[2]))

    def out_copy(b):
        rows = pl.ds(b * TQ, TQ)
        return pltpu.make_async_copy(out_ref.at[rows, :], out_hbm.at[0, rows, :], sem_out.at[b])

    def layer_norm(b):
        for c in range(TQ // 128):
            r0 = b * TQ + c * 128
            outs = []
            for xf in _even_odd(_pack(x_ref[r0:r0 + 128, :])):
                mean = jnp.sum(xf, axis=-1, keepdims=True) / D
                xc = xf - mean
                var = jnp.sum(xc * xc, axis=-1, keepdims=True) / D
                d = _rb(xf - _rb(mean))
                den = _rb(jnp.sqrt(_rb(_rb(var) + EPS_BF16)))
                outs.append(d * (1.0 / den))
            xn_ref[r0 // 2:r0 // 2 + 64, :] = _pack2(*outs)

    def gate_router(c):
        prow = pl.ds(pl.multiple_of(c * (GR // 2), GR // 2), GR // 2)
        wr = wr_ref[...].astype(f32).reshape(1, D)
        gs = []
        row = jax.lax.broadcasted_iota(i32, (GR // 2, 128), 0)
        for par, xn in enumerate(_even_odd(xn_ref[prow, :])):
            gs.append(xn * _rb(_sigmoid(xn)))
            r = _rb(jnp.sum(xn * wr, axis=-1, keepdims=True))
            r = jnp.broadcast_to(r, (GR // 2, 128))
            idx = (c * GR + par + 2 * row).astype(f32)
            v1 = top_ref[par, 0]
            j1 = top_ref[par, 1]
            v2 = top_ref[par, 2]
            j2 = top_ref[par, 3]
            gt1 = r > v1
            gt2 = r > v2
            top_ref[par, 0] = jnp.where(gt1, r, v1)
            top_ref[par, 1] = jnp.where(gt1, idx, j1)
            top_ref[par, 2] = jnp.where(gt1, v1, jnp.where(gt2, r, v2))
            top_ref[par, 3] = jnp.where(gt1, j1, jnp.where(gt2, idx, j2))
        g_ref[prow, :] = _pack2(*gs)

    def q_stage(p, b):
        prow = pl.ds(pl.multiple_of(b * (TQ // 2), TQ // 2), TQ // 2)
        q = _dot(_unpack(xn_ref[prow, :]), wq_ref[p])
        q_ref[...] = _pack((q * QSCALE).astype(bf16))

    def k_prep(p, t):
        h = t // 2
        half = t % 2
        if isinstance(t, int):
            cols = pl.ds(half * 256, 256)
            prow = pl.ds(half * 128, 128)
        else:
            cols = pl.ds(pl.multiple_of(half * 256, 256), 256)
            prow = pl.ds(pl.multiple_of(half * 128, 128), 128)
        ke, ko = _even_odd(_pack(kt_ref[2 * p + h, :, cols].T))
        kb_ref[p % 2, h, prow, :] = _pack(jnp.concatenate([ke, ko], axis=0).astype(bf16))

    def v_prep(p, t):
        h = t // 2
        half = t % 2
        if isinstance(t, int):
            cols = pl.ds(half * 256, 256)
        else:
            cols = pl.ds(pl.multiple_of(half * 256, 256), 256)
        vb_ref[p % 2, h, :, cols] = _pack(vt_ref[2 * p + h, :, cols])

    def s_stage(p):
        slot = p % 2
        for j in range(NJ):
            for h in range(2):
                qh = _unpack(q_ref[64 * j:64 * (j + 1), 128 * h:128 * h + 256])
                st = _dot_nt(_unpack(kb_ref[slot, h]), qh)
                s_ref[2 * j + h] = st
                m_ref[2 * j + h] = jnp.max(st.reshape(W // 8, 8, 128), axis=0)

    def c_stage():
        ls = []
        ps = []
        for u in range(2 * NJ):
            m = jnp.max(m_ref[u], axis=0, keepdims=True)
            pt = jnp.exp2(s_ref[u] - m)
            ls.append(jnp.sum(pt, axis=0, keepdims=True))
            ps.append(jnp.concatenate(
                [_pack2(pt[256 * c:256 * c + 128], pt[256 * c + 128:256 * c + 256])
                 for c in range(2)], axis=0))
        return ls, ps

    def p_stage(p, ls, ps):
        slot = p % 2
        os_ = []
        for j in range(NJ):
            ots = []
            for h in range(2):
                ot = _dot(_unpack(vb_ref[slot, h]), _unpack(ps[2 * j + h]))
                ots.append(ot * (1.0 / ls[2 * j + h]))
            os_.append(jnp.concatenate(ots, axis=0).T)
        o_ref[...] = _pack(jnp.concatenate(os_, axis=0).astype(bf16))

    def o_dot(p):
        return _dot(_unpack(o_ref[...]), wo_ref[p])

    def rows_of(b):
        if isinstance(b, int):
            return pl.ds(b * TQ, TQ)
        return pl.ds(pl.multiple_of(b * TQ, TQ), TQ)

    def finish(b, s):
        rows = rows_of(b)
        g = _unpack(g_ref[b * (TQ // 2):(b + 1) * (TQ // 2), :]).astype(f32)
        out_ref[rows, :] = (x_ref[rows, :].astype(f32) + _rb(_rb(s) * g)).astype(bf16)

    p0 = pair_copies(0, sem_p0)
    x_copy(0).start()
    p0[0].start()
    p0[1].start()
    p0[2].start()
    for h in range(H):
        kt_ref[h, pl.ds(DH if h % 2 == 0 else 0, 64), :] = jnp.zeros((64, W), bf16)
    neg = jnp.full((GR // 2, 128), -jnp.inf, f32)
    big = jnp.full((GR // 2, 128), float(S), f32)
    for par in range(2):
        top_ref[par, 0] = neg
        top_ref[par, 1] = big
        top_ref[par, 2] = neg
        top_ref[par, 3] = big

    x_copy(0).wait()
    x_copy(1).start()
    p0[3].start()
    p0[4].start()
    layer_norm(0)

    p0[0].wait()
    p0[1].wait()
    p0[2].wait()
    x_copy(2).start()
    x_copy(3).start()
    p0[5].start()
    for t in range(4):
        k_prep(0, t)
    q_stage(0, 0)

    x_copy(1).wait()
    p0[3].wait()
    p0[4].wait()
    for c in pair_copies(1):
        c.start()
    for t in range(4):
        v_prep(0, t)
    layer_norm(1)
    s_stage(0)

    x_copy(2).wait()
    x_copy(3).wait()
    p0[5].wait()
    for c in pair_copies(1):
        c.wait()
    for c in pair_copies(2):
        c.start()
    for c in moe_copies():
        c.start()
    k_prep(1, 0)
    v_prep(1, 0)
    layer_norm(2)
    layer_norm(3)
    gate_router(0)
    gate_router(1)
    acc_ref[...] = jnp.zeros(acc_ref.shape, f32)
    ls, ps = c_stage()
    q_stage(0, 1)
    p_stage(0, ls, ps)
    s_stage(0)

    def pair_body(p, carry):
        @pl.when(jnp.logical_and(p >= 1, p + 1 < NP))
        def _():
            for c in pair_copies(p + 1):
                c.wait()

        @pl.when(jnp.logical_and(p >= 1, p + 2 < NP))
        def _():
            for c in pair_copies(p + 2):
                c.start()

        pn = jnp.where(p + 1 < NP, p + 1, p - 1)

        def body(b, carry):
            i = p * NB + b
            nxt = i + 1
            prv = i - 1
            k_prep(pn, b)
            v_prep(pn, b)
            gate_router(nxt)
            ls, ps = c_stage()
            q_stage(nxt // NB, nxt % NB)
            acc_ref[rows_of(prv % NB), :] += o_dot(prv // NB)
            p_stage(p, ls, ps)
            s_stage(nxt // NB)
            return carry

        lo = jnp.where(p == 0, 1, 0)
        hi = jnp.where(p == NP - 1, NB - 1, NB)
        jax.lax.fori_loop(lo, hi, body, 0)
        return carry

    jax.lax.fori_loop(0, NP, pair_body, 0)

    vals = jnp.concatenate([top_ref[0, 0], top_ref[1, 0], top_ref[0, 2], top_ref[1, 2]], axis=0)
    idxs = jnp.concatenate([top_ref[0, 1], top_ref[1, 1], top_ref[0, 3], top_ref[1, 3]], axis=0)
    m1 = jnp.max(vals)
    j1 = jnp.min(jnp.where(vals == m1, idxs, float(S)))
    vals2 = jnp.where(idxs == j1, -jnp.inf, vals)
    m2 = jnp.max(vals2)
    j2 = jnp.min(jnp.where(vals2 == m2, idxs, float(S)))
    i1 = jnp.clip(j1.astype(i32), 0, S - 1)
    i2 = jnp.clip(j2.astype(i32), 0, S - 1)

    for c in moe_copies():
        c.wait()
    row16 = jax.lax.broadcasted_iota(i32, (16, D), 0)
    xrows = []
    for idx in (i1, i2):
        e, o = _even_odd(xn_ref[pl.ds(idx // 2, 1), :])
        xrows.append(jnp.where(idx % 2 == 0, e, o))
    xs = jnp.where(row16 == 0, xrows[0], jnp.where(row16 == 1, xrows[1], 0.0)).astype(bf16)
    hg = _rb(_dot(xs, wg_ref[...]))
    hg = _rb(hg * _rb(_sigmoid(hg)))
    hu = _rb(_dot(xs, wu_ref[...]))
    y = _rb(_dot((hg * hu).astype(bf16), wd_ref[...]))
    rs = jnp.where(row16 == 0, m1, m2)
    y = _rb(y * _rb(_sigmoid(rs)))
    for j, idx in enumerate((i1, i2)):
        gin = _rb(xrows[j] + y[j:j + 1, :])
        gbits = pltpu.bitcast(_rb(gin * _rb(_sigmoid(gin))), u32)
        word = pl.ds(idx // 2, 1)
        old = g_ref[word, :]
        g_ref[word, :] = jnp.where(idx % 2 == 0,
                                   (old & jnp.uint32(0xFFFF0000)) | (gbits >> 16),
                                   (old & jnp.uint32(0x0000FFFF)) | gbits)

    ls, ps = c_stage()
    acc_ref[rows_of(NB - 2), :] += o_dot(NP - 1)
    p_stage(NP - 1, ls, ps)
    finish(0, acc_ref[rows_of(0), :])
    finish(1, acc_ref[rows_of(1), :])
    out_copy(0).start()
    out_copy(1).start()

    finish(2, acc_ref[rows_of(2), :])
    finish(3, acc_ref[rows_of(3), :] + o_dot(NP - 1))
    out_copy(2).start()
    out_copy(3).start()
    for b in range(NB):
        out_copy(b).wait()


@jax.jit
def pallas_recurrent_scan__sliding_block_cached__moe_arch_mod__prompt_kernel(
    A_x, A_k_cache, A_v_cache, A_wq, A_wo, B_x, B_w_r, B_w_gate, B_w_up, B_w_down,
):
    kt = jnp.swapaxes(A_k_cache, 2, 3)
    vt = jnp.swapaxes(A_v_cache, 2, 3)
    any_spec = pl.BlockSpec(memory_space=pl.ANY)
    return pl.pallas_call(
        _kernel,
        in_specs=[any_spec, any_spec, any_spec, any_spec, any_spec,
                  pl.BlockSpec(memory_space=pltpu.VMEM),
                  any_spec, any_spec, any_spec],
        out_specs=any_spec,
        out_shape=jax.ShapeDtypeStruct(A_x.shape, A_x.dtype),
        scratch_shapes=[
            pltpu.VMEM((S, D), bf16),
            pltpu.VMEM((S // 2, D), u32),
            pltpu.VMEM((S, D), f32),
            pltpu.VMEM((NP, D, PW), bf16),
            pltpu.VMEM((NP, PW, D), bf16),
            pltpu.VMEM((H, KP, W), bf16),
            pltpu.VMEM((H, DH, W), bf16),
            pltpu.VMEM((2, 2, W // 2, KP), u32),
            pltpu.VMEM((2, 2, DH // 2, W), u32),
            pltpu.VMEM((TQ // 2, PW), u32),
            pltpu.VMEM((TQ // 2, PW), u32),
            pltpu.VMEM((2 * NJ, W, 128), f32),
            pltpu.VMEM((2 * NJ, 8, 128), f32),
            pltpu.VMEM((S // 2, D), u32),
            pltpu.VMEM((2, 4, GR // 2, 128), f32),
            pltpu.VMEM((D, F), bf16),
            pltpu.VMEM((D, F), bf16),
            pltpu.VMEM((F, D), bf16),
            pltpu.VMEM((S, D), bf16),
            pltpu.SemaphoreType.DMA((NB,)),
            pltpu.SemaphoreType.DMA((6,)),
            pltpu.SemaphoreType.DMA((NP,)),
            pltpu.SemaphoreType.DMA((3,)),
            pltpu.SemaphoreType.DMA((NB,)),
        ],
        compiler_params=pltpu.CompilerParams(
            vmem_limit_bytes=128 * 1024 * 1024,
            disable_bounds_checks=True,
        ),
    )(A_x, kt, vt, A_wq, A_wo, B_w_r, B_w_gate, B_w_up, B_w_down)
```

```python
import math

import jax
import jax.numpy as jnp
import jax.experimental.pallas as pl
import jax.experimental.pallas.tpu as pltpu

S, D = 2048, 640
H, DH, W = 32, 192, 512
F = 1536
NP = H // 2
PW = 2 * DH
TQ = 512
NB = S // TQ
NJ = TQ // 128
NIT = NP * NB
KP = 256
GR = S // NIT
ROUTER_LEAD = 4
NT_DIMS = (((1,), (1,)), ((), ()))
QSCALE = (DH ** -0.5) * math.log2(math.e)
LOG2E = math.log2(math.e)
EPS_BF16 = 1.0013580322265625e-05

bf16 = jnp.bfloat16
f32 = jnp.float32
u32 = jnp.uint32
i32 = jnp.int32


def _rb(t):
    return t.astype(bf16).astype(f32)


def _sigmoid(t):
    return 0.5 * jnp.tanh(0.5 * t) + 0.5


def _recip(t):
    r = pl.reciprocal(t, approx=True)
    return r * (2.0 - t * r)


def _pack(t):
    return pltpu.bitcast(t, u32)


def _unpack(t):
    return pltpu.bitcast(t, bf16)


def _even_odd(u):
    return (pltpu.unpack_elementwise(u, index=0, packed_dtype=bf16, unpacked_dtype=f32),
            pltpu.unpack_elementwise(u, index=1, packed_dtype=bf16, unpacked_dtype=f32))


def _pack2(e, o):
    return pltpu.pack_elementwise([e, o], packed_dtype=bf16)


def _dot(a, b):
    return jnp.dot(a, b, preferred_element_type=f32)


def _dot_nt(a, b):
    return jax.lax.dot_general(a, b, NT_DIMS, preferred_element_type=f32)


def _kernel(x_hbm, kt_hbm, vt_hbm, wq_hbm, wo_hbm, wr_ref, wg_hbm, wu_hbm, wd_hbm,
            out_hbm,
            x_ref, xn_ref, acc_ref, wq_ref, wo_ref, kt_ref, vt_ref, kb_ref, vb_ref,
            q_ref, o_ref, s_ref, m_ref, g_ref, top_ref,
            wg_ref, wu_ref, wd_ref, out_ref,
            sem_x, sem_p0, sem_pair, sem_moe, sem_out):
    sk = kt_hbm.shape[-1]

    def x_copy(b):
        rows = pl.ds(b * TQ, TQ)
        return pltpu.make_async_copy(x_hbm.at[0, rows, :], x_ref.at[rows, :], sem_x.at[b])

    def pair_copies(p, sems=None):
        sem = (lambda j: sem_pair.at[p]) if sems is None else (lambda j: sems.at[j])
        cs = [pltpu.make_async_copy(wq_hbm.at[:, pl.ds(p * PW, PW)], wq_ref.at[p], sem(0))]
        for h in range(2):
            cs.append(pltpu.make_async_copy(
                kt_hbm.at[0, 2 * p + h, :, pl.ds(sk - W, W)],
                kt_ref.at[2 * p + h], sem(1 + h)))
        for h in range(2):
            cs.append(pltpu.make_async_copy(
                vt_hbm.at[0, 2 * p + h, :, pl.ds(sk - W, W)],
                vt_ref.at[2 * p + h], sem(3 + h)))
        cs.append(pltpu.make_async_copy(wo_hbm.at[pl.ds(p * PW, PW), :], wo_ref.at[p], sem(5)))
        return cs

    def moe_copies():
        return (pltpu.make_async_copy(wg_hbm, wg_ref, sem_moe.at[0]),
                pltpu.make_async_copy(wu_hbm, wu_ref, sem_moe.at[1]),
                pltpu.make_async_copy(wd_hbm, wd_ref, sem_moe.at[2]))

    def out_copy(b):
        rows = pl.ds(b * TQ, TQ)
        return pltpu.make_async_copy(out_ref.at[rows, :], out_hbm.at[0, rows, :], sem_out.at[b])

    def layer_norm(b):
        for c in range(TQ // 128):
            r0 = b * TQ + c * 128
            outs = []
            for xf in _even_odd(_pack(x_ref[r0:r0 + 128, :])):
                mean = jnp.sum(xf, axis=-1, keepdims=True) * (1.0 / D)
                xc = xf - mean
                var = jnp.sum(xc * xc, axis=-1, keepdims=True) * (1.0 / D)
                d = _rb(xf - _rb(mean))
                ve = _rb(_rb(var) + EPS_BF16)
                den = _rb(ve * jax.lax.rsqrt(ve))
                outs.append(d * _recip(den))
            xn_ref[r0 // 2:r0 // 2 + 64, :] = _pack2(*outs)

    def gate_router(c):
        valid = c < NIT
        c = jnp.minimum(c, NIT - 1)
        prow = pl.ds(pl.multiple_of(c * (GR // 2), GR // 2), GR // 2)
        wr = wr_ref[...].astype(f32).reshape(1, D)
        gs = []
        row = jax.lax.broadcasted_iota(i32, (GR // 2, 128), 0)
        for par, xn in enumerate(_even_odd(xn_ref[prow, :])):
            gs.append(xn * _rb(_sigmoid(xn)))
            r = _rb(jnp.sum(xn * wr, axis=-1, keepdims=True))
            r = jnp.where(valid, jnp.broadcast_to(r, (GR // 2, 128)), -jnp.inf)
            idx = (c * GR + par + 2 * row).astype(f32)
            v1 = top_ref[par, 0]
            j1 = top_ref[par, 1]
            v2 = top_ref[par, 2]
            j2 = top_ref[par, 3]
            gt1 = r > v1
            gt2 = r > v2
            top_ref[par, 0] = jnp.where(gt1, r, v1)
            top_ref[par, 1] = jnp.where(gt1, idx, j1)
            top_ref[par, 2] = jnp.where(gt1, v1, jnp.where(gt2, r, v2))
            top_ref[par, 3] = jnp.where(gt1, j1, jnp.where(gt2, idx, j2))
        g_ref[prow, :] = _pack2(*gs)

    def q_stage(p, b):
        prow = pl.ds(pl.multiple_of(b * (TQ // 2), TQ // 2), TQ // 2)
        q = _dot(_unpack(xn_ref[prow, :]), wq_ref[p])
        q_ref[...] = _pack((q * QSCALE).astype(bf16))

    def _quarter(t):
        if isinstance(t, int):
            return pl.ds(t * 128, 128), pl.ds(t * 64, 64)
        return (pl.ds(pl.multiple_of(t * 128, 128), 128), pl.ds(pl.multiple_of(t * 64, 64), 64))

    def k_prep(p, t):
        cols, prow = _quarter(t)
        zpad = jnp.zeros((KP - DH, 128), bf16)
        for h in range(2):
            kt = kt_ref[2 * p + h, :, cols]
            kt = jnp.concatenate([kt, zpad] if h == 0 else [zpad, kt], axis=0)
            ke, ko = _even_odd(_pack(kt.T))
            kb_ref[p % 2, h, prow, :] = _pack(jnp.concatenate([ke, ko], axis=0).astype(bf16))

    def v_prep(p, t):
        cols, _ = _quarter(t)
        for h in range(2):
            vb_ref[p % 2, h, :, cols] = _pack(vt_ref[2 * p + h, :, cols])

    def s_stage(p):
        slot = p % 2
        for j in range(NJ):
            for h in range(2):
                qh = _unpack(q_ref[64 * j:64 * (j + 1), 128 * h:128 * h + 256])
                st = _dot_nt(_unpack(kb_ref[slot, h]), qh)
                s_ref[2 * j + h] = st
                m_ref[2 * j + h] = jnp.max(st.reshape(W // 8, 8, 128), axis=0)

    def c_stage():
        ls = []
        ps = []
        for u in range(2 * NJ):
            m = jnp.max(m_ref[u], axis=0, keepdims=True)
            pt = jnp.exp2(s_ref[u] - m)
            ls.append(jnp.sum(pt, axis=0, keepdims=True))
            ps.append(jnp.concatenate(
                [_pack2(pt[128 * c:128 * c + 64], pt[128 * c + 64:128 * c + 128])
                 for c in range(W // 128)], axis=0))
        return ls, ps

    def p_stage(p, ls, ps):
        slot = p % 2
        os_ = []
        for j in range(NJ):
            ots = []
            for h in range(2):
                ot = _dot(_unpack(vb_ref[slot, h]), _unpack(ps[2 * j + h]))
                ots.append(ot * (1.0 / ls[2 * j + h]))
            os_.append(jnp.concatenate(ots, axis=0).T)
        o_ref[...] = _pack(jnp.concatenate(os_, axis=0).astype(bf16))

    def o_dot(p):
        return _dot(_unpack(o_ref[...]), wo_ref[p])

    def rows_of(b):
        if isinstance(b, int):
            return pl.ds(b * TQ, TQ)
        return pl.ds(pl.multiple_of(b * TQ, TQ), TQ)

    def finish(b, s):
        rows = rows_of(b)
        if isinstance(b, int):
            prow = pl.ds(b * (TQ // 2), TQ // 2)
        else:
            prow = pl.ds(pl.multiple_of(b * (TQ // 2), TQ // 2), TQ // 2)
        g = _unpack(g_ref[prow, :]).astype(f32)
        out_ref[rows, :] = (x_ref[rows, :].astype(f32) + _rb(_rb(s) * g)).astype(bf16)

    p0 = pair_copies(0, sem_p0)
    x_copy(0).start()
    p0[0].start()
    p0[1].start()
    p0[2].start()
    acc_ref[...] = jnp.zeros(acc_ref.shape, f32)
    neg = jnp.full((GR // 2, 128), -jnp.inf, f32)
    big = jnp.full((GR // 2, 128), float(S), f32)
    for par in range(2):
        top_ref[par, 0] = neg
        top_ref[par, 1] = big
        top_ref[par, 2] = neg
        top_ref[par, 3] = big

    x_copy(0).wait()
    x_copy(1).start()
    p0[3].start()
    p0[4].start()
    layer_norm(0)

    for j in range(5):
        p0[j].wait()
    x_copy(1).wait()
    x_copy(2).start()
    x_copy(3).start()
    p0[5].start()
    for c in pair_copies(1):
        c.start()
    for t in range(4):
        k_prep(0, t)
    q_stage(0, 0)
    for t in range(4):
        v_prep(0, t)
    layer_norm(1)
    for c in range(ROUTER_LEAD):
        gate_router(c)
    s_stage(0)

    x_copy(2).wait()
    x_copy(3).wait()
    p0[5].wait()
    for c in pair_copies(1):
        c.wait()
    for c in pair_copies(2):
        c.start()
    for c in moe_copies():
        c.start()
    k_prep(1, 0)
    v_prep(1, 0)
    ls, ps = c_stage()
    q_stage(0, 1)
    p_stage(0, ls, ps)
    s_stage(0)
    layer_norm(2)
    layer_norm(3)
    gate_router(ROUTER_LEAD)

    def pair_body(p, carry):
        @pl.when(jnp.logical_and(p >= 1, p + 1 < NP))
        def _():
            for c in pair_copies(p + 1):
                c.wait()

        @pl.when(jnp.logical_and(p >= 1, p + 2 < NP))
        def _():
            for c in pair_copies(p + 2):
                c.start()

        pn = jnp.where(p + 1 < NP, p + 1, p - 1)

        def body(b, carry):
            i = p * NB + b
            nxt = i + 1
            prv = i - 1
            k_prep(pn, b)
            v_prep(pn, b)
            gate_router(i + ROUTER_LEAD)
            ls, ps = c_stage()
            q_stage(nxt // NB, nxt % NB)
            acc_ref[rows_of(prv % NB), :] += o_dot(prv // NB)
            p_stage(p, ls, ps)
            s_stage(nxt // NB)
            return carry

        lo = jnp.where(p == 0, 1, 0)
        hi = jnp.where(p == NP - 1, 1, NB)
        jax.lax.fori_loop(lo, hi, body, 0)
        return carry

    jax.lax.fori_loop(0, NP, pair_body, 0)

    vals = jnp.concatenate([top_ref[0, 0], top_ref[1, 0], top_ref[0, 2], top_ref[1, 2]], axis=0)
    idxs = jnp.concatenate([top_ref[0, 1], top_ref[1, 1], top_ref[0, 3], top_ref[1, 3]], axis=0)
    m1 = jnp.max(vals)
    j1 = jnp.min(jnp.where(vals == m1, idxs, float(S)))
    vals2 = jnp.where(idxs == j1, -jnp.inf, vals)
    m2 = jnp.max(vals2)
    j2 = jnp.min(jnp.where(vals2 == m2, idxs, float(S)))
    i1 = jnp.clip(j1.astype(i32), 0, S - 1)
    i2 = jnp.clip(j2.astype(i32), 0, S - 1)

    for c in moe_copies():
        c.wait()
    row16 = jax.lax.broadcasted_iota(i32, (16, D), 0)
    xrows = []
    for idx in (i1, i2):
        e, o = _even_odd(xn_ref[pl.ds(idx // 2, 1), :])
        xrows.append(jnp.where(idx % 2 == 0, e, o))
    xs = jnp.where(row16 == 0, xrows[0], jnp.where(row16 == 1, xrows[1], 0.0)).astype(bf16)
    hg = _rb(_dot(xs, wg_ref[...]))
    hg = _rb(hg * _rb(_sigmoid(hg)))
    hu = _rb(_dot(xs, wu_ref[...]))
    y = _rb(_dot((hg * hu).astype(bf16), wd_ref[...]))
    rs = jnp.where(row16 == 0, m1, m2)
    y = _rb(y * _rb(_sigmoid(rs)))
    for j, idx in enumerate((i1, i2)):
        gin = _rb(xrows[j] + y[j:j + 1, :])
        gbits = pltpu.bitcast(_rb(gin * _rb(_sigmoid(gin))), u32)
        word = pl.ds(idx // 2, 1)
        old = g_ref[word, :]
        g_ref[word, :] = jnp.where(idx % 2 == 0,
                                   (old & jnp.uint32(0xFFFF0000)) | (gbits >> 16),
                                   (old & jnp.uint32(0x0000FFFF)) | gbits)

    def tail_body(b, carry):
        ls, ps = c_stage()
        q_stage(NP - 1, b + 1)
        finish(b - 1, acc_ref[rows_of(b - 1), :] + o_dot(NP - 1))
        p_stage(NP - 1, ls, ps)
        s_stage(NP - 1)
        out_copy(b - 1).start()
        return carry

    jax.lax.fori_loop(1, NB - 1, tail_body, 0)

    ls, ps = c_stage()
    finish(NB - 2, acc_ref[rows_of(NB - 2), :] + o_dot(NP - 1))
    p_stage(NP - 1, ls, ps)
    out_copy(NB - 2).start()

    finish(NB - 1, acc_ref[rows_of(NB - 1), :] + o_dot(NP - 1))
    out_copy(NB - 1).start()
    for b in range(NB):
        out_copy(b).wait()


@jax.jit
def pallas_recurrent_scan__sliding_block_cached__moe_arch_mod__prompt_kernel(
    A_x, A_k_cache, A_v_cache, A_wq, A_wo, B_x, B_w_r, B_w_gate, B_w_up, B_w_down,
):
    kt = jnp.swapaxes(A_k_cache, 2, 3)
    vt = jnp.swapaxes(A_v_cache, 2, 3)
    any_spec = pl.BlockSpec(memory_space=pl.ANY)
    return pl.pallas_call(
        _kernel,
        in_specs=[any_spec, any_spec, any_spec, any_spec, any_spec,
                  pl.BlockSpec(memory_space=pltpu.VMEM),
                  any_spec, any_spec, any_spec],
        out_specs=any_spec,
        out_shape=jax.ShapeDtypeStruct(A_x.shape, A_x.dtype),
        scratch_shapes=[
            pltpu.VMEM((S, D), bf16),
            pltpu.VMEM((S // 2, D), u32),
            pltpu.VMEM((S, D), f32),
            pltpu.VMEM((NP, D, PW), bf16),
            pltpu.VMEM((NP, PW, D), bf16),
            pltpu.VMEM((H, DH, W), bf16),
            pltpu.VMEM((H, DH, W), bf16),
            pltpu.VMEM((2, 2, W // 2, KP), u32),
            pltpu.VMEM((2, 2, DH // 2, W), u32),
            pltpu.VMEM((TQ // 2, PW), u32),
            pltpu.VMEM((TQ // 2, PW), u32),
            pltpu.VMEM((2 * NJ, W, 128), f32),
            pltpu.VMEM((2 * NJ, 8, 128), f32),
            pltpu.VMEM((S // 2, D), u32),
            pltpu.VMEM((2, 4, GR // 2, 128), f32),
            pltpu.VMEM((D, F), bf16),
            pltpu.VMEM((D, F), bf16),
            pltpu.VMEM((F, D), bf16),
            pltpu.VMEM((S, D), bf16),
            pltpu.SemaphoreType.DMA((NB,)),
            pltpu.SemaphoreType.DMA((6,)),
            pltpu.SemaphoreType.DMA((NP,)),
            pltpu.SemaphoreType.DMA((3,)),
            pltpu.SemaphoreType.DMA((NB,)),
        ],
        compiler_params=pltpu.CompilerParams(
            vmem_limit_bytes=128 * 1024 * 1024,
            disable_bounds_checks=True,
        ),
    )(A_x, kt, vt, A_wq, A_wo, B_w_r, B_w_gate, B_w_up, B_w_down)
```

```python
import math

import jax
import jax.numpy as jnp
import jax.experimental.pallas as pl
import jax.experimental.pallas.tpu as pltpu

S, D = 2048, 640
H, DH, W = 32, 192, 512
F = 1536
NP = H // 2
PW = 2 * DH
TQ = 512
NB = S // TQ
NJ = TQ // 128
NIT = NP * NB
KP = 256
GR = S // NIT
ROUTER_LEAD = 4
NT_DIMS = (((1,), (1,)), ((), ()))
QSCALE = (DH ** -0.5) * math.log2(math.e)
LOG2E = math.log2(math.e)
EPS_BF16 = 1.0013580322265625e-05

bf16 = jnp.bfloat16
f32 = jnp.float32
u32 = jnp.uint32
i32 = jnp.int32


def _rb(t):
    return t.astype(bf16).astype(f32)


def _sigmoid(t):
    return 0.5 * jnp.tanh(0.5 * t) + 0.5


def _recip(t):
    r = pl.reciprocal(t, approx=True)
    return r * (2.0 - t * r)


def _pack(t):
    return pltpu.bitcast(t, u32)


def _unpack(t):
    return pltpu.bitcast(t, bf16)


def _even_odd(u):
    return (pltpu.unpack_elementwise(u, index=0, packed_dtype=bf16, unpacked_dtype=f32),
            pltpu.unpack_elementwise(u, index=1, packed_dtype=bf16, unpacked_dtype=f32))


def _pack2(e, o):
    return pltpu.pack_elementwise([e, o], packed_dtype=bf16)


def _dot(a, b):
    return jnp.dot(a, b, preferred_element_type=f32)


def _dot_nt(a, b):
    return jax.lax.dot_general(a, b, NT_DIMS, preferred_element_type=f32)


def _span(i, n):
    if isinstance(i, int):
        return pl.ds(i * n, n)
    return pl.ds(pl.multiple_of(i * n, n), n)


def _kernel(x_hbm, kt_hbm, vt_hbm, wq_hbm, wo_hbm, wr_ref, wg_hbm, wu_hbm, wd_hbm,
            out_hbm,
            x_ref, xn_ref, acc_ref, wq_ref, wo_ref, kt_ref, vt_ref, kb_ref, vb_ref,
            q_ref, o_ref, s_ref, m_ref, g_ref, top_ref,
            wg_ref, wu_ref, wd_ref, out_ref,
            sem_x, sem_g0, sem_g1, sem_g2, sem_g3, sem_moe, sem_out):
    sk = kt_hbm.shape[-1]

    win = pl.ds(sk - W, W)

    def x_copy(r0, n, sem):
        rows = pl.ds(r0, n)
        return pltpu.make_async_copy(x_hbm.at[0, rows, :], x_ref.at[rows, :], sem)

    def wq_copy(p0, n, sem):
        cols = pl.ds(p0 * PW, n * PW)
        return pltpu.make_async_copy(wq_hbm.at[:, cols], wq_ref.at[:, cols], sem)

    def wo_copy(p0, n, sem):
        rows = pl.ds(p0 * PW, n * PW)
        return pltpu.make_async_copy(wo_hbm.at[rows, :], wo_ref.at[rows, :], sem)

    def kv_copy(src, dst, p0, n, sem):
        heads = pl.ds(2 * p0, 2 * n)
        return pltpu.make_async_copy(src.at[0, heads, :, win], dst.at[heads], sem)

    def group_copies(p0, n, sems):
        return [wq_copy(p0, n, sems.at[0]), kv_copy(kt_hbm, kt_ref, p0, n, sems.at[1]),
                kv_copy(vt_hbm, vt_ref, p0, n, sems.at[2]), wo_copy(p0, n, sems.at[3])]

    x0_copies = [x_copy(c * 128, 128, sem_x.at[c]) for c in range(4)]
    x_copies = [None] + [x_copy(b * TQ, TQ, sem_x.at[3 + b]) for b in range(1, NB)]
    g0 = group_copies(0, 1, sem_g0)
    g1 = group_copies(1, 1, sem_g1)
    g2 = group_copies(2, 2, sem_g2)
    g3 = group_copies(4, NP - 4, sem_g3)
    moe_copies = [pltpu.make_async_copy(wg_hbm, wg_ref, sem_moe.at[0]),
                  pltpu.make_async_copy(wu_hbm, wu_ref, sem_moe.at[1]),
                  pltpu.make_async_copy(wd_hbm, wd_ref, sem_moe.at[2])]

    def out_copy(b):
        rows = pl.ds(b * TQ, TQ)
        return pltpu.make_async_copy(out_ref.at[rows, :], out_hbm.at[0, rows, :], sem_out.at[b])

    def layer_norm_rows(r0):
        outs = []
        for xf in _even_odd(_pack(x_ref[r0:r0 + 128, :])):
            mean = jnp.sum(xf, axis=-1, keepdims=True) * (1.0 / D)
            xc = xf - mean
            var = jnp.sum(xc * xc, axis=-1, keepdims=True) * (1.0 / D)
            d = _rb(xf - _rb(mean))
            ve = _rb(_rb(var) + EPS_BF16)
            den = _rb(ve * jax.lax.rsqrt(ve))
            outs.append(d * _recip(den))
        xn_ref[r0 // 2:r0 // 2 + 64, :] = _pack2(*outs)

    def layer_norm(b):
        for c in range(TQ // 128):
            layer_norm_rows(b * TQ + c * 128)

    def gate_router(c):
        valid = c < NIT
        c = jnp.minimum(c, NIT - 1)
        prow = pl.ds(pl.multiple_of(c * (GR // 2), GR // 2), GR // 2)
        wr = wr_ref[...].astype(f32).reshape(1, D)
        gs = []
        row = jax.lax.broadcasted_iota(i32, (GR // 2, 128), 0)
        for par, xn in enumerate(_even_odd(xn_ref[prow, :])):
            gs.append(xn * _rb(_sigmoid(xn)))
            r = _rb(jnp.sum(xn * wr, axis=-1, keepdims=True))
            r = jnp.where(valid, jnp.broadcast_to(r, (GR // 2, 128)), -jnp.inf)
            idx = (c * GR + par + 2 * row).astype(f32)
            v1 = top_ref[par, 0]
            j1 = top_ref[par, 1]
            v2 = top_ref[par, 2]
            j2 = top_ref[par, 3]
            gt1 = r > v1
            gt2 = r > v2
            top_ref[par, 0] = jnp.where(gt1, r, v1)
            top_ref[par, 1] = jnp.where(gt1, idx, j1)
            top_ref[par, 2] = jnp.where(gt1, v1, jnp.where(gt2, r, v2))
            top_ref[par, 3] = jnp.where(gt1, j1, jnp.where(gt2, idx, j2))
        g_ref[prow, :] = _pack2(*gs)

    def q_stage(p, b):
        prow = pl.ds(pl.multiple_of(b * (TQ // 2), TQ // 2), TQ // 2)
        q = _dot(_unpack(xn_ref[prow, :]), wq_ref[:, _span(p, PW)])
        q_ref[...] = _pack((q * QSCALE).astype(bf16))

    def _quarter(t):
        if isinstance(t, int):
            return pl.ds(t * 128, 128), pl.ds(t * 64, 64)
        return (pl.ds(pl.multiple_of(t * 128, 128), 128), pl.ds(pl.multiple_of(t * 64, 64), 64))

    def k_prep(p, t, dst=None):
        dst = p if dst is None else dst
        cols, prow = _quarter(t)
        zpad = jnp.zeros((KP - DH, 128), bf16)
        for h in range(2):
            kt = kt_ref[2 * p + h, :, cols]
            kt = jnp.concatenate([kt, zpad] if h == 0 else [zpad, kt], axis=0)
            ke, ko = _even_odd(_pack(kt.T))
            kb_ref[dst, h, prow, :] = _pack(jnp.concatenate([ke, ko], axis=0).astype(bf16))

    def v_prep(p, t, dst=None):
        dst = p if dst is None else dst
        cols, _ = _quarter(t)
        for h in range(2):
            vb_ref[dst, h, :, cols] = _pack(vt_ref[2 * p + h, :, cols])

    def s_stage(p):
        slot = p
        for j in range(NJ):
            for h in range(2):
                qh = _unpack(q_ref[64 * j:64 * (j + 1), 128 * h:128 * h + 256])
                st = _dot_nt(_unpack(kb_ref[slot, h]), qh)
                s_ref[2 * j + h] = st
                m_ref[2 * j + h] = jnp.max(st.reshape(W // 8, 8, 128), axis=0)

    def c_stage():
        ls = []
        ps = []
        for u in range(2 * NJ):
            m = jnp.max(m_ref[u], axis=0, keepdims=True)
            pt = jnp.exp2(s_ref[u] - m)
            ls.append(jnp.sum(pt, axis=0, keepdims=True))
            ps.append(jnp.concatenate(
                [_pack2(pt[128 * c:128 * c + 64], pt[128 * c + 64:128 * c + 128])
                 for c in range(W // 128)], axis=0))
        return ls, ps

    def p_stage(p, ls, ps):
        slot = p
        os_ = []
        for j in range(NJ):
            ots = []
            for h in range(2):
                ot = _dot(_unpack(vb_ref[slot, h]), _unpack(ps[2 * j + h]))
                ots.append(ot * (1.0 / ls[2 * j + h]))
            os_.append(jnp.concatenate(ots, axis=0).T)
        o_ref[...] = _pack(jnp.concatenate(os_, axis=0).astype(bf16))

    def o_dot(p):
        return _dot(_unpack(o_ref[...]), wo_ref[_span(p, PW), :])

    def rows_of(b):
        if isinstance(b, int):
            return pl.ds(b * TQ, TQ)
        return pl.ds(pl.multiple_of(b * TQ, TQ), TQ)

    def finish(b, s):
        rows = rows_of(b)
        if isinstance(b, int):
            prow = pl.ds(b * (TQ // 2), TQ // 2)
        else:
            prow = pl.ds(pl.multiple_of(b * (TQ // 2), TQ // 2), TQ // 2)
        g = _unpack(g_ref[prow, :]).astype(f32)
        out_ref[rows, :] = (x_ref[rows, :].astype(f32) + _rb(_rb(s) * g)).astype(bf16)

    for c in x0_copies:
        c.start()
    g0[0].start()
    g0[1].start()
    acc_ref[...] = jnp.zeros(acc_ref.shape, f32)
    neg = jnp.full((GR // 2, 128), -jnp.inf, f32)
    big = jnp.full((GR // 2, 128), float(S), f32)
    for par in range(2):
        top_ref[par, 0] = neg
        top_ref[par, 1] = big
        top_ref[par, 2] = neg
        top_ref[par, 3] = big

    for c in range(4):
        x0_copies[c].wait()
        if c == 0:
            x_copies[1].start()
            g0[2].start()
        layer_norm_rows(c * 128)

    g0[0].wait()
    g0[1].wait()
    x_copies[2].start()
    x_copies[3].start()
    g1[1].start()
    g1[2].start()
    for t in range(4):
        k_prep(0, t)
    q_stage(0, 0)
    for c in range(ROUTER_LEAD):
        gate_router(c)

    x_copies[1].wait()
    g0[2].wait()
    g0[3].start()
    g1[0].start()
    g1[3].start()
    for t in range(4):
        v_prep(0, t)
    layer_norm(1)
    s_stage(0)

    x_copies[2].wait()
    x_copies[3].wait()
    g1[1].wait()
    g1[2].wait()
    for c in g2:
        c.start()
    k_prep(1, 0)
    v_prep(1, 0)
    ls, ps = c_stage()
    q_stage(0, 1)
    p_stage(0, ls, ps)
    s_stage(0)
    layer_norm(2)
    layer_norm(3)
    gate_router(ROUTER_LEAD)
    g0[3].wait()
    g1[0].wait()
    g1[3].wait()

    def prep(j):
        dst = j // NB + 1
        src = jnp.minimum(dst, NP - 1)
        k_prep(src, j % NB, dst)
        v_prep(src, j % NB, dst)

    def step(i):
        nxt = i + 1
        prv = i - 1
        ls, ps = c_stage()
        q_stage(nxt // NB, nxt % NB)
        acc_ref[rows_of(prv % NB), :] += o_dot(prv // NB)
        p_stage(i // NB, ls, ps)
        s_stage(nxt // NB)

    def body(m, carry):
        i = 2 * m + 1
        prep(i)
        prep(i + 1)
        gate_router(i + ROUTER_LEAD)
        gate_router(i + 1 + ROUTER_LEAD)
        step(i)
        step(i + 1)
        return carry

    def segment(sgm, carry):
        @pl.when(sgm == 1)
        def _():
            for c in g2:
                c.wait()
            for c in g3:
                c.start()

        @pl.when(sgm == 2)
        def _():
            for c in g3:
                c.wait()
            for c in moe_copies:
                c.start()

        lo = jnp.where(sgm == 0, 0, jnp.where(sgm == 1, 1, 5))
        hi = jnp.where(sgm == 0, 1, jnp.where(sgm == 1, 5, (NIT - NB + 1 - 1) // 2))
        jax.lax.fori_loop(lo, hi, body, 0)
        return carry

    jax.lax.fori_loop(0, 3, segment, 0)

    vals = jnp.concatenate([top_ref[0, 0], top_ref[1, 0], top_ref[0, 2], top_ref[1, 2]], axis=0)
    idxs = jnp.concatenate([top_ref[0, 1], top_ref[1, 1], top_ref[0, 3], top_ref[1, 3]], axis=0)
    m1 = jnp.max(vals)
    j1 = jnp.min(jnp.where(vals == m1, idxs, float(S)))
    vals2 = jnp.where(idxs == j1, -jnp.inf, vals)
    m2 = jnp.max(vals2)
    j2 = jnp.min(jnp.where(vals2 == m2, idxs, float(S)))
    i1 = jnp.clip(j1.astype(i32), 0, S - 1)
    i2 = jnp.clip(j2.astype(i32), 0, S - 1)

    for c in moe_copies:
        c.wait()
    row16 = jax.lax.broadcasted_iota(i32, (16, D), 0)
    xrows = []
    for idx in (i1, i2):
        e, o = _even_odd(xn_ref[pl.ds(idx // 2, 1), :])
        xrows.append(jnp.where(idx % 2 == 0, e, o))
    xs = jnp.where(row16 == 0, xrows[0], jnp.where(row16 == 1, xrows[1], 0.0)).astype(bf16)
    hg = _rb(_dot(xs, wg_ref[...]))
    hg = _rb(hg * _rb(_sigmoid(hg)))
    hu = _rb(_dot(xs, wu_ref[...]))
    y = _rb(_dot((hg * hu).astype(bf16), wd_ref[...]))
    rs = jnp.where(row16 == 0, m1, m2)
    y = _rb(y * _rb(_sigmoid(rs)))
    for j, idx in enumerate((i1, i2)):
        gin = _rb(xrows[j] + y[j:j + 1, :])
        gbits = pltpu.bitcast(_rb(gin * _rb(_sigmoid(gin))), u32)
        word = pl.ds(idx // 2, 1)
        old = g_ref[word, :]
        g_ref[word, :] = jnp.where(idx % 2 == 0,
                                   (old & jnp.uint32(0xFFFF0000)) | (gbits >> 16),
                                   (old & jnp.uint32(0x0000FFFF)) | gbits)

    def tail_body(b, carry):
        ls, ps = c_stage()
        q_stage(NP - 1, b + 1)
        finish(b - 1, acc_ref[rows_of(b - 1), :] + o_dot(NP - 1))
        p_stage(NP - 1, ls, ps)
        s_stage(NP - 1)
        out_copy(b - 1).start()
        return carry

    jax.lax.fori_loop(1, NB - 1, tail_body, 0)

    ls, ps = c_stage()
    finish(NB - 2, acc_ref[rows_of(NB - 2), :] + o_dot(NP - 1))
    p_stage(NP - 1, ls, ps)
    out_copy(NB - 2).start()

    finish(NB - 1, acc_ref[rows_of(NB - 1), :] + o_dot(NP - 1))
    out_copy(NB - 1).start()
    for b in range(NB):
        out_copy(b).wait()

@jax.jit
def pallas_recurrent_scan__sliding_block_cached__moe_arch_mod__prompt_kernel(
    A_x, A_k_cache, A_v_cache, A_wq, A_wo, B_x, B_w_r, B_w_gate, B_w_up, B_w_down,
):
    kt = jnp.swapaxes(A_k_cache, 2, 3)
    vt = jnp.swapaxes(A_v_cache, 2, 3)
    any_spec = pl.BlockSpec(memory_space=pl.ANY)
    return pl.pallas_call(
        _kernel,
        in_specs=[any_spec, any_spec, any_spec, any_spec, any_spec,
                  pl.BlockSpec(memory_space=pltpu.VMEM),
                  any_spec, any_spec, any_spec],
        out_specs=any_spec,
        out_shape=jax.ShapeDtypeStruct(A_x.shape, A_x.dtype),
        scratch_shapes=[
            pltpu.VMEM((S, D), bf16),
            pltpu.VMEM((S // 2, D), u32),
            pltpu.VMEM((S, D), f32),
            pltpu.VMEM((D, H * DH), bf16),
            pltpu.VMEM((H * DH, D), bf16),
            pltpu.VMEM((H, DH, W), bf16),
            pltpu.VMEM((H, DH, W), bf16),
            pltpu.VMEM((NP + 1, 2, W // 2, KP), u32),
            pltpu.VMEM((NP + 1, 2, DH // 2, W), u32),
            pltpu.VMEM((TQ // 2, PW), u32),
            pltpu.VMEM((TQ // 2, PW), u32),
            pltpu.VMEM((2 * NJ, W, 128), f32),
            pltpu.VMEM((2 * NJ, 8, 128), f32),
            pltpu.VMEM((S // 2, D), u32),
            pltpu.VMEM((2, 4, GR // 2, 128), f32),
            pltpu.VMEM((D, F), bf16),
            pltpu.VMEM((D, F), bf16),
            pltpu.VMEM((F, D), bf16),
            pltpu.VMEM((S, D), bf16),
            pltpu.SemaphoreType.DMA((4 + NB - 1,)),
            pltpu.SemaphoreType.DMA((4,)),
            pltpu.SemaphoreType.DMA((4,)),
            pltpu.SemaphoreType.DMA((4,)),
            pltpu.SemaphoreType.DMA((4,)),
            pltpu.SemaphoreType.DMA((3,)),
            pltpu.SemaphoreType.DMA((NB,)),
        ],
        compiler_params=pltpu.CompilerParams(
            vmem_limit_bytes=128 * 1024 * 1024,
            disable_bounds_checks=True,
        ),
    )(A_x, kt, vt, A_wq, A_wo, B_w_r, B_w_gate, B_w_up, B_w_down)
```

```python
import math

import jax
import jax.numpy as jnp
import jax.experimental.pallas as pl
import jax.experimental.pallas.tpu as pltpu

S, D = 2048, 640
H, DH, W = 32, 192, 512
F = 1536
NP = H // 2
PW = 2 * DH
TQ = 512
NB = S // TQ
NJ = TQ // 128
NIT = NP * NB
KP = 256
GR = S // NIT
ROUTER_LEAD = 4
KEY_MIN = -2 ** 31
NT_DIMS = (((1,), (1,)), ((), ()))
QSCALE = (DH ** -0.5) * math.log2(math.e)
LOG2E = math.log2(math.e)
EPS_BF16 = 1.0013580322265625e-05

bf16 = jnp.bfloat16
f32 = jnp.float32
u32 = jnp.uint32
i32 = jnp.int32


def _rb(t):
    return t.astype(bf16).astype(f32)


def _sigmoid(t):
    return 0.5 * jnp.tanh(0.5 * t) + 0.5


def _recip(t):
    r = pl.reciprocal(t, approx=True)
    return r * (2.0 - t * r)


def _pack(t):
    return pltpu.bitcast(t, u32)


def _unpack(t):
    return pltpu.bitcast(t, bf16)


def _even_odd(u):
    return (pltpu.unpack_elementwise(u, index=0, packed_dtype=bf16, unpacked_dtype=f32),
            pltpu.unpack_elementwise(u, index=1, packed_dtype=bf16, unpacked_dtype=f32))


def _pack2(e, o):
    return pltpu.pack_elementwise([e, o], packed_dtype=bf16)


def _dot(a, b):
    return jnp.dot(a, b, preferred_element_type=f32)


def _dot_nt(a, b):
    return jax.lax.dot_general(a, b, NT_DIMS, preferred_element_type=f32)


def _span(i, n):
    if isinstance(i, int):
        return pl.ds(i * n, n)
    return pl.ds(pl.multiple_of(i * n, n), n)


def _kernel(x_hbm, kt_hbm, vt_hbm, wq_hbm, wo_hbm, wr_ref, wg_hbm, wu_hbm, wd_hbm,
            out_hbm,
            x_ref, xn_ref, acc_ref, wq_ref, wo_ref, kt_ref, vt_ref, kb_ref, vb_ref,
            q_ref, o_ref, s_ref, m_ref, g_ref, top_ref,
            wg_ref, wu_ref, wd_ref, out_ref,
            sem_x, sem_g0, sem_g1, sem_g2, sem_g3, sem_g4, sem_moe, sem_out):
    sk = kt_hbm.shape[-1]

    win = pl.ds(sk - W, W)

    def x_copy(r0, n, sem):
        rows = pl.ds(r0, n)
        return pltpu.make_async_copy(x_hbm.at[0, rows, :], x_ref.at[rows, :], sem)

    def wq_copy(p0, n, sem):
        cols = pl.ds(p0 * PW, n * PW)
        return pltpu.make_async_copy(wq_hbm.at[:, cols], wq_ref.at[:, cols], sem)

    def wo_copy(p0, n, sem):
        rows = pl.ds(p0 * PW, n * PW)
        return pltpu.make_async_copy(wo_hbm.at[rows, :], wo_ref.at[rows, :], sem)

    def kv_copy(src, dst, p0, n, sem):
        heads = pl.ds(2 * p0, 2 * n)
        return pltpu.make_async_copy(src.at[0, heads, :, win], dst.at[heads], sem)

    def group_copies(p0, n, sems):
        return [wq_copy(p0, n, sems.at[0]), kv_copy(kt_hbm, kt_ref, p0, n, sems.at[1]),
                kv_copy(vt_hbm, vt_ref, p0, n, sems.at[2]), wo_copy(p0, n, sems.at[3])]

    x0_copies = [x_copy(c * 128, 128, sem_x.at[c]) for c in range(4)]
    x_copies = [None] + [x_copy(b * TQ, TQ, sem_x.at[3 + b]) for b in range(1, NB)]
    g0 = group_copies(0, 1, sem_g0)
    g1 = group_copies(1, 1, sem_g1)
    g2 = group_copies(2, 1, sem_g2)
    g3 = group_copies(3, 2, sem_g3)
    g4 = group_copies(5, NP - 5, sem_g4)
    moe_copies = [pltpu.make_async_copy(wg_hbm, wg_ref, sem_moe.at[0]),
                  pltpu.make_async_copy(wu_hbm, wu_ref, sem_moe.at[1]),
                  pltpu.make_async_copy(wd_hbm, wd_ref, sem_moe.at[2])]

    def out_copy(b):
        rows = pl.ds(b * TQ, TQ)
        return pltpu.make_async_copy(out_ref.at[rows, :], out_hbm.at[0, rows, :], sem_out.at[b])

    def layer_norm_rows(r0):
        outs = []
        for xf in _even_odd(_pack(x_ref[r0:r0 + 128, :])):
            mean = jnp.sum(xf, axis=-1, keepdims=True) * (1.0 / D)
            xc = xf - mean
            var = jnp.sum(xc * xc, axis=-1, keepdims=True) * (1.0 / D)
            d = _rb(xf - _rb(mean))
            ve = _rb(_rb(var) + EPS_BF16)
            den = _rb(ve * jax.lax.rsqrt(ve))
            outs.append(d * _recip(den))
        xn_ref[r0 // 2:r0 // 2 + 64, :] = _pack2(*outs)

    def layer_norm(b):
        for c in range(TQ // 128):
            layer_norm_rows(b * TQ + c * 128)

    def gate_router(c):
        valid = c < NIT
        c = jnp.minimum(c, NIT - 1)
        prow = _span(c, GR // 2)
        wr = wr_ref[...].astype(f32).reshape(1, D)
        gs = []
        row = jax.lax.broadcasted_iota(i32, (GR // 2, 128), 0)
        for par, xn in enumerate(_even_odd(xn_ref[prow, :])):
            gs.append(xn * _rb(_sigmoid(xn)))
            r = _rb(jnp.sum(xn * wr, axis=-1, keepdims=True)) + 0.0
            bits = pltpu.bitcast(jnp.broadcast_to(r, (GR // 2, 128)), i32)
            key = jnp.where(bits < 0, bits ^ jnp.int32(0x7FFF0000), bits)
            key = key | (0xFFFF - (c * GR + par + 2 * row))
            key = jnp.where(valid, key, KEY_MIN)
            k1 = top_ref[par, 0]
            top_ref[par, 0] = jnp.maximum(k1, key)
            top_ref[par, 1] = jnp.maximum(top_ref[par, 1], jnp.minimum(k1, key))
        g_ref[prow, :] = _pack2(*gs)

    def q_stage(p, b):
        prow = pl.ds(pl.multiple_of(b * (TQ // 2), TQ // 2), TQ // 2)
        q = _dot(_unpack(xn_ref[prow, :]), wq_ref[:, _span(p, PW)])
        q_ref[...] = _pack((q * QSCALE).astype(bf16))

    def _quarter(t):
        if isinstance(t, int):
            return pl.ds(t * 128, 128), pl.ds(t * 64, 64)
        return (pl.ds(pl.multiple_of(t * 128, 128), 128), pl.ds(pl.multiple_of(t * 64, 64), 64))

    def k_prep(p, t, dst=None):
        dst = p if dst is None else dst
        cols, prow = _quarter(t)
        zpad = jnp.zeros((KP - DH, 128), bf16)
        for h in range(2):
            kt = kt_ref[2 * p + h, :, cols]
            kt = jnp.concatenate([kt, zpad] if h == 0 else [zpad, kt], axis=0)
            ke, ko = _even_odd(_pack(kt.T))
            kb_ref[dst, h, prow, :] = _pack(jnp.concatenate([ke, ko], axis=0).astype(bf16))

    def v_prep(p, t, dst=None):
        dst = p if dst is None else dst
        cols, _ = _quarter(t)
        for h in range(2):
            vb_ref[dst, h, :, cols] = _pack(vt_ref[2 * p + h, :, cols])

    def s_stage(p):
        slot = p
        for j in range(NJ):
            for h in range(2):
                qh = _unpack(q_ref[64 * j:64 * (j + 1), 128 * h:128 * h + 256])
                st = _dot_nt(_unpack(kb_ref[slot, h]), qh)
                s_ref[2 * j + h] = st
                m_ref[2 * j + h] = jnp.max(st.reshape(W // 8, 8, 128), axis=0)

    def c_stage():
        ls = []
        ps = []
        for u in range(2 * NJ):
            m = jnp.max(m_ref[u], axis=0, keepdims=True)
            pt = jnp.exp2(s_ref[u] - m)
            ls.append(jnp.sum(pt, axis=0, keepdims=True))
            ps.append(jnp.concatenate(
                [_pack2(pt[128 * c:128 * c + 64], pt[128 * c + 64:128 * c + 128])
                 for c in range(W // 128)], axis=0))
        return ls, ps

    def p_stage(p, ls, ps):
        slot = p
        os_ = []
        for j in range(NJ):
            ots = []
            for h in range(2):
                ot = _dot(_unpack(vb_ref[slot, h]), _unpack(ps[2 * j + h]))
                ots.append(ot * (1.0 / ls[2 * j + h]))
            os_.append(jnp.concatenate(ots, axis=0).T)
        o_ref[...] = _pack(jnp.concatenate(os_, axis=0).astype(bf16))

    def o_dot(p):
        return _dot(_unpack(o_ref[...]), wo_ref[_span(p, PW), :])

    def rows_of(b):
        if isinstance(b, int):
            return pl.ds(b * TQ, TQ)
        return pl.ds(pl.multiple_of(b * TQ, TQ), TQ)

    def finish(b, s):
        rows = rows_of(b)
        if isinstance(b, int):
            prow = pl.ds(b * (TQ // 2), TQ // 2)
        else:
            prow = pl.ds(pl.multiple_of(b * (TQ // 2), TQ // 2), TQ // 2)
        g = _unpack(g_ref[prow, :]).astype(f32)
        out_ref[rows, :] = (x_ref[rows, :].astype(f32) + _rb(_rb(s) * g)).astype(bf16)

    for c in x0_copies:
        c.start()
    g0[0].start()
    g0[1].start()
    for par in range(2):
        for j in range(2):
            top_ref[par, j] = jnp.full((GR // 2, 128), KEY_MIN, i32)

    for c in range(4):
        x0_copies[c].wait()
        if c == 0:
            x_copies[1].start()
            g0[2].start()
        layer_norm_rows(c * 128)

    g0[0].wait()
    g0[1].wait()
    x_copies[2].start()
    x_copies[3].start()
    g1[1].start()
    g1[2].start()
    for t in range(4):
        k_prep(0, t)
    q_stage(0, 0)
    acc_ref[...] = jnp.zeros(acc_ref.shape, f32)
    for c in range(ROUTER_LEAD):
        gate_router(c)

    x_copies[1].wait()
    g0[2].wait()
    for t in range(4):
        v_prep(0, t)
    layer_norm(1)
    s_stage(0)

    x_copies[2].wait()
    x_copies[3].wait()
    g1[1].wait()
    g1[2].wait()
    g0[3].start()
    g1[0].start()
    g1[3].start()
    for c in g2:
        c.start()
    k_prep(1, 0)
    v_prep(1, 0)
    ls, ps = c_stage()
    q_stage(0, 1)
    p_stage(0, ls, ps)
    s_stage(0)
    layer_norm(2)
    layer_norm(3)
    gate_router(ROUTER_LEAD)
    g0[3].wait()
    g1[0].wait()
    g1[3].wait()
    for c in g2:
        c.wait()
    for c in g3:
        c.start()

    def prep(dst, t):
        src = jnp.minimum(dst, NP - 1)
        k_prep(src, t, dst)
        v_prep(src, t, dst)

    def step(p, b):
        pn, bn = (p, b + 1) if b + 1 < NB else (p + 1, 0)
        pp, bp = (p, b - 1) if b > 0 else (p - 1, NB - 1)
        ls, ps = c_stage()
        q_stage(pn, bn)
        acc_ref[rows_of(bp), :] += o_dot(pp)
        p_stage(p, ls, ps)
        s_stage(pn)

    def quad(p, carry):
        @pl.when(p == 1)
        def _():
            for c in g3:
                c.wait()
            for c in g4:
                c.start()

        @pl.when(p == 3)
        def _():
            for c in g4:
                c.wait()
            for c in moe_copies:
                c.start()

        for b in range(1, NB):
            prep(p + 1, b)
        prep(p + 2, 0)
        for b in range(1, NB + 1):
            gate_router(p * NB + b + ROUTER_LEAD)
        for b in range(1, NB):
            step(p, b)
        step(p + 1, 0)
        return carry

    jax.lax.fori_loop(0, NP - 1, quad, 0)

    keys = jnp.concatenate([top_ref[0, 0], top_ref[1, 0], top_ref[0, 1], top_ref[1, 1]], axis=0)
    key1 = jnp.max(keys)
    key2 = jnp.max(jnp.where(keys == key1, KEY_MIN, keys))

    def decode(key):
        idx = jnp.clip(0xFFFF - (key & 0xFFFF), 0, S - 1)
        hi = key & jnp.int32(-65536)
        bits = jnp.where(hi < 0, hi ^ jnp.int32(0x7FFF0000), hi)
        return idx, bits

    i1, b1 = decode(key1)
    i2, b2 = decode(key2)

    for c in moe_copies:
        c.wait()
    row16 = jax.lax.broadcasted_iota(i32, (16, D), 0)
    xrows = []
    for idx in (i1, i2):
        e, o = _even_odd(xn_ref[pl.ds(idx // 2, 1), :])
        xrows.append(jnp.where(idx % 2 == 0, e, o))
    xs = jnp.where(row16 == 0, xrows[0], jnp.where(row16 == 1, xrows[1], 0.0)).astype(bf16)
    hg = _rb(_dot(xs, wg_ref[...]))
    hg = _rb(hg * _rb(_sigmoid(hg)))
    hu = _rb(_dot(xs, wu_ref[...]))
    y = _rb(_dot((hg * hu).astype(bf16), wd_ref[...]))
    rs = pltpu.bitcast(jnp.where(row16 == 0, b1, b2), f32)
    y = _rb(y * _rb(_sigmoid(rs)))
    for j, idx in enumerate((i1, i2)):
        gin = _rb(xrows[j] + y[j:j + 1, :])
        gbits = pltpu.bitcast(_rb(gin * _rb(_sigmoid(gin))), u32)
        word = pl.ds(idx // 2, 1)
        old = g_ref[word, :]
        g_ref[word, :] = jnp.where(idx % 2 == 0,
                                   (old & jnp.uint32(0xFFFF0000)) | (gbits >> 16),
                                   (old & jnp.uint32(0x0000FFFF)) | gbits)

    def tail_body(b, carry):
        ls, ps = c_stage()
        q_stage(NP - 1, b + 1)
        finish(b - 1, acc_ref[rows_of(b - 1), :] + o_dot(NP - 1))
        p_stage(NP - 1, ls, ps)
        s_stage(NP - 1)
        out_copy(b - 1).start()
        return carry

    jax.lax.fori_loop(1, NB - 1, tail_body, 0)

    ls, ps = c_stage()
    finish(NB - 2, acc_ref[rows_of(NB - 2), :] + o_dot(NP - 1))
    p_stage(NP - 1, ls, ps)
    out_copy(NB - 2).start()

    finish(NB - 1, acc_ref[rows_of(NB - 1), :] + o_dot(NP - 1))
    out_copy(NB - 1).start()
    for b in range(NB):
        out_copy(b).wait()

@jax.jit
def pallas_recurrent_scan__sliding_block_cached__moe_arch_mod__prompt_kernel(
    A_x, A_k_cache, A_v_cache, A_wq, A_wo, B_x, B_w_r, B_w_gate, B_w_up, B_w_down,
):
    kt = jnp.swapaxes(A_k_cache, 2, 3)
    vt = jnp.swapaxes(A_v_cache, 2, 3)
    any_spec = pl.BlockSpec(memory_space=pl.ANY)
    return pl.pallas_call(
        _kernel,
        in_specs=[any_spec, any_spec, any_spec, any_spec, any_spec,
                  pl.BlockSpec(memory_space=pltpu.VMEM),
                  any_spec, any_spec, any_spec],
        out_specs=any_spec,
        out_shape=jax.ShapeDtypeStruct(A_x.shape, A_x.dtype),
        scratch_shapes=[
            pltpu.VMEM((S, D), bf16),
            pltpu.VMEM((S // 2, D), u32),
            pltpu.VMEM((S, D), f32),
            pltpu.VMEM((D, H * DH), bf16),
            pltpu.VMEM((H * DH, D), bf16),
            pltpu.VMEM((H, DH, W), bf16),
            pltpu.VMEM((H, DH, W), bf16),
            pltpu.VMEM((NP + 1, 2, W // 2, KP), u32),
            pltpu.VMEM((NP + 1, 2, DH // 2, W), u32),
            pltpu.VMEM((TQ // 2, PW), u32),
            pltpu.VMEM((TQ // 2, PW), u32),
            pltpu.VMEM((2 * NJ, W, 128), f32),
            pltpu.VMEM((2 * NJ, 8, 128), f32),
            pltpu.VMEM((S // 2, D), u32),
            pltpu.VMEM((2, 2, GR // 2, 128), i32),
            pltpu.VMEM((D, F), bf16),
            pltpu.VMEM((D, F), bf16),
            pltpu.VMEM((F, D), bf16),
            pltpu.VMEM((S, D), bf16),
            pltpu.SemaphoreType.DMA((4 + NB - 1,)),
            pltpu.SemaphoreType.DMA((4,)),
            pltpu.SemaphoreType.DMA((4,)),
            pltpu.SemaphoreType.DMA((4,)),
            pltpu.SemaphoreType.DMA((4,)),
            pltpu.SemaphoreType.DMA((4,)),
            pltpu.SemaphoreType.DMA((3,)),
            pltpu.SemaphoreType.DMA((NB,)),
        ],
        compiler_params=pltpu.CompilerParams(
            vmem_limit_bytes=128 * 1024 * 1024,
            disable_bounds_checks=True,
        ),
    )(A_x, kt, vt, A_wq, A_wo, B_w_r, B_w_gate, B_w_up, B_w_down)
```

```python
import math

import jax
import jax.numpy as jnp
import jax.experimental.pallas as pl
import jax.experimental.pallas.tpu as pltpu

S, D = 2048, 640
H, DH, W = 32, 192, 512
F = 1536
NP = H // 2
PW = 2 * DH
TQ = 512
NB = S // TQ
NJ = TQ // 128
NIT = NP * NB
KP = 256
GR = S // NIT
ROUTER_LEAD = 4
KEY_MIN = -2 ** 31
NT_DIMS = (((1,), (1,)), ((), ()))
QSCALE = (DH ** -0.5) * math.log2(math.e)
LOG2E = math.log2(math.e)
EPS_BF16 = 1.0013580322265625e-05

bf16 = jnp.bfloat16
f32 = jnp.float32
u32 = jnp.uint32
i32 = jnp.int32


def _rb(t):
    return t.astype(bf16).astype(f32)


def _sigmoid(t):
    return 0.5 * jnp.tanh(0.5 * t) + 0.5


def _recip(t):
    r = pl.reciprocal(t, approx=True)
    return r * (2.0 - t * r)


def _pack(t):
    return pltpu.bitcast(t, u32)


def _unpack(t):
    return pltpu.bitcast(t, bf16)


def _even_odd(u):
    return (pltpu.unpack_elementwise(u, index=0, packed_dtype=bf16, unpacked_dtype=f32),
            pltpu.unpack_elementwise(u, index=1, packed_dtype=bf16, unpacked_dtype=f32))


def _pack2(e, o):
    return pltpu.pack_elementwise([e, o], packed_dtype=bf16)


def _dot(a, b):
    return jnp.dot(a, b, preferred_element_type=f32)


def _dot_nt(a, b):
    return jax.lax.dot_general(a, b, NT_DIMS, preferred_element_type=f32)


def _span(i, n):
    if isinstance(i, int):
        return pl.ds(i * n, n)
    return pl.ds(pl.multiple_of(i * n, n), n)


def _kernel(x_hbm, kt_hbm, vt_hbm, wq_hbm, wo_hbm, wr_ref, wg_hbm, wu_hbm, wd_hbm,
            out_hbm,
            x_ref, xn_ref, acc_ref, wq_ref, wo_ref, kt_ref, vt_ref, kb_ref, vb_ref,
            q_ref, o_ref, s_ref, m_ref, g_ref, top_ref,
            wg_ref, wu_ref, wd_ref, out_ref,
            sem_x, sem_g0, sem_ga, sem_gb, sem_gc, sem_moe, sem_out):
    sk = kt_hbm.shape[-1]

    win = pl.ds(sk - W, W)

    def x_copy(r0, n, sem):
        rows = pl.ds(r0, n)
        return pltpu.make_async_copy(x_hbm.at[0, rows, :], x_ref.at[rows, :], sem)

    def wq_copy(p0, n, sem):
        cols = pl.ds(p0 * PW, n * PW)
        return pltpu.make_async_copy(wq_hbm.at[:, cols], wq_ref.at[:, cols], sem)

    def wo_copy(p0, n, sem):
        rows = pl.ds(p0 * PW, n * PW)
        return pltpu.make_async_copy(wo_hbm.at[rows, :], wo_ref.at[rows, :], sem)

    def kv_copy(src, dst, p0, n, sem):
        heads = pl.ds(2 * p0, 2 * n)
        return pltpu.make_async_copy(src.at[0, heads, :, win], dst.at[heads], sem)

    def group_copies(p0, n, sems, n_wo=None):
        return [kv_copy(kt_hbm, kt_ref, p0 + 1, n, sems.at[0]),
                kv_copy(vt_hbm, vt_ref, p0 + 1, n, sems.at[1]),
                wq_copy(p0 + 1, n, sems.at[2]),
                wo_copy(p0, n if n_wo is None else n_wo, sems.at[3])]

    x0_copies = [x_copy(c * 128, 128, sem_x.at[c]) for c in range(4)]
    x_copies = [None] + [x_copy(b * TQ, TQ, sem_x.at[3 + b]) for b in range(1, NB)]
    wq0_copy = wq_copy(0, 1, sem_g0.at[0])
    kt0_copy = kv_copy(kt_hbm, kt_ref, 0, 1, sem_g0.at[1])
    vt0_copy = kv_copy(vt_hbm, vt_ref, 0, 1, sem_g0.at[2])
    ga = group_copies(0, 1, sem_ga)
    gb = group_copies(1, 2, sem_gb)
    gc = group_copies(3, NP - 4, sem_gc, n_wo=NP - 3)
    moe_copies = [pltpu.make_async_copy(wg_hbm, wg_ref, sem_moe.at[0]),
                  pltpu.make_async_copy(wu_hbm, wu_ref, sem_moe.at[1]),
                  pltpu.make_async_copy(wd_hbm, wd_ref, sem_moe.at[2])]

    def out_copy(b):
        rows = pl.ds(b * TQ, TQ)
        return pltpu.make_async_copy(out_ref.at[rows, :], out_hbm.at[0, rows, :], sem_out.at[b])

    def layer_norm_rows(r0):
        outs = []
        for xf in _even_odd(_pack(x_ref[r0:r0 + 128, :])):
            mean = jnp.sum(xf, axis=-1, keepdims=True) * (1.0 / D)
            xc = xf - mean
            var = jnp.sum(xc * xc, axis=-1, keepdims=True) * (1.0 / D)
            d = _rb(xf - _rb(mean))
            ve = _rb(_rb(var) + EPS_BF16)
            den = _rb(ve * jax.lax.rsqrt(ve))
            outs.append(d * _recip(den))
        xn_ref[r0 // 2:r0 // 2 + 64, :] = _pack2(*outs)

    def layer_norm(b):
        for c in range(TQ // 128):
            layer_norm_rows(b * TQ + c * 128)

    def gate_router(c):
        valid = c < NIT
        c = jnp.minimum(c, NIT - 1)
        prow = _span(c, GR // 2)
        wr = wr_ref[...].astype(f32).reshape(1, D)
        gs = []
        row = jax.lax.broadcasted_iota(i32, (GR // 2, 128), 0)
        for par, xn in enumerate(_even_odd(xn_ref[prow, :])):
            gs.append(xn * _rb(_sigmoid(xn)))
            r = _rb(jnp.sum(xn * wr, axis=-1, keepdims=True)) + 0.0
            bits = pltpu.bitcast(jnp.broadcast_to(r, (GR // 2, 128)), i32)
            key = jnp.where(bits < 0, bits ^ jnp.int32(0x7FFF0000), bits)
            key = key | (0xFFFF - (c * GR + par + 2 * row))
            key = jnp.where(valid, key, KEY_MIN)
            k1 = top_ref[par, 0]
            top_ref[par, 0] = jnp.maximum(k1, key)
            top_ref[par, 1] = jnp.maximum(top_ref[par, 1], jnp.minimum(k1, key))
        g_ref[prow, :] = _pack2(*gs)

    def q_stage(p, b):
        prow = pl.ds(pl.multiple_of(b * (TQ // 2), TQ // 2), TQ // 2)
        q = _dot(_unpack(xn_ref[prow, :]), wq_ref[:, _span(p, PW)])
        q_ref[...] = _pack((q * QSCALE).astype(bf16))

    def _quarter(t):
        if isinstance(t, int):
            return pl.ds(t * 128, 128), pl.ds(t * 64, 64)
        return (pl.ds(pl.multiple_of(t * 128, 128), 128), pl.ds(pl.multiple_of(t * 64, 64), 64))

    def k_prep(p, t, dst=None):
        dst = p if dst is None else dst
        cols, prow = _quarter(t)
        zpad = jnp.zeros((KP - DH, 128), bf16)
        for h in range(2):
            kt = kt_ref[2 * p + h, :, cols]
            kt = jnp.concatenate([kt, zpad] if h == 0 else [zpad, kt], axis=0)
            ke, ko = _even_odd(_pack(kt.T))
            kb_ref[dst, h, prow, :] = _pack(jnp.concatenate([ke, ko], axis=0).astype(bf16))

    def v_prep(p, t, dst=None):
        dst = p if dst is None else dst
        cols, _ = _quarter(t)
        for h in range(2):
            vb_ref[dst, h, :, cols] = _pack(vt_ref[2 * p + h, :, cols])

    def s_stage(p):
        slot = p
        for j in range(NJ):
            for h in range(2):
                qh = _unpack(q_ref[64 * j:64 * (j + 1), 128 * h:128 * h + 256])
                st = _dot_nt(_unpack(kb_ref[slot, h]), qh)
                s_ref[2 * j + h] = st
                m_ref[2 * j + h] = jnp.max(st.reshape(W // 8, 8, 128), axis=0)

    def c_stage():
        ls = []
        ps = []
        for u in range(2 * NJ):
            m = jnp.max(m_ref[u], axis=0, keepdims=True)
            pt = jnp.exp2(s_ref[u] - m)
            ls.append(jnp.sum(pt, axis=0, keepdims=True))
            ps.append(jnp.concatenate(
                [_pack2(pt[128 * c:128 * c + 64], pt[128 * c + 64:128 * c + 128])
                 for c in range(W // 128)], axis=0))
        return ls, ps

    def p_stage(p, ls, ps):
        slot = p
        os_ = []
        for j in range(NJ):
            ots = []
            for h in range(2):
                ot = _dot(_unpack(vb_ref[slot, h]), _unpack(ps[2 * j + h]))
                ots.append(ot * (1.0 / ls[2 * j + h]))
            os_.append(jnp.concatenate(ots, axis=0).T)
        o_ref[...] = _pack(jnp.concatenate(os_, axis=0).astype(bf16))

    def o_dot(p):
        return _dot(_unpack(o_ref[...]), wo_ref[_span(p, PW), :])

    def rows_of(b):
        if isinstance(b, int):
            return pl.ds(b * TQ, TQ)
        return pl.ds(pl.multiple_of(b * TQ, TQ), TQ)

    def finish(b, s):
        rows = rows_of(b)
        if isinstance(b, int):
            prow = pl.ds(b * (TQ // 2), TQ // 2)
        else:
            prow = pl.ds(pl.multiple_of(b * (TQ // 2), TQ // 2), TQ // 2)
        g = _unpack(g_ref[prow, :]).astype(f32)
        out_ref[rows, :] = (x_ref[rows, :].astype(f32) + _rb(_rb(s) * g)).astype(bf16)

    for c in x0_copies:
        c.start()
    wq0_copy.start()
    kt0_copy.start()
    for par in range(2):
        for j in range(2):
            top_ref[par, j] = jnp.full((GR // 2, 128), KEY_MIN, i32)

    for c in range(4):
        x0_copies[c].wait()
        if c == 2:
            x_copies[1].start()
        layer_norm_rows(c * 128)

    wq0_copy.wait()
    kt0_copy.wait()
    vt0_copy.start()
    x_copies[2].start()
    x_copies[3].start()
    for t in range(4):
        k_prep(0, t)
    q_stage(0, 0)
    for c in range(ROUTER_LEAD):
        gate_router(c)

    x_copies[1].wait()
    layer_norm(1)
    s_stage(0)

    vt0_copy.wait()
    x_copies[2].wait()
    x_copies[3].wait()
    for c in ga:
        c.start()
    for t in range(4):
        v_prep(0, t)
    ls, ps = c_stage()
    q_stage(0, 1)
    p_stage(0, ls, ps)
    s_stage(0)
    layer_norm(2)
    layer_norm(3)
    gate_router(ROUTER_LEAD)
    for c in ga:
        c.wait()
    for c in gb:
        c.start()

    def step(p, b, first):
        pn, bn = (p, b + 1) if b + 1 < NB else (p + 1, 0)
        pp, bp = (p, b - 1) if b > 0 else (p - 1, NB - 1)
        ls, ps = c_stage()
        q_stage(pn, bn)
        rows = rows_of(bp)
        acc_ref[rows, :] = jnp.where(first, 0.0, acc_ref[rows, :]) + o_dot(pp)
        p_stage(p, ls, ps)
        s_stage(pn)

    def quad(p, carry):
        first = p == 0
        for t in range(NB):
            k_prep(p + 1, t)
            v_prep(p + 1, t)
        for b in range(1, NB + 1):
            gate_router(p * NB + b + ROUTER_LEAD)
        for b in range(1, NB):
            step(p, b, first)
        step(p + 1, 0, first)
        return carry

    def segment(sgm, carry):
        @pl.when(sgm == 1)
        def _():
            for c in gb:
                c.wait()
            for c in gc:
                c.start()

        @pl.when(sgm == 2)
        def _():
            for c in gc:
                c.wait()
            for c in moe_copies:
                c.start()

        lo = jnp.where(sgm == 0, 0, jnp.where(sgm == 1, 1, 3))
        hi = jnp.where(sgm == 0, 1, jnp.where(sgm == 1, 3, NP - 1))
        jax.lax.fori_loop(lo, hi, quad, 0)
        return carry

    jax.lax.fori_loop(0, 3, segment, 0)

    keys = jnp.concatenate([top_ref[0, 0], top_ref[1, 0], top_ref[0, 1], top_ref[1, 1]], axis=0)
    top1 = jnp.max(keys, axis=0, keepdims=True)
    top2 = jnp.max(jnp.where(keys == top1, KEY_MIN, keys), axis=0, keepdims=True)
    key1 = top1[0, 0]
    key2 = top2[0, 0]

    def decode(key):
        idx = jnp.clip(0xFFFF - (key & 0xFFFF), 0, S - 1)
        hi = key & jnp.int32(-65536)
        bits = jnp.where(hi < 0, hi ^ jnp.int32(0x7FFF0000), hi)
        return idx, bits

    i1, b1 = decode(key1)
    i2, b2 = decode(key2)

    for c in moe_copies:
        c.wait()
    row16 = jax.lax.broadcasted_iota(i32, (16, D), 0)
    xrows = []
    for idx in (i1, i2):
        e, o = _even_odd(xn_ref[pl.ds(idx // 2, 1), :])
        xrows.append(jnp.where(idx % 2 == 0, e, o))
    xs = jnp.where(row16 == 0, xrows[0], jnp.where(row16 == 1, xrows[1], 0.0)).astype(bf16)
    hg = _rb(_dot(xs, wg_ref[...]))
    hg = _rb(hg * _rb(_sigmoid(hg)))
    hu = _rb(_dot(xs, wu_ref[...]))
    y = _rb(_dot((hg * hu).astype(bf16), wd_ref[...]))
    rs = pltpu.bitcast(jnp.where(row16 == 0, b1, b2), f32)
    y = _rb(y * _rb(_sigmoid(rs)))
    for j, idx in enumerate((i1, i2)):
        gin = _rb(xrows[j] + y[j:j + 1, :])
        gbits = pltpu.bitcast(_rb(gin * _rb(_sigmoid(gin))), u32)
        word = pl.ds(idx // 2, 1)
        old = g_ref[word, :]
        g_ref[word, :] = jnp.where(idx % 2 == 0,
                                   (old & jnp.uint32(0xFFFF0000)) | (gbits >> 16),
                                   (old & jnp.uint32(0x0000FFFF)) | gbits)

    def tail_body(b, carry):
        ls, ps = c_stage()
        q_stage(NP - 1, b + 1)
        finish(b - 1, acc_ref[rows_of(b - 1), :] + o_dot(NP - 1))
        p_stage(NP - 1, ls, ps)
        s_stage(NP - 1)
        out_copy(b - 1).start()
        return carry

    jax.lax.fori_loop(1, NB - 1, tail_body, 0)

    ls, ps = c_stage()
    finish(NB - 2, acc_ref[rows_of(NB - 2), :] + o_dot(NP - 1))
    p_stage(NP - 1, ls, ps)
    out_copy(NB - 2).start()

    finish(NB - 1, acc_ref[rows_of(NB - 1), :] + o_dot(NP - 1))
    out_copy(NB - 1).start()
    for b in range(NB):
        out_copy(b).wait()

@jax.jit
def pallas_recurrent_scan__sliding_block_cached__moe_arch_mod__prompt_kernel(
    A_x, A_k_cache, A_v_cache, A_wq, A_wo, B_x, B_w_r, B_w_gate, B_w_up, B_w_down,
):
    kt = jnp.swapaxes(A_k_cache, 2, 3)
    vt = jnp.swapaxes(A_v_cache, 2, 3)
    any_spec = pl.BlockSpec(memory_space=pl.ANY)
    return pl.pallas_call(
        _kernel,
        in_specs=[any_spec, any_spec, any_spec, any_spec, any_spec,
                  pl.BlockSpec(memory_space=pltpu.VMEM),
                  any_spec, any_spec, any_spec],
        out_specs=any_spec,
        out_shape=jax.ShapeDtypeStruct(A_x.shape, A_x.dtype),
        scratch_shapes=[
            pltpu.VMEM((S, D), bf16),
            pltpu.VMEM((S // 2, D), u32),
            pltpu.VMEM((S, D), f32),
            pltpu.VMEM((D, H * DH), bf16),
            pltpu.VMEM((H * DH, D), bf16),
            pltpu.VMEM((H, DH, W), bf16),
            pltpu.VMEM((H, DH, W), bf16),
            pltpu.VMEM((NP, 2, W // 2, KP), u32),
            pltpu.VMEM((NP, 2, DH // 2, W), u32),
            pltpu.VMEM((TQ // 2, PW), u32),
            pltpu.VMEM((TQ // 2, PW), u32),
            pltpu.VMEM((2 * NJ, W, 128), f32),
            pltpu.VMEM((2 * NJ, 8, 128), f32),
            pltpu.VMEM((S // 2, D), u32),
            pltpu.VMEM((2, 2, GR // 2, 128), i32),
            pltpu.VMEM((D, F), bf16),
            pltpu.VMEM((D, F), bf16),
            pltpu.VMEM((F, D), bf16),
            pltpu.VMEM((S, D), bf16),
            pltpu.SemaphoreType.DMA((4 + NB - 1,)),
            pltpu.SemaphoreType.DMA((3,)),
            pltpu.SemaphoreType.DMA((4,)),
            pltpu.SemaphoreType.DMA((4,)),
            pltpu.SemaphoreType.DMA((4,)),
            pltpu.SemaphoreType.DMA((3,)),
            pltpu.SemaphoreType.DMA((NB,)),
        ],
        compiler_params=pltpu.CompilerParams(
            vmem_limit_bytes=128 * 1024 * 1024,
            disable_bounds_checks=True,
        ),
    )(A_x, kt, vt, A_wq, A_wo, B_w_r, B_w_gate, B_w_up, B_w_down)
```

```python
import math

import jax
import jax.numpy as jnp
import jax.experimental.pallas as pl
import jax.experimental.pallas.tpu as pltpu

S, D = 2048, 640
H, DH, W = 32, 192, 512
F = 1536
NP = H // 2
PW = 2 * DH
TQ = 512
NB = S // TQ
NJ = TQ // 128
NIT = NP * NB
KP = 256
GR = S // NIT
ROUTER_LEAD = 4
KEY_MIN = -2 ** 31
NT_DIMS = (((1,), (1,)), ((), ()))
QSCALE = (DH ** -0.5) * math.log2(math.e)
LOG2E = math.log2(math.e)
EPS_BF16 = 1.0013580322265625e-05

bf16 = jnp.bfloat16
f32 = jnp.float32
u32 = jnp.uint32
i32 = jnp.int32


def _rb(t):
    return t.astype(bf16).astype(f32)


def _sigmoid(t):
    return 0.5 * jnp.tanh(0.5 * t) + 0.5


def _recip(t):
    r = pl.reciprocal(t, approx=True)
    return r * (2.0 - t * r)


def _pack(t):
    return pltpu.bitcast(t, u32)


def _unpack(t):
    return pltpu.bitcast(t, bf16)


def _even_odd(u):
    return (pltpu.unpack_elementwise(u, index=0, packed_dtype=bf16, unpacked_dtype=f32),
            pltpu.unpack_elementwise(u, index=1, packed_dtype=bf16, unpacked_dtype=f32))


def _pack2(e, o):
    return pltpu.pack_elementwise([e, o], packed_dtype=bf16)


def _dot(a, b):
    return jnp.dot(a, b, preferred_element_type=f32)


def _dot_nt(a, b):
    return jax.lax.dot_general(a, b, NT_DIMS, preferred_element_type=f32)


def _span(i, n):
    if isinstance(i, int):
        return pl.ds(i * n, n)
    return pl.ds(pl.multiple_of(i * n, n), n)


def _kernel(x_hbm, kt_hbm, vt_hbm, wq_hbm, wo_hbm, wr_hbm, wg_hbm, wu_hbm, wd_hbm,
            out_hbm,
            x_ref, xn_ref, acc_ref, wq_ref, wo_ref, kt_ref, vt_ref, kb_ref, vb_ref,
            q_ref, o_ref, s_ref, m_ref, g_ref, top_ref,
            wr_ref, wg_ref, wu_ref, wd_ref, out_ref,
            sem_x, sem_g0, sem_ga, sem_gb, sem_gc, sem_moe, sem_out):
    sk = kt_hbm.shape[-1]

    win = pl.ds(sk - W, W)

    def x_copy(r0, n, sem):
        rows = pl.ds(r0, n)
        return pltpu.make_async_copy(x_hbm.at[0, rows, :], x_ref.at[rows, :], sem)

    def wq_copy(p0, n, sem):
        cols = pl.ds(p0 * PW, n * PW)
        return pltpu.make_async_copy(wq_hbm.at[:, cols], wq_ref.at[:, cols], sem)

    def wo_copy(p0, n, sem):
        rows = pl.ds(p0 * PW, n * PW)
        return pltpu.make_async_copy(wo_hbm.at[rows, :], wo_ref.at[rows, :], sem)

    def kv_copy(src, dst, p0, n, sem):
        heads = pl.ds(2 * p0, 2 * n)
        return pltpu.make_async_copy(src.at[0, heads, :, win], dst.at[heads], sem)

    def group_copies(p0, n, sems, n_wo=None):
        return [kv_copy(kt_hbm, kt_ref, p0 + 1, n, sems.at[0]),
                kv_copy(vt_hbm, vt_ref, p0 + 1, n, sems.at[1]),
                wq_copy(p0 + 1, n, sems.at[2]),
                wo_copy(p0, n if n_wo is None else n_wo, sems.at[3])]

    x0_copies = [x_copy(c * 128, 128, sem_x.at[c]) for c in range(4)]
    x_copies = [None] + [x_copy(b * TQ, TQ, sem_x.at[3 + b]) for b in range(1, NB)]
    wq0_copy = wq_copy(0, 1, sem_g0.at[0])
    kt0_copy = kv_copy(kt_hbm, kt_ref, 0, 1, sem_g0.at[1])
    vt0_copy = kv_copy(vt_hbm, vt_ref, 0, 1, sem_g0.at[2])
    wr_copy = pltpu.make_async_copy(wr_hbm, wr_ref, sem_g0.at[3])
    ga = group_copies(0, 1, sem_ga)
    gb = group_copies(1, 2, sem_gb)
    gc = group_copies(3, NP - 4, sem_gc, n_wo=NP - 3)
    moe_copies = [pltpu.make_async_copy(wg_hbm, wg_ref, sem_moe.at[0]),
                  pltpu.make_async_copy(wu_hbm, wu_ref, sem_moe.at[1]),
                  pltpu.make_async_copy(wd_hbm, wd_ref, sem_moe.at[2])]

    def out_copy(b):
        rows = pl.ds(b * TQ, TQ)
        return pltpu.make_async_copy(out_ref.at[rows, :], out_hbm.at[0, rows, :], sem_out.at[b])

    def layer_norm_rows(r0):
        outs = []
        for xf in _even_odd(_pack(x_ref[r0:r0 + 128, :])):
            mean = jnp.sum(xf, axis=-1, keepdims=True) * (1.0 / D)
            xc = xf - mean
            var = jnp.sum(xc * xc, axis=-1, keepdims=True) * (1.0 / D)
            d = _rb(xf - _rb(mean))
            ve = _rb(_rb(var) + EPS_BF16)
            den = _rb(ve * jax.lax.rsqrt(ve))
            outs.append(d * _recip(den))
        xn_ref[r0 // 2:r0 // 2 + 64, :] = _pack2(*outs)

    def layer_norm(b):
        for c in range(TQ // 128):
            layer_norm_rows(b * TQ + c * 128)

    def gate_router(c):
        valid = c < NIT
        c = jnp.minimum(c, NIT - 1)
        prow = _span(c, GR // 2)
        wr = wr_ref[...].astype(f32).reshape(1, D)
        gs = []
        row = jax.lax.broadcasted_iota(i32, (GR // 2, 128), 0)
        for par, xn in enumerate(_even_odd(xn_ref[prow, :])):
            gs.append(xn * _rb(_sigmoid(xn)))
            r = _rb(jnp.sum(xn * wr, axis=-1, keepdims=True)) + 0.0
            bits = pltpu.bitcast(jnp.broadcast_to(r, (GR // 2, 128)), i32)
            key = jnp.where(bits < 0, bits ^ jnp.int32(0x7FFF0000), bits)
            key = key | (0xFFFF - (c * GR + par + 2 * row))
            key = jnp.where(valid, key, KEY_MIN)
            k1 = top_ref[par, 0]
            top_ref[par, 0] = jnp.maximum(k1, key)
            top_ref[par, 1] = jnp.maximum(top_ref[par, 1], jnp.minimum(k1, key))
        g_ref[prow, :] = _pack2(*gs)

    def q_stage(p, b, half=None):
        if half is None:
            src, dst = _span(b, TQ // 2), pl.ds(0, TQ // 2)
        else:
            src, dst = _span(2 * b + half, TQ // 4), _span(half, TQ // 4)
        q = _dot(_unpack(xn_ref[src, :]), wq_ref[:, _span(p, PW)])
        q_ref[dst, :] = _pack((q * QSCALE).astype(bf16))

    def _quarter(t):
        if isinstance(t, int):
            return pl.ds(t * 128, 128), pl.ds(t * 64, 64)
        return (pl.ds(pl.multiple_of(t * 128, 128), 128), pl.ds(pl.multiple_of(t * 64, 64), 64))

    def k_prep(p, t, dst=None):
        dst = p if dst is None else dst
        cols, prow = _quarter(t)
        zpad = jnp.zeros((KP - DH, 128), bf16)
        for h in range(2):
            kt = kt_ref[2 * p + h, :, cols]
            kt = jnp.concatenate([kt, zpad] if h == 0 else [zpad, kt], axis=0)
            ke, ko = _even_odd(_pack(kt.T))
            kb_ref[dst, h, prow, :] = _pack(jnp.concatenate([ke, ko], axis=0).astype(bf16))

    def v_prep(p, t, dst=None):
        dst = p if dst is None else dst
        cols, _ = _quarter(t)
        for h in range(2):
            vb_ref[dst, h, :, cols] = _pack(vt_ref[2 * p + h, :, cols])

    def s_stage(p):
        slot = p
        for j in range(NJ):
            for h in range(2):
                qh = _unpack(q_ref[64 * j:64 * (j + 1), 128 * h:128 * h + 256])
                st = _dot_nt(_unpack(kb_ref[slot, h]), qh)
                s_ref[2 * j + h] = st
                m_ref[2 * j + h] = jnp.max(st.reshape(W // 8, 8, 128), axis=0)

    def c_stage():
        ls = []
        ps = []
        for u in range(2 * NJ):
            m = jnp.max(m_ref[u], axis=0, keepdims=True)
            pt = jnp.exp2(s_ref[u] - m)
            ls.append(jnp.sum(pt, axis=0, keepdims=True))
            ps.append(jnp.concatenate(
                [_pack2(pt[128 * c:128 * c + 64], pt[128 * c + 64:128 * c + 128])
                 for c in range(W // 128)], axis=0))
        return ls, ps

    def p_stage(p, ls, ps):
        slot = p
        os_ = []
        for j in range(NJ):
            ots = []
            for h in range(2):
                ot = _dot(_unpack(vb_ref[slot, h]), _unpack(ps[2 * j + h]))
                ots.append(ot * (1.0 / ls[2 * j + h]))
            os_.append(jnp.concatenate(ots, axis=0).T)
        o_ref[...] = _pack(jnp.concatenate(os_, axis=0).astype(bf16))

    def o_dot(p):
        return _dot(_unpack(o_ref[...]), wo_ref[_span(p, PW), :])

    def rows_of(b):
        if isinstance(b, int):
            return pl.ds(b * TQ, TQ)
        return pl.ds(pl.multiple_of(b * TQ, TQ), TQ)

    def finish(b, s):
        rows = rows_of(b)
        if isinstance(b, int):
            prow = pl.ds(b * (TQ // 2), TQ // 2)
        else:
            prow = pl.ds(pl.multiple_of(b * (TQ // 2), TQ // 2), TQ // 2)
        g = _unpack(g_ref[prow, :]).astype(f32)
        out_ref[rows, :] = (x_ref[rows, :].astype(f32) + _rb(_rb(s) * g)).astype(bf16)

    for c in x0_copies:
        c.start()
    wq0_copy.start()
    for par in range(2):
        for j in range(2):
            top_ref[par, j] = jnp.full((GR // 2, 128), KEY_MIN, i32)

    for c in range(4):
        x0_copies[c].wait()
        if c == 0:
            kt0_copy.start()
        if c == 3:
            x_copies[1].start()
        layer_norm_rows(c * 128)

    wq0_copy.wait()
    q_stage(0, 0, 0)
    kt0_copy.wait()
    wr_copy.start()
    vt0_copy.start()
    x_copies[2].start()
    x_copies[3].start()
    for t in range(4):
        k_prep(0, t)
    q_stage(0, 0, 1)

    x_copies[1].wait()
    layer_norm(1)
    s_stage(0)

    wr_copy.wait()
    vt0_copy.wait()
    x_copies[2].wait()
    x_copies[3].wait()
    for c in ga:
        c.start()
    for t in range(4):
        v_prep(0, t)
    ls, ps = c_stage()
    q_stage(0, 1)
    p_stage(0, ls, ps)
    s_stage(0)
    layer_norm(2)
    layer_norm(3)
    for c in range(ROUTER_LEAD + 1):
        gate_router(c)
    for c in ga:
        c.wait()
    for c in gb:
        c.start()

    def step(p, b, first):
        pn, bn = (p, b + 1) if b + 1 < NB else (p + 1, 0)
        pp, bp = (p, b - 1) if b > 0 else (p - 1, NB - 1)
        ls, ps = c_stage()
        q_stage(pn, bn)
        rows = rows_of(bp)
        acc_ref[rows, :] = jnp.where(first, 0.0, acc_ref[rows, :]) + o_dot(pp)
        p_stage(p, ls, ps)
        s_stage(pn)

    def quad(p, carry):
        first = p == 0
        for t in range(NB):
            k_prep(p + 1, t)
            v_prep(p + 1, t)
        for b in range(1, NB + 1):
            gate_router(p * NB + b + ROUTER_LEAD)
        for b in range(1, NB):
            step(p, b, first)
        step(p + 1, 0, first)
        return carry

    def segment(sgm, carry):
        @pl.when(sgm == 1)
        def _():
            for c in gb:
                c.wait()
            for c in gc:
                c.start()

        @pl.when(sgm == 2)
        def _():
            for c in gc:
                c.wait()
            for c in moe_copies:
                c.start()

        lo = jnp.where(sgm == 0, 0, jnp.where(sgm == 1, 1, 3))
        hi = jnp.where(sgm == 0, 1, jnp.where(sgm == 1, 3, NP - 1))
        jax.lax.fori_loop(lo, hi, quad, 0)
        return carry

    jax.lax.fori_loop(0, 3, segment, 0)

    keys = jnp.concatenate([top_ref[0, 0], top_ref[1, 0], top_ref[0, 1], top_ref[1, 1]], axis=0)
    top1 = jnp.max(keys, axis=0, keepdims=True)
    top2 = jnp.max(jnp.where(keys == top1, KEY_MIN, keys), axis=0, keepdims=True)
    key1 = top1[0, 0]
    key2 = top2[0, 0]

    def decode(key):
        idx = jnp.clip(0xFFFF - (key & 0xFFFF), 0, S - 1)
        hi = key & jnp.int32(-65536)
        bits = jnp.where(hi < 0, hi ^ jnp.int32(0x7FFF0000), hi)
        return idx, bits

    i1, b1 = decode(key1)
    i2, b2 = decode(key2)

    for c in moe_copies:
        c.wait()
    row16 = jax.lax.broadcasted_iota(i32, (16, D), 0)
    xrows = []
    for idx in (i1, i2):
        e, o = _even_odd(xn_ref[pl.ds(idx // 2, 1), :])
        xrows.append(jnp.where(idx % 2 == 0, e, o))
    xs = jnp.where(row16 == 0, xrows[0], jnp.where(row16 == 1, xrows[1], 0.0)).astype(bf16)
    hg = _rb(_dot(xs, wg_ref[...]))
    hg = _rb(hg * _rb(_sigmoid(hg)))
    hu = _rb(_dot(xs, wu_ref[...]))
    y = _rb(_dot((hg * hu).astype(bf16), wd_ref[...]))
    rs = pltpu.bitcast(jnp.where(row16 == 0, b1, b2), f32)
    y = _rb(y * _rb(_sigmoid(rs)))
    for j, idx in enumerate((i1, i2)):
        gin = _rb(xrows[j] + y[j:j + 1, :])
        gbits = pltpu.bitcast(_rb(gin * _rb(_sigmoid(gin))), u32)
        word = pl.ds(idx // 2, 1)
        old = g_ref[word, :]
        g_ref[word, :] = jnp.where(idx % 2 == 0,
                                   (old & jnp.uint32(0xFFFF0000)) | (gbits >> 16),
                                   (old & jnp.uint32(0x0000FFFF)) | gbits)

    for b in range(1, NB):
        ls, ps = c_stage()
        if b + 1 < NB:
            q_stage(NP - 1, b + 1)
        finish(b - 1, acc_ref[rows_of(b - 1), :] + o_dot(NP - 1))
        p_stage(NP - 1, ls, ps)
        if b + 1 < NB:
            s_stage(NP - 1)
        out_copy(b - 1).start()
    finish(NB - 1, acc_ref[rows_of(NB - 1), :] + o_dot(NP - 1))
    out_copy(NB - 1).start()
    for b in range(NB):
        out_copy(b).wait()

@jax.jit
def pallas_recurrent_scan__sliding_block_cached__moe_arch_mod__prompt_kernel(
    A_x, A_k_cache, A_v_cache, A_wq, A_wo, B_x, B_w_r, B_w_gate, B_w_up, B_w_down,
):
    kt = jnp.swapaxes(A_k_cache, 2, 3)
    vt = jnp.swapaxes(A_v_cache, 2, 3)
    any_spec = pl.BlockSpec(memory_space=pl.ANY)
    return pl.pallas_call(
        _kernel,
        in_specs=[any_spec] * 9,
        out_specs=any_spec,
        out_shape=jax.ShapeDtypeStruct(A_x.shape, A_x.dtype),
        scratch_shapes=[
            pltpu.VMEM((S, D), bf16),
            pltpu.VMEM((S // 2, D), u32),
            pltpu.VMEM((S, D), f32),
            pltpu.VMEM((D, H * DH), bf16),
            pltpu.VMEM((H * DH, D), bf16),
            pltpu.VMEM((H, DH, W), bf16),
            pltpu.VMEM((H, DH, W), bf16),
            pltpu.VMEM((NP, 2, W // 2, KP), u32),
            pltpu.VMEM((NP, 2, DH // 2, W), u32),
            pltpu.VMEM((TQ // 2, PW), u32),
            pltpu.VMEM((TQ // 2, PW), u32),
            pltpu.VMEM((2 * NJ, W, 128), f32),
            pltpu.VMEM((2 * NJ, 8, 128), f32),
            pltpu.VMEM((S // 2, D), u32),
            pltpu.VMEM((2, 2, GR // 2, 128), i32),
            pltpu.VMEM((D,), bf16),
            pltpu.VMEM((D, F), bf16),
            pltpu.VMEM((D, F), bf16),
            pltpu.VMEM((F, D), bf16),
            pltpu.VMEM((S, D), bf16),
            pltpu.SemaphoreType.DMA((4 + NB - 1,)),
            pltpu.SemaphoreType.DMA((4,)),
            pltpu.SemaphoreType.DMA((4,)),
            pltpu.SemaphoreType.DMA((4,)),
            pltpu.SemaphoreType.DMA((4,)),
            pltpu.SemaphoreType.DMA((3,)),
            pltpu.SemaphoreType.DMA((NB,)),
        ],
        compiler_params=pltpu.CompilerParams(
            vmem_limit_bytes=128 * 1024 * 1024,
            disable_bounds_checks=True,
        ),
    )(A_x, kt, vt, A_wq, A_wo, B_w_r, B_w_gate, B_w_up, B_w_down)
```

```python
import math

import jax
import jax.numpy as jnp
import jax.experimental.pallas as pl
import jax.experimental.pallas.tpu as pltpu

S, D = 2048, 640
H, DH, W = 32, 192, 512
F = 1536
NP = H // 2
PW = 2 * DH
TQ = 512
NB = S // TQ
NJ = TQ // 128
NIT = NP * NB
KP = 256
GR = S // NIT
ROUTER_LEAD = 4
NLAST = 4
KEY_MIN = -2 ** 31
NT_DIMS = (((1,), (1,)), ((), ()))
QSCALE = (DH ** -0.5) * math.log2(math.e)
LOG2E = math.log2(math.e)
EPS_BF16 = 1.0013580322265625e-05

bf16 = jnp.bfloat16
f32 = jnp.float32
u32 = jnp.uint32
i32 = jnp.int32


def _rb(t):
    return t.astype(bf16).astype(f32)


def _sigmoid(t):
    return 0.5 * jnp.tanh(0.5 * t) + 0.5


def _recip(t):
    r = pl.reciprocal(t, approx=True)
    return r * (2.0 - t * r)


def _pack(t):
    return pltpu.bitcast(t, u32)


def _unpack(t):
    return pltpu.bitcast(t, bf16)


def _even_odd(u):
    return (pltpu.unpack_elementwise(u, index=0, packed_dtype=bf16, unpacked_dtype=f32),
            pltpu.unpack_elementwise(u, index=1, packed_dtype=bf16, unpacked_dtype=f32))


def _pack2(e, o):
    return pltpu.pack_elementwise([e, o], packed_dtype=bf16)


def _dot(a, b):
    return jnp.dot(a, b, preferred_element_type=f32)


def _dot_nt(a, b):
    return jax.lax.dot_general(a, b, NT_DIMS, preferred_element_type=f32)


def _span(i, n):
    if isinstance(i, int):
        return pl.ds(i * n, n)
    return pl.ds(pl.multiple_of(i * n, n), n)


def _kernel(x_hbm, kt_hbm, vt_hbm, wq_hbm, wo_hbm, wr_hbm, wg_hbm, wu_hbm, wd_hbm,
            out_hbm,
            x_ref, xn_ref, acc_ref, wq_ref, wo_ref, kt_ref, vt_ref, kb_ref, vb_ref,
            q_ref, o_ref, s_ref, m_ref, g_ref, top_ref,
            wr_ref, wg_ref, wu_ref, wd_ref, out_ref,
            sem_x, sem_g0, sem_ga, sem_gb, sem_gc, sem_moe, sem_out):
    sk = kt_hbm.shape[-1]

    win = pl.ds(sk - W, W)

    def x_copy(r0, n, sem):
        rows = pl.ds(r0, n)
        return pltpu.make_async_copy(x_hbm.at[0, rows, :], x_ref.at[rows, :], sem)

    def wq_copy(p0, n, sem):
        cols = pl.ds(p0 * PW, n * PW)
        return pltpu.make_async_copy(wq_hbm.at[:, cols], wq_ref.at[:, cols], sem)

    def wo_copy(p0, n, sem):
        rows = pl.ds(p0 * PW, n * PW)
        return pltpu.make_async_copy(wo_hbm.at[rows, :], wo_ref.at[rows, :], sem)

    def kv_copy(src, dst, p0, n, sem):
        heads = pl.ds(2 * p0, 2 * n)
        return pltpu.make_async_copy(src.at[0, heads, :, win], dst.at[heads], sem)

    def group_copies(p0, n, sems, n_wo=None):
        return [kv_copy(kt_hbm, kt_ref, p0 + 1, n, sems.at[0]),
                kv_copy(vt_hbm, vt_ref, p0 + 1, n, sems.at[1]),
                wq_copy(p0 + 1, n, sems.at[2]),
                wo_copy(p0, n if n_wo is None else n_wo, sems.at[3])]

    x0_copies = [x_copy(c * 128, 128, sem_x.at[c]) for c in range(4)]
    x_copies = [None] + [x_copy(b * TQ, TQ, sem_x.at[3 + b]) for b in range(1, NB)]
    wq0_copy = wq_copy(0, 1, sem_g0.at[0])
    kt0_copy = kv_copy(kt_hbm, kt_ref, 0, 1, sem_g0.at[1])
    vt0_copy = kv_copy(vt_hbm, vt_ref, 0, 1, sem_g0.at[2])
    wr_copy = pltpu.make_async_copy(wr_hbm, wr_ref, sem_g0.at[3])
    ga = group_copies(0, 1, sem_ga)
    gb = group_copies(1, 2, sem_gb)
    gc = group_copies(3, NP - 4, sem_gc, n_wo=NP - 3)
    moe_copies = [pltpu.make_async_copy(wg_hbm, wg_ref, sem_moe.at[0]),
                  pltpu.make_async_copy(wu_hbm, wu_ref, sem_moe.at[1]),
                  pltpu.make_async_copy(wd_hbm, wd_ref, sem_moe.at[2])]

    def out_copy(b):
        rows = pl.ds(b * TQ, TQ)
        return pltpu.make_async_copy(out_ref.at[rows, :], out_hbm.at[0, rows, :], sem_out.at[b])

    last_copies = [
        pltpu.make_async_copy(out_ref.at[pl.ds((NB - 1) * TQ + c * (TQ // NLAST), TQ // NLAST), :],
                              out_hbm.at[0, pl.ds((NB - 1) * TQ + c * (TQ // NLAST), TQ // NLAST), :],
                              sem_out.at[NB - 1 + c]) for c in range(NLAST)]

    def layer_norm_rows(r0):
        outs = []
        for xf in _even_odd(_pack(x_ref[r0:r0 + 128, :])):
            mean = jnp.sum(xf, axis=-1, keepdims=True) * (1.0 / D)
            xc = xf - mean
            var = jnp.sum(xc * xc, axis=-1, keepdims=True) * (1.0 / D)
            d = _rb(xf - _rb(mean))
            ve = _rb(_rb(var) + EPS_BF16)
            den = _rb(ve * jax.lax.rsqrt(ve))
            outs.append(d * _recip(den))
        xn_ref[r0 // 2:r0 // 2 + 64, :] = _pack2(*outs)

    def layer_norm(b):
        for c in range(TQ // 128):
            layer_norm_rows(b * TQ + c * 128)

    def gate_router(c):
        valid = c < NIT
        c = jnp.minimum(c, NIT - 1)
        prow = _span(c, GR // 2)
        wr = wr_ref[...].astype(f32).reshape(1, D)
        gs = []
        row = jax.lax.broadcasted_iota(i32, (GR // 2, 128), 0)
        for par, xn in enumerate(_even_odd(xn_ref[prow, :])):
            gs.append(xn * _rb(_sigmoid(xn)))
            r = _rb(jnp.sum(xn * wr, axis=-1, keepdims=True)) + 0.0
            bits = pltpu.bitcast(jnp.broadcast_to(r, (GR // 2, 128)), i32)
            key = jnp.where(bits < 0, bits ^ jnp.int32(0x7FFF0000), bits)
            key = key | (0xFFFF - (c * GR + par + 2 * row))
            key = jnp.where(valid, key, KEY_MIN)
            k1 = top_ref[par, 0]
            top_ref[par, 0] = jnp.maximum(k1, key)
            top_ref[par, 1] = jnp.maximum(top_ref[par, 1], jnp.minimum(k1, key))
        g_ref[prow, :] = _pack2(*gs)

    def q_stage(p, b, half=None):
        if half is None:
            src, dst = _span(b, TQ // 2), pl.ds(0, TQ // 2)
        else:
            src, dst = _span(2 * b + half, TQ // 4), _span(half, TQ // 4)
        q = _dot(_unpack(xn_ref[src, :]), wq_ref[:, _span(p, PW)])
        q_ref[dst, :] = _pack((q * QSCALE).astype(bf16))

    def _quarter(t):
        if isinstance(t, int):
            return pl.ds(t * 128, 128), pl.ds(t * 64, 64)
        return (pl.ds(pl.multiple_of(t * 128, 128), 128), pl.ds(pl.multiple_of(t * 64, 64), 64))

    def k_prep(p, t, dst=None):
        dst = p if dst is None else dst
        cols, prow = _quarter(t)
        zpad = jnp.zeros((KP - DH, 128), bf16)
        for h in range(2):
            kt = kt_ref[2 * p + h, :, cols]
            kt = jnp.concatenate([kt, zpad] if h == 0 else [zpad, kt], axis=0)
            ke, ko = _even_odd(_pack(kt.T))
            kb_ref[dst, h, prow, :] = _pack(jnp.concatenate([ke, ko], axis=0).astype(bf16))

    def v_prep(p, t, dst=None):
        dst = p if dst is None else dst
        cols, _ = _quarter(t)
        for h in range(2):
            vb_ref[dst, h, :, cols] = _pack(vt_ref[2 * p + h, :, cols])

    def s_stage(p):
        slot = p
        for j in range(NJ):
            for h in range(2):
                qh = _unpack(q_ref[64 * j:64 * (j + 1), 128 * h:128 * h + 256])
                st = _dot_nt(_unpack(kb_ref[slot, h]), qh)
                s_ref[2 * j + h] = st
                m_ref[2 * j + h] = jnp.max(st.reshape(W // 8, 8, 128), axis=0)

    def c_stage():
        ls = []
        ps = []
        for u in range(2 * NJ):
            m = jnp.max(m_ref[u], axis=0, keepdims=True)
            pt = jnp.exp2(s_ref[u] - m)
            ls.append(jnp.sum(pt, axis=0, keepdims=True))
            ps.append(jnp.concatenate(
                [_pack2(pt[128 * c:128 * c + 64], pt[128 * c + 64:128 * c + 128])
                 for c in range(W // 128)], axis=0))
        return ls, ps

    def p_stage(p, ls, ps):
        slot = p
        os_ = []
        for j in range(NJ):
            ots = []
            for h in range(2):
                ot = _dot(_unpack(vb_ref[slot, h]), _unpack(ps[2 * j + h]))
                ots.append(ot * (1.0 / ls[2 * j + h]))
            os_.append(jnp.concatenate(ots, axis=0).T)
        o_ref[...] = _pack(jnp.concatenate(os_, axis=0).astype(bf16))

    def o_dot(p):
        return _dot(_unpack(o_ref[...]), wo_ref[_span(p, PW), :])

    def rows_of(b):
        if isinstance(b, int):
            return pl.ds(b * TQ, TQ)
        return pl.ds(pl.multiple_of(b * TQ, TQ), TQ)

    def finish(b, s):
        rows = rows_of(b)
        if isinstance(b, int):
            prow = pl.ds(b * (TQ // 2), TQ // 2)
        else:
            prow = pl.ds(pl.multiple_of(b * (TQ // 2), TQ // 2), TQ // 2)
        g = _unpack(g_ref[prow, :]).astype(f32)
        out_ref[rows, :] = (x_ref[rows, :].astype(f32) + _rb(_rb(s) * g)).astype(bf16)

    for c in x0_copies:
        c.start()
    wq0_copy.start()
    for par in range(2):
        for j in range(2):
            top_ref[par, j] = jnp.full((GR // 2, 128), KEY_MIN, i32)

    for c in range(4):
        x0_copies[c].wait()
        if c == 0:
            kt0_copy.start()
        if c == 3:
            x_copies[1].start()
        layer_norm_rows(c * 128)

    wq0_copy.wait()
    q_stage(0, 0, 0)
    kt0_copy.wait()
    wr_copy.start()
    vt0_copy.start()
    x_copies[2].start()
    x_copies[3].start()
    for t in range(4):
        k_prep(0, t)
    q_stage(0, 0, 1)

    x_copies[1].wait()
    layer_norm(1)
    s_stage(0)

    wr_copy.wait()
    vt0_copy.wait()
    x_copies[2].wait()
    x_copies[3].wait()
    for c in ga:
        c.start()
    for t in range(4):
        v_prep(0, t)
    ls, ps = c_stage()
    q_stage(0, 1)
    p_stage(0, ls, ps)
    s_stage(0)
    layer_norm(2)
    layer_norm(3)
    for c in range(ROUTER_LEAD + 1):
        gate_router(c)
    for c in ga:
        c.wait()
    for c in gb:
        c.start()

    def step(p, b, first):
        pn, bn = (p, b + 1) if b + 1 < NB else (p + 1, 0)
        pp, bp = (p, b - 1) if b > 0 else (p - 1, NB - 1)
        ls, ps = c_stage()
        q_stage(pn, bn)
        rows = rows_of(bp)
        acc_ref[rows, :] = jnp.where(first, 0.0, acc_ref[rows, :]) + o_dot(pp)
        p_stage(p, ls, ps)
        s_stage(pn)

    def quad(p, carry):
        first = p == 0
        for t in range(NB):
            k_prep(p + 1, t)
            v_prep(p + 1, t)
        for b in range(1, NB + 1):
            gate_router(p * NB + b + ROUTER_LEAD)
        for b in range(1, NB):
            step(p, b, first)
        step(p + 1, 0, first)
        return carry

    def segment(sgm, carry):
        @pl.when(sgm == 1)
        def _():
            for c in gb:
                c.wait()
            for c in gc:
                c.start()

        @pl.when(sgm == 2)
        def _():
            for c in gc:
                c.wait()
            for c in moe_copies:
                c.start()

        lo = jnp.where(sgm == 0, 0, jnp.where(sgm == 1, 1, 3))
        hi = jnp.where(sgm == 0, 1, jnp.where(sgm == 1, 3, NP - 1))
        jax.lax.fori_loop(lo, hi, quad, 0)
        return carry

    jax.lax.fori_loop(0, 3, segment, 0)

    keys = jnp.concatenate([top_ref[0, 0], top_ref[1, 0], top_ref[0, 1], top_ref[1, 1]], axis=0)
    top1 = jnp.max(keys, axis=0, keepdims=True)
    top2 = jnp.max(jnp.where(keys == top1, KEY_MIN, keys), axis=0, keepdims=True)
    key1 = top1[0, 0]
    key2 = top2[0, 0]

    def decode(key):
        idx = jnp.clip(0xFFFF - (key & 0xFFFF), 0, S - 1)
        hi = key & jnp.int32(-65536)
        bits = jnp.where(hi < 0, hi ^ jnp.int32(0x7FFF0000), hi)
        return idx, bits

    i1, b1 = decode(key1)
    i2, b2 = decode(key2)

    for c in moe_copies:
        c.wait()
    row16 = jax.lax.broadcasted_iota(i32, (16, D), 0)
    xrows = []
    for idx in (i1, i2):
        e, o = _even_odd(xn_ref[pl.ds(idx // 2, 1), :])
        xrows.append(jnp.where(idx % 2 == 0, e, o))
    xs = jnp.where(row16 == 0, xrows[0], jnp.where(row16 == 1, xrows[1], 0.0)).astype(bf16)
    hg = _rb(_dot(xs, wg_ref[...]))
    hg = _rb(hg * _rb(_sigmoid(hg)))
    hu = _rb(_dot(xs, wu_ref[...]))
    y = _rb(_dot((hg * hu).astype(bf16), wd_ref[...]))
    rs = pltpu.bitcast(jnp.where(row16 == 0, b1, b2), f32)
    y = _rb(y * _rb(_sigmoid(rs)))
    for j, idx in enumerate((i1, i2)):
        gin = _rb(xrows[j] + y[j:j + 1, :])
        gbits = pltpu.bitcast(_rb(gin * _rb(_sigmoid(gin))), u32)
        word = pl.ds(idx // 2, 1)
        old = g_ref[word, :]
        g_ref[word, :] = jnp.where(idx % 2 == 0,
                                   (old & jnp.uint32(0xFFFF0000)) | (gbits >> 16),
                                   (old & jnp.uint32(0x0000FFFF)) | gbits)

    for b in range(1, NB):
        ls, ps = c_stage()
        if b + 1 < NB:
            q_stage(NP - 1, b + 1)
        finish(b - 1, acc_ref[rows_of(b - 1), :] + o_dot(NP - 1))
        p_stage(NP - 1, ls, ps)
        if b + 1 < NB:
            s_stage(NP - 1)
        out_copy(b - 1).start()
    for c in range(NLAST):
        n = TQ // NLAST
        r0 = (NB - 1) * TQ + c * n
        o = _unpack(o_ref[c * n // 2:(c + 1) * n // 2, :])
        sacc = acc_ref[r0:r0 + n, :] + _dot(o, wo_ref[_span(NP - 1, PW), :])
        g = _unpack(g_ref[r0 // 2:(r0 + n) // 2, :]).astype(f32)
        out_ref[r0:r0 + n, :] = (x_ref[r0:r0 + n, :].astype(f32) + _rb(_rb(sacc) * g)).astype(bf16)
        last_copies[c].start()
    for b in range(NB - 1):
        out_copy(b).wait()
    for c in last_copies:
        c.wait()

@jax.jit
def pallas_recurrent_scan__sliding_block_cached__moe_arch_mod__prompt_kernel(
    A_x, A_k_cache, A_v_cache, A_wq, A_wo, B_x, B_w_r, B_w_gate, B_w_up, B_w_down,
):
    kt = jnp.swapaxes(A_k_cache, 2, 3)
    vt = jnp.swapaxes(A_v_cache, 2, 3)
    any_spec = pl.BlockSpec(memory_space=pl.ANY)
    return pl.pallas_call(
        _kernel,
        in_specs=[any_spec] * 9,
        out_specs=any_spec,
        out_shape=jax.ShapeDtypeStruct(A_x.shape, A_x.dtype),
        scratch_shapes=[
            pltpu.VMEM((S, D), bf16),
            pltpu.VMEM((S // 2, D), u32),
            pltpu.VMEM((S, D), f32),
            pltpu.VMEM((D, H * DH), bf16),
            pltpu.VMEM((H * DH, D), bf16),
            pltpu.VMEM((H, DH, W), bf16),
            pltpu.VMEM((H, DH, W), bf16),
            pltpu.VMEM((NP, 2, W // 2, KP), u32),
            pltpu.VMEM((NP, 2, DH // 2, W), u32),
            pltpu.VMEM((TQ // 2, PW), u32),
            pltpu.VMEM((TQ // 2, PW), u32),
            pltpu.VMEM((2 * NJ, W, 128), f32),
            pltpu.VMEM((2 * NJ, 8, 128), f32),
            pltpu.VMEM((S // 2, D), u32),
            pltpu.VMEM((2, 2, GR // 2, 128), i32),
            pltpu.VMEM((D,), bf16),
            pltpu.VMEM((D, F), bf16),
            pltpu.VMEM((D, F), bf16),
            pltpu.VMEM((F, D), bf16),
            pltpu.VMEM((S, D), bf16),
            pltpu.SemaphoreType.DMA((4 + NB - 1,)),
            pltpu.SemaphoreType.DMA((4,)),
            pltpu.SemaphoreType.DMA((4,)),
            pltpu.SemaphoreType.DMA((4,)),
            pltpu.SemaphoreType.DMA((4,)),
            pltpu.SemaphoreType.DMA((3,)),
            pltpu.SemaphoreType.DMA((NB - 1 + NLAST,)),
        ],
        compiler_params=pltpu.CompilerParams(
            vmem_limit_bytes=128 * 1024 * 1024,
            disable_bounds_checks=True,
        ),
    )(A_x, kt, vt, A_wq, A_wo, B_w_r, B_w_gate, B_w_up, B_w_down)
```

```python
import math

import jax
import jax.numpy as jnp
import jax.experimental.pallas as pl
import jax.experimental.pallas.tpu as pltpu

S, D = 2048, 640
H, DH, W = 32, 192, 512
F = 1536
NP = H // 2
PW = 2 * DH
TQ = 512
NB = S // TQ
NJ = TQ // 128
NIT = NP * NB
KP = 256
GR = S // NIT
ROUTER_LEAD = 4
NLAST = 4
KEY_MIN = -2 ** 31
NT_DIMS = (((1,), (1,)), ((), ()))
QSCALE = (DH ** -0.5) * math.log2(math.e)
LOG2E = math.log2(math.e)
EPS_BF16 = 1.0013580322265625e-05

bf16 = jnp.bfloat16
f32 = jnp.float32
u32 = jnp.uint32
i32 = jnp.int32


def _rb(t):
    return t.astype(bf16).astype(f32)


def _sigmoid(t):
    return 0.5 * jnp.tanh(0.5 * t) + 0.5


def _recip(t):
    r = pl.reciprocal(t, approx=True)
    return r * (2.0 - t * r)


def _pack(t):
    return pltpu.bitcast(t, u32)


def _unpack(t):
    return pltpu.bitcast(t, bf16)


def _even_odd(u):
    return (pltpu.unpack_elementwise(u, index=0, packed_dtype=bf16, unpacked_dtype=f32),
            pltpu.unpack_elementwise(u, index=1, packed_dtype=bf16, unpacked_dtype=f32))


def _pack2(e, o):
    return pltpu.pack_elementwise([e, o], packed_dtype=bf16)


def _dot(a, b):
    return jnp.dot(a, b, preferred_element_type=f32)


def _dot_nt(a, b):
    return jax.lax.dot_general(a, b, NT_DIMS, preferred_element_type=f32)


def _span(i, n):
    if isinstance(i, int):
        return pl.ds(i * n, n)
    return pl.ds(pl.multiple_of(i * n, n), n)


def _kernel(x_hbm, kt_hbm, vt_hbm, wq_hbm, wo_hbm, wr_hbm, wg_hbm, wu_hbm, wd_hbm,
            out_hbm,
            x_ref, xn_ref, acc_ref, wq_ref, wo_ref, kt_ref, vt_ref, kb_ref, vb_ref,
            q_ref, o_ref, s_ref, m_ref, g_ref, top_ref,
            wr_ref, wg_ref, wu_ref, wd_ref, out_ref,
            sem_x, sem_g0, sem_ga, sem_gb, sem_gc, sem_moe, sem_out):
    sk = kt_hbm.shape[-1]

    win = pl.ds(sk - W, W)

    def x_copy(r0, n, sem):
        rows = pl.ds(r0, n)
        return pltpu.make_async_copy(x_hbm.at[0, rows, :], x_ref.at[rows, :], sem)

    def wq_copy(p0, n, sem):
        cols = pl.ds(p0 * PW, n * PW)
        return pltpu.make_async_copy(wq_hbm.at[:, cols], wq_ref.at[:, cols], sem)

    def wo_copy(p0, n, sem):
        rows = pl.ds(p0 * PW, n * PW)
        return pltpu.make_async_copy(wo_hbm.at[rows, :], wo_ref.at[rows, :], sem)

    def kv_copy(src, dst, p0, n, sem):
        heads = pl.ds(2 * p0, 2 * n)
        return pltpu.make_async_copy(src.at[0, heads, :, win], dst.at[heads], sem)

    def group_copies(p0, n, sems, n_wo=None):
        return [kv_copy(kt_hbm, kt_ref, p0 + 1, n, sems.at[0]),
                kv_copy(vt_hbm, vt_ref, p0 + 1, n, sems.at[1]),
                wq_copy(p0 + 1, n, sems.at[2]),
                wo_copy(p0, n if n_wo is None else n_wo, sems.at[3])]

    x0_copies = [x_copy(c * 128, 128, sem_x.at[c]) for c in range(4)]
    x_copies = [None] + [x_copy(b * TQ, TQ, sem_x.at[3 + b]) for b in range(1, NB)]
    wq0_copy = wq_copy(0, 1, sem_g0.at[0])
    kt0_copy = kv_copy(kt_hbm, kt_ref, 0, 1, sem_g0.at[1])
    vt0_copy = kv_copy(vt_hbm, vt_ref, 0, 1, sem_g0.at[2])
    wr_copy = pltpu.make_async_copy(wr_hbm, wr_ref, sem_g0.at[3])
    ga = group_copies(0, 1, sem_ga)
    gb = group_copies(1, 2, sem_gb)
    gc = group_copies(3, NP - 4, sem_gc, n_wo=NP - 3)
    moe_copies = [pltpu.make_async_copy(wg_hbm, wg_ref, sem_moe.at[0]),
                  pltpu.make_async_copy(wu_hbm, wu_ref, sem_moe.at[1]),
                  pltpu.make_async_copy(wd_hbm, wd_ref, sem_moe.at[2])]

    def out_copy(b):
        rows = pl.ds(b * TQ, TQ)
        return pltpu.make_async_copy(out_ref.at[rows, :], out_hbm.at[0, rows, :], sem_out.at[b])

    last_copies = [
        pltpu.make_async_copy(out_ref.at[pl.ds((NB - 1) * TQ + c * (TQ // NLAST), TQ // NLAST), :],
                              out_hbm.at[0, pl.ds((NB - 1) * TQ + c * (TQ // NLAST), TQ // NLAST), :],
                              sem_out.at[NB - 1 + c]) for c in range(NLAST)]

    def layer_norm_rows(r0):
        outs = []
        for xf in _even_odd(_pack(x_ref[r0:r0 + 128, :])):
            mean = jnp.sum(xf, axis=-1, keepdims=True) * (1.0 / D)
            xc = xf - mean
            var = jnp.sum(xc * xc, axis=-1, keepdims=True) * (1.0 / D)
            d = _rb(xf - _rb(mean))
            ve = _rb(_rb(var) + EPS_BF16)
            den = _rb(ve * jax.lax.rsqrt(ve))
            outs.append(d * _recip(den))
        xn_ref[r0 // 2:r0 // 2 + 64, :] = _pack2(*outs)

    def layer_norm(b):
        for c in range(TQ // 128):
            layer_norm_rows(b * TQ + c * 128)

    def gate_router(c):
        valid = c < NIT
        c = jnp.minimum(c, NIT - 1)
        prow = _span(c, GR // 2)
        wr = wr_ref[...].astype(f32).reshape(1, D)
        gs = []
        row = jax.lax.broadcasted_iota(i32, (GR // 2, 128), 0)
        for par, xn in enumerate(_even_odd(xn_ref[prow, :])):
            gs.append(xn * _rb(_sigmoid(xn)))
            r = _rb(jnp.sum(xn * wr, axis=-1, keepdims=True)) + 0.0
            bits = pltpu.bitcast(jnp.broadcast_to(r, (GR // 2, 128)), i32)
            key = jnp.where(bits < 0, bits ^ jnp.int32(0x7FFF0000), bits)
            key = key | (0xFFFF - (c * GR + par + 2 * row))
            key = jnp.where(valid, key, KEY_MIN)
            k1 = top_ref[par, 0]
            top_ref[par, 0] = jnp.maximum(k1, key)
            top_ref[par, 1] = jnp.maximum(top_ref[par, 1], jnp.minimum(k1, key))
        g_ref[prow, :] = _pack2(*gs)

    def q_stage(p, b, half=None):
        if half is None:
            src, dst = _span(b, TQ // 2), pl.ds(0, TQ // 2)
        else:
            src, dst = _span(2 * b + half, TQ // 4), _span(half, TQ // 4)
        q = _dot(_unpack(xn_ref[src, :]), wq_ref[:, _span(p, PW)])
        q_ref[dst, :] = _pack((q * QSCALE).astype(bf16))

    def _quarter(t):
        if isinstance(t, int):
            return pl.ds(t * 128, 128), pl.ds(t * 64, 64)
        return (pl.ds(pl.multiple_of(t * 128, 128), 128), pl.ds(pl.multiple_of(t * 64, 64), 64))

    def k_prep(p, t, dst=None):
        dst = p if dst is None else dst
        cols, prow = _quarter(t)
        zpad = jnp.zeros((KP - DH, 128), bf16)
        for h in range(2):
            kt = kt_ref[2 * p + h, :, cols]
            kt = jnp.concatenate([kt, zpad] if h == 0 else [zpad, kt], axis=0)
            ke, ko = _even_odd(_pack(kt.T))
            kb_ref[dst % 2, h, prow, :] = _pack(jnp.concatenate([ke, ko], axis=0).astype(bf16))

    def v_prep(p, t, dst=None):
        dst = p if dst is None else dst
        cols, _ = _quarter(t)
        for h in range(2):
            vb_ref[dst % 2, h, :, cols] = _pack(vt_ref[2 * p + h, :, cols])

    def s_stage(p):
        slot = p % 2
        for j in range(NJ):
            for h in range(2):
                qh = _unpack(q_ref[64 * j:64 * (j + 1), 128 * h:128 * h + 256])
                st = _dot_nt(_unpack(kb_ref[slot, h]), qh)
                s_ref[2 * j + h] = st
                m_ref[2 * j + h] = jnp.max(st.reshape(W // 8, 8, 128), axis=0)

    def c_stage():
        ls = []
        ps = []
        for u in range(2 * NJ):
            m = jnp.max(m_ref[u], axis=0, keepdims=True)
            pt = jnp.exp2(s_ref[u] - m)
            ls.append(jnp.sum(pt, axis=0, keepdims=True))
            ps.append(jnp.concatenate(
                [_pack2(pt[128 * c:128 * c + 64], pt[128 * c + 64:128 * c + 128])
                 for c in range(W // 128)], axis=0))
        return ls, ps

    def p_stage(p, ls, ps):
        slot = p % 2
        os_ = []
        for j in range(NJ):
            ots = []
            for h in range(2):
                ot = _dot(_unpack(vb_ref[slot, h]), _unpack(ps[2 * j + h]))
                ots.append(ot * (1.0 / ls[2 * j + h]))
            os_.append(jnp.concatenate(ots, axis=0).T)
        o_ref[...] = _pack(jnp.concatenate(os_, axis=0).astype(bf16))

    def o_dot(p):
        return _dot(_unpack(o_ref[...]), wo_ref[_span(p, PW), :])

    def rows_of(b):
        if isinstance(b, int):
            return pl.ds(b * TQ, TQ)
        return pl.ds(pl.multiple_of(b * TQ, TQ), TQ)

    def finish(b, s):
        rows = rows_of(b)
        if isinstance(b, int):
            prow = pl.ds(b * (TQ // 2), TQ // 2)
        else:
            prow = pl.ds(pl.multiple_of(b * (TQ // 2), TQ // 2), TQ // 2)
        g = _unpack(g_ref[prow, :]).astype(f32)
        out_ref[rows, :] = (x_ref[rows, :].astype(f32) + _rb(_rb(s) * g)).astype(bf16)

    for c in x0_copies:
        c.start()
    wq0_copy.start()
    for par in range(2):
        for j in range(2):
            top_ref[par, j] = jnp.full((GR // 2, 128), KEY_MIN, i32)

    for c in range(4):
        x0_copies[c].wait()
        if c == 0:
            kt0_copy.start()
        if c == 3:
            x_copies[1].start()
        layer_norm_rows(c * 128)

    wq0_copy.wait()
    q_stage(0, 0, 0)
    kt0_copy.wait()
    wr_copy.start()
    vt0_copy.start()
    x_copies[2].start()
    x_copies[3].start()
    for t in range(4):
        k_prep(0, t)
    q_stage(0, 0, 1)

    x_copies[1].wait()
    layer_norm(1)
    s_stage(0)

    wr_copy.wait()
    vt0_copy.wait()
    x_copies[2].wait()
    x_copies[3].wait()
    for c in ga:
        c.start()
    for t in range(4):
        v_prep(0, t)
    ls, ps = c_stage()
    q_stage(0, 1)
    p_stage(0, ls, ps)
    s_stage(0)
    layer_norm(2)
    layer_norm(3)
    for c in range(ROUTER_LEAD + 1):
        gate_router(c)
    for c in ga:
        c.wait()
    for c in gb:
        c.start()

    def step(p, b, first):
        pn, bn = (p, b + 1) if b + 1 < NB else (p + 1, 0)
        pp, bp = (p, b - 1) if b > 0 else (p - 1, NB - 1)
        ls, ps = c_stage()
        q_stage(pn, bn)
        rows = rows_of(bp)
        acc_ref[rows, :] = jnp.where(first, 0.0, acc_ref[rows, :]) + o_dot(pp)
        p_stage(p, ls, ps)
        s_stage(pn)

    def quad(p, carry):
        first = p == 0
        for t in range(NB):
            k_prep(p + 1, t)
            v_prep(p + 1, t)
        for b in range(1, NB + 1):
            gate_router(p * NB + b + ROUTER_LEAD)
        for b in range(1, NB):
            step(p, b, first)
        step(p + 1, 0, first)
        return carry

    def segment(sgm, carry):
        @pl.when(sgm == 1)
        def _():
            for c in gb:
                c.wait()
            for c in gc:
                c.start()

        @pl.when(sgm == 2)
        def _():
            for c in gc:
                c.wait()
            for c in moe_copies:
                c.start()

        lo = jnp.where(sgm == 0, 0, jnp.where(sgm == 1, 1, 3))
        hi = jnp.where(sgm == 0, 1, jnp.where(sgm == 1, 3, NP - 1))
        jax.lax.fori_loop(lo, hi, quad, 0)
        return carry

    jax.lax.fori_loop(0, 3, segment, 0)

    keys = jnp.concatenate([top_ref[0, 0], top_ref[1, 0], top_ref[0, 1], top_ref[1, 1]], axis=0)
    top1 = jnp.max(keys, axis=0, keepdims=True)
    top2 = jnp.max(jnp.where(keys == top1, KEY_MIN, keys), axis=0, keepdims=True)
    key1 = top1[0, 0]
    key2 = top2[0, 0]

    def decode(key):
        idx = jnp.clip(0xFFFF - (key & 0xFFFF), 0, S - 1)
        hi = key & jnp.int32(-65536)
        bits = jnp.where(hi < 0, hi ^ jnp.int32(0x7FFF0000), hi)
        return idx, bits

    i1, b1 = decode(key1)
    i2, b2 = decode(key2)

    for c in moe_copies:
        c.wait()
    row16 = jax.lax.broadcasted_iota(i32, (16, D), 0)
    xrows = []
    for idx in (i1, i2):
        e, o = _even_odd(xn_ref[pl.ds(idx // 2, 1), :])
        xrows.append(jnp.where(idx % 2 == 0, e, o))
    xs = jnp.where(row16 == 0, xrows[0], jnp.where(row16 == 1, xrows[1], 0.0)).astype(bf16)
    hg = _rb(_dot(xs, wg_ref[...]))
    hg = _rb(hg * _rb(_sigmoid(hg)))
    hu = _rb(_dot(xs, wu_ref[...]))
    y = _rb(_dot((hg * hu).astype(bf16), wd_ref[...]))
    rs = pltpu.bitcast(jnp.where(row16 == 0, b1, b2), f32)
    y = _rb(y * _rb(_sigmoid(rs)))
    for j, idx in enumerate((i1, i2)):
        gin = _rb(xrows[j] + y[j:j + 1, :])
        gbits = pltpu.bitcast(_rb(gin * _rb(_sigmoid(gin))), u32)
        word = pl.ds(idx // 2, 1)
        old = g_ref[word, :]
        g_ref[word, :] = jnp.where(idx % 2 == 0,
                                   (old & jnp.uint32(0xFFFF0000)) | (gbits >> 16),
                                   (old & jnp.uint32(0x0000FFFF)) | gbits)

    for b in range(1, NB):
        ls, ps = c_stage()
        if b + 1 < NB:
            q_stage(NP - 1, b + 1)
        finish(b - 1, acc_ref[rows_of(b - 1), :] + o_dot(NP - 1))
        p_stage(NP - 1, ls, ps)
        if b + 1 < NB:
            s_stage(NP - 1)
        out_copy(b - 1).start()
    for c in range(NLAST):
        n = TQ // NLAST
        r0 = (NB - 1) * TQ + c * n
        o = _unpack(o_ref[c * n // 2:(c + 1) * n // 2, :])
        sacc = acc_ref[r0:r0 + n, :] + _dot(o, wo_ref[_span(NP - 1, PW), :])
        g = _unpack(g_ref[r0 // 2:(r0 + n) // 2, :]).astype(f32)
        out_ref[r0:r0 + n, :] = (x_ref[r0:r0 + n, :].astype(f32) + _rb(_rb(sacc) * g)).astype(bf16)
        last_copies[c].start()
    for b in range(NB - 1):
        out_copy(b).wait()
    for c in last_copies:
        c.wait()

@jax.jit
def pallas_recurrent_scan__sliding_block_cached__moe_arch_mod__prompt_kernel(
    A_x, A_k_cache, A_v_cache, A_wq, A_wo, B_x, B_w_r, B_w_gate, B_w_up, B_w_down,
):
    kt = jnp.swapaxes(A_k_cache, 2, 3)
    vt = jnp.swapaxes(A_v_cache, 2, 3)
    any_spec = pl.BlockSpec(memory_space=pl.ANY)
    return pl.pallas_call(
        _kernel,
        in_specs=[any_spec] * 9,
        out_specs=any_spec,
        out_shape=jax.ShapeDtypeStruct(A_x.shape, A_x.dtype),
        scratch_shapes=[
            pltpu.VMEM((S, D), bf16),
            pltpu.VMEM((S // 2, D), u32),
            pltpu.VMEM((S, D), f32),
            pltpu.VMEM((D, H * DH), bf16),
            pltpu.VMEM((H * DH, D), bf16),
            pltpu.VMEM((H, DH, W), bf16),
            pltpu.VMEM((H, DH, W), bf16),
            pltpu.VMEM((2, 2, W // 2, KP), u32),
            pltpu.VMEM((2, 2, DH // 2, W), u32),
            pltpu.VMEM((TQ // 2, PW), u32),
            pltpu.VMEM((TQ // 2, PW), u32),
            pltpu.VMEM((2 * NJ, W, 128), f32),
            pltpu.VMEM((2 * NJ, 8, 128), f32),
            pltpu.VMEM((S // 2, D), u32),
            pltpu.VMEM((2, 2, GR // 2, 128), i32),
            pltpu.VMEM((D,), bf16),
            pltpu.VMEM((D, F), bf16),
            pltpu.VMEM((D, F), bf16),
            pltpu.VMEM((F, D), bf16),
            pltpu.VMEM((S, D), bf16),
            pltpu.SemaphoreType.DMA((4 + NB - 1,)),
            pltpu.SemaphoreType.DMA((4,)),
            pltpu.SemaphoreType.DMA((4,)),
            pltpu.SemaphoreType.DMA((4,)),
            pltpu.SemaphoreType.DMA((4,)),
            pltpu.SemaphoreType.DMA((3,)),
            pltpu.SemaphoreType.DMA((NB - 1 + NLAST,)),
        ],
        compiler_params=pltpu.CompilerParams(
            vmem_limit_bytes=128 * 1024 * 1024,
            disable_bounds_checks=True,
        ),
    )(A_x, kt, vt, A_wq, A_wo, B_w_r, B_w_gate, B_w_up, B_w_down)
```

```python
import math

import jax
import jax.numpy as jnp
import jax.experimental.pallas as pl
import jax.experimental.pallas.tpu as pltpu

S, D = 2048, 640
H, DH, W = 32, 192, 512
F = 1536
NP = H // 2
PW = 2 * DH
TQ = 512
NB = S // TQ
NJ = TQ // 128
NIT = NP * NB
KP = 256
GR = S // NIT
ROUTER_LEAD = 4
NLAST = 4
KEY_MIN = -2 ** 31
NT_DIMS = (((1,), (1,)), ((), ()))
QSCALE = (DH ** -0.5) * math.log2(math.e)
LOG2E = math.log2(math.e)
EPS_BF16 = 1.0013580322265625e-05

bf16 = jnp.bfloat16
f32 = jnp.float32
u32 = jnp.uint32
i32 = jnp.int32


def _rb(t):
    return t.astype(bf16).astype(f32)


def _sigmoid(t):
    return 0.5 * jnp.tanh(0.5 * t) + 0.5


def _recip(t):
    r = pl.reciprocal(t, approx=True)
    return r * (2.0 - t * r)


def _pack(t):
    return pltpu.bitcast(t, u32)


def _unpack(t):
    return pltpu.bitcast(t, bf16)


def _even_odd(u):
    return (pltpu.unpack_elementwise(u, index=0, packed_dtype=bf16, unpacked_dtype=f32),
            pltpu.unpack_elementwise(u, index=1, packed_dtype=bf16, unpacked_dtype=f32))


def _pack2(e, o):
    return pltpu.pack_elementwise([e, o], packed_dtype=bf16)


def _dot(a, b):
    return jnp.dot(a, b, preferred_element_type=f32)


def _dot_nt(a, b):
    return jax.lax.dot_general(a, b, NT_DIMS, preferred_element_type=f32)


def _span(i, n):
    if isinstance(i, int):
        return pl.ds(i * n, n)
    return pl.ds(pl.multiple_of(i * n, n), n)


def _kernel(x_hbm, kt_hbm, vt_hbm, wq_hbm, wo_hbm, wr_hbm, wg_hbm, wu_hbm, wd_hbm,
            out_hbm,
            x_ref, xn_ref, acc_ref, wq_ref, wo_ref, kt_ref, vt_ref, kb_ref, vb_ref,
            q_ref, o_ref, s_ref, m_ref, g_ref, top_ref,
            wr_ref, wg_ref, wu_ref, wd_ref, out_ref,
            sem_x, sem_g0, sem_ga, sem_gb, sem_gc, sem_moe, sem_out):
    sk = kt_hbm.shape[-1]

    win = pl.ds(sk - W, W)

    def x_copy(r0, n, sem):
        rows = pl.ds(r0, n)
        return pltpu.make_async_copy(x_hbm.at[0, rows, :], x_ref.at[rows, :], sem)

    def wq_copies(p0, n, sem):
        return [pltpu.make_async_copy(wq_hbm.at[:, pl.ds(p * PW, PW)], wq_ref.at[p], sem)
                for p in range(p0, p0 + n)]

    def wo_copy(p0, n, sem):
        rows = pl.ds(p0 * PW, n * PW)
        return pltpu.make_async_copy(wo_hbm.at[rows, :], wo_ref.at[rows, :], sem)

    def kv_copy(src, dst, p0, n, sem):
        heads = pl.ds(2 * p0, 2 * n)
        return pltpu.make_async_copy(src.at[0, heads, :, win], dst.at[heads], sem)

    def group_copies(p0, n, sems, n_wo=None):
        return [kv_copy(kt_hbm, kt_ref, p0 + 1, n, sems.at[0]),
                kv_copy(vt_hbm, vt_ref, p0 + 1, n, sems.at[1]),
                wo_copy(p0, n if n_wo is None else n_wo, sems.at[3])] + wq_copies(p0 + 1, n, sems.at[2])

    x0_copies = [x_copy(c * 128, 128, sem_x.at[c]) for c in range(4)]
    x_copies = [None] + [x_copy(b * TQ, TQ, sem_x.at[3 + b]) for b in range(1, NB)]
    wq0_copy, = wq_copies(0, 1, sem_g0.at[0])
    kt0_copy = kv_copy(kt_hbm, kt_ref, 0, 1, sem_g0.at[1])
    vt0_copy = kv_copy(vt_hbm, vt_ref, 0, 1, sem_g0.at[2])
    wr_copy = pltpu.make_async_copy(wr_hbm, wr_ref, sem_g0.at[3])
    ga = group_copies(0, 1, sem_ga)
    gb = group_copies(1, 2, sem_gb)
    gc = group_copies(3, NP - 4, sem_gc, n_wo=NP - 3)
    moe_copies = [pltpu.make_async_copy(wg_hbm, wg_ref, sem_moe.at[0]),
                  pltpu.make_async_copy(wu_hbm, wu_ref, sem_moe.at[1]),
                  pltpu.make_async_copy(wd_hbm, wd_ref, sem_moe.at[2])]

    def out_copy(b):
        rows = pl.ds(b * TQ, TQ)
        return pltpu.make_async_copy(out_ref.at[rows, :], out_hbm.at[0, rows, :], sem_out.at[b])

    last_copies = [
        pltpu.make_async_copy(out_ref.at[pl.ds((NB - 1) * TQ + c * (TQ // NLAST), TQ // NLAST), :],
                              out_hbm.at[0, pl.ds((NB - 1) * TQ + c * (TQ // NLAST), TQ // NLAST), :],
                              sem_out.at[NB - 1 + c]) for c in range(NLAST)]

    def layer_norm_rows(r0):
        outs = []
        for xf in _even_odd(_pack(x_ref[r0:r0 + 128, :])):
            mean = jnp.sum(xf, axis=-1, keepdims=True) * (1.0 / D)
            xc = xf - mean
            var = jnp.sum(xc * xc, axis=-1, keepdims=True) * (1.0 / D)
            d = _rb(xf - _rb(mean))
            ve = _rb(_rb(var) + EPS_BF16)
            den = _rb(ve * jax.lax.rsqrt(ve))
            outs.append(d * _recip(den))
        xn_ref[r0 // 2:r0 // 2 + 64, :] = _pack2(*outs)

    def layer_norm(b):
        for c in range(TQ // 128):
            layer_norm_rows(b * TQ + c * 128)

    def gate_router(c):
        valid = c < NIT
        c = jnp.minimum(c, NIT - 1)
        prow = _span(c, GR // 2)
        wr = wr_ref[...].astype(f32).reshape(1, D)
        gs = []
        row = jax.lax.broadcasted_iota(i32, (GR // 2, 128), 0)
        for par, xn in enumerate(_even_odd(xn_ref[prow, :])):
            gs.append(xn * _rb(_sigmoid(xn)))
            r = _rb(jnp.sum(xn * wr, axis=-1, keepdims=True)) + 0.0
            bits = pltpu.bitcast(jnp.broadcast_to(r, (GR // 2, 128)), i32)
            key = jnp.where(bits < 0, bits ^ jnp.int32(0x7FFF0000), bits)
            key = key | (0xFFFF - (c * GR + par + 2 * row))
            key = jnp.where(valid, key, KEY_MIN)
            k1 = top_ref[par, 0]
            top_ref[par, 0] = jnp.maximum(k1, key)
            top_ref[par, 1] = jnp.maximum(top_ref[par, 1], jnp.minimum(k1, key))
        g_ref[prow, :] = _pack2(*gs)

    def q_stage(p, b, half=None):
        if half is None:
            src, dst = _span(b, TQ // 2), pl.ds(0, TQ // 2)
        else:
            src, dst = _span(2 * b + half, TQ // 4), _span(half, TQ // 4)
        q = _dot(_unpack(xn_ref[src, :]), wq_ref[p])
        q_ref[dst, :] = _pack((q * QSCALE).astype(bf16))

    def _quarter(t):
        if isinstance(t, int):
            return pl.ds(t * 128, 128), pl.ds(t * 64, 64)
        return (pl.ds(pl.multiple_of(t * 128, 128), 128), pl.ds(pl.multiple_of(t * 64, 64), 64))

    def k_prep(p, t, dst=None):
        dst = p if dst is None else dst
        cols, prow = _quarter(t)
        zpad = jnp.zeros((KP - DH, 128), bf16)
        for h in range(2):
            kt = kt_ref[2 * p + h, :, cols]
            kt = jnp.concatenate([kt, zpad] if h == 0 else [zpad, kt], axis=0)
            ke, ko = _even_odd(_pack(kt.T))
            kb_ref[dst % 2, h, prow, :] = _pack(jnp.concatenate([ke, ko], axis=0).astype(bf16))

    def v_prep(p, t, dst=None):
        dst = p if dst is None else dst
        cols, _ = _quarter(t)
        for h in range(2):
            vb_ref[dst % 2, h, :, cols] = _pack(vt_ref[2 * p + h, :, cols])

    def s_stage(p):
        slot = p % 2
        for j in range(NJ):
            for h in range(2):
                qh = _unpack(q_ref[64 * j:64 * (j + 1), 128 * h:128 * h + 256])
                st = _dot_nt(_unpack(kb_ref[slot, h]), qh)
                s_ref[2 * j + h] = st
                m_ref[2 * j + h] = jnp.max(st.reshape(W // 8, 8, 128), axis=0)

    def c_stage():
        ls = []
        ps = []
        for u in range(2 * NJ):
            m = jnp.max(m_ref[u], axis=0, keepdims=True)
            pt = jnp.exp2(s_ref[u] - m)
            ls.append(jnp.sum(pt, axis=0, keepdims=True))
            ps.append(jnp.concatenate(
                [_pack2(pt[128 * c:128 * c + 64], pt[128 * c + 64:128 * c + 128])
                 for c in range(W // 128)], axis=0))
        return ls, ps

    def p_stage(p, ls, ps):
        slot = p % 2
        os_ = []
        for j in range(NJ):
            ots = []
            for h in range(2):
                ot = _dot(_unpack(vb_ref[slot, h]), _unpack(ps[2 * j + h]))
                ots.append(ot * (1.0 / ls[2 * j + h]))
            os_.append(jnp.concatenate(ots, axis=0).T)
        o_ref[...] = _pack(jnp.concatenate(os_, axis=0).astype(bf16))

    def o_dot(p):
        return _dot(_unpack(o_ref[...]), wo_ref[_span(p, PW), :])

    def rows_of(b):
        if isinstance(b, int):
            return pl.ds(b * TQ, TQ)
        return pl.ds(pl.multiple_of(b * TQ, TQ), TQ)

    def finish(b, s):
        rows = rows_of(b)
        if isinstance(b, int):
            prow = pl.ds(b * (TQ // 2), TQ // 2)
        else:
            prow = pl.ds(pl.multiple_of(b * (TQ // 2), TQ // 2), TQ // 2)
        g = _unpack(g_ref[prow, :]).astype(f32)
        out_ref[rows, :] = (x_ref[rows, :].astype(f32) + _rb(_rb(s) * g)).astype(bf16)

    for c in x0_copies:
        c.start()
    wq0_copy.start()
    for par in range(2):
        for j in range(2):
            top_ref[par, j] = jnp.full((GR // 2, 128), KEY_MIN, i32)

    for c in range(4):
        x0_copies[c].wait()
        if c == 0:
            kt0_copy.start()
        if c == 3:
            x_copies[1].start()
        layer_norm_rows(c * 128)

    wq0_copy.wait()
    q_stage(0, 0, 0)
    kt0_copy.wait()
    wr_copy.start()
    vt0_copy.start()
    x_copies[2].start()
    x_copies[3].start()
    for t in range(4):
        k_prep(0, t)
    q_stage(0, 0, 1)

    x_copies[1].wait()
    layer_norm(1)
    s_stage(0)

    wr_copy.wait()
    vt0_copy.wait()
    x_copies[2].wait()
    x_copies[3].wait()
    for c in ga:
        c.start()
    for t in range(4):
        v_prep(0, t)
    ls, ps = c_stage()
    q_stage(0, 1)
    p_stage(0, ls, ps)
    s_stage(0)
    layer_norm(2)
    layer_norm(3)
    for c in range(ROUTER_LEAD + 1):
        gate_router(c)
    for c in ga:
        c.wait()
    for c in gb:
        c.start()

    def step(p, b, first):
        pn, bn = (p, b + 1) if b + 1 < NB else (p + 1, 0)
        pp, bp = (p, b - 1) if b > 0 else (p - 1, NB - 1)
        ls, ps = c_stage()
        q_stage(pn, bn)
        rows = rows_of(bp)
        acc_ref[rows, :] = jnp.where(first, 0.0, acc_ref[rows, :]) + o_dot(pp)
        p_stage(p, ls, ps)
        s_stage(pn)

    def quad(p, carry):
        first = p == 0
        for t in range(NB):
            k_prep(p + 1, t)
            v_prep(p + 1, t)
        for b in range(1, NB + 1):
            gate_router(p * NB + b + ROUTER_LEAD)
        for b in range(1, NB):
            step(p, b, first)
        step(p + 1, 0, first)
        return carry

    def segment(sgm, carry):
        @pl.when(sgm == 1)
        def _():
            for c in gb:
                c.wait()
            for c in gc:
                c.start()

        @pl.when(sgm == 2)
        def _():
            for c in gc:
                c.wait()
            for c in moe_copies:
                c.start()

        lo = jnp.where(sgm == 0, 0, jnp.where(sgm == 1, 1, 3))
        hi = jnp.where(sgm == 0, 1, jnp.where(sgm == 1, 3, NP - 1))
        jax.lax.fori_loop(lo, hi, quad, 0)
        return carry

    jax.lax.fori_loop(0, 3, segment, 0)

    keys = jnp.concatenate([top_ref[0, 0], top_ref[1, 0], top_ref[0, 1], top_ref[1, 1]], axis=0)
    top1 = jnp.max(keys, axis=0, keepdims=True)
    top2 = jnp.max(jnp.where(keys == top1, KEY_MIN, keys), axis=0, keepdims=True)
    key1 = top1[0, 0]
    key2 = top2[0, 0]

    def decode(key):
        idx = jnp.clip(0xFFFF - (key & 0xFFFF), 0, S - 1)
        hi = key & jnp.int32(-65536)
        bits = jnp.where(hi < 0, hi ^ jnp.int32(0x7FFF0000), hi)
        return idx, bits

    i1, b1 = decode(key1)
    i2, b2 = decode(key2)

    for c in moe_copies:
        c.wait()
    row16 = jax.lax.broadcasted_iota(i32, (16, D), 0)
    xrows = []
    for idx in (i1, i2):
        e, o = _even_odd(xn_ref[pl.ds(idx // 2, 1), :])
        xrows.append(jnp.where(idx % 2 == 0, e, o))
    xs = jnp.where(row16 == 0, xrows[0], jnp.where(row16 == 1, xrows[1], 0.0)).astype(bf16)
    hg = _rb(_dot(xs, wg_ref[...]))
    hg = _rb(hg * _rb(_sigmoid(hg)))
    hu = _rb(_dot(xs, wu_ref[...]))
    y = _rb(_dot((hg * hu).astype(bf16), wd_ref[...]))
    rs = pltpu.bitcast(jnp.where(row16 == 0, b1, b2), f32)
    y = _rb(y * _rb(_sigmoid(rs)))
    for j, idx in enumerate((i1, i2)):
        gin = _rb(xrows[j] + y[j:j + 1, :])
        gbits = pltpu.bitcast(_rb(gin * _rb(_sigmoid(gin))), u32)
        word = pl.ds(idx // 2, 1)
        old = g_ref[word, :]
        g_ref[word, :] = jnp.where(idx % 2 == 0,
                                   (old & jnp.uint32(0xFFFF0000)) | (gbits >> 16),
                                   (old & jnp.uint32(0x0000FFFF)) | gbits)

    for b in range(1, NB):
        ls, ps = c_stage()
        if b + 1 < NB:
            q_stage(NP - 1, b + 1)
        finish(b - 1, acc_ref[rows_of(b - 1), :] + o_dot(NP - 1))
        p_stage(NP - 1, ls, ps)
        if b + 1 < NB:
            s_stage(NP - 1)
        out_copy(b - 1).start()
    for c in range(NLAST):
        n = TQ // NLAST
        r0 = (NB - 1) * TQ + c * n
        o = _unpack(o_ref[c * n // 2:(c + 1) * n // 2, :])
        sacc = acc_ref[r0:r0 + n, :] + _dot(o, wo_ref[_span(NP - 1, PW), :])
        g = _unpack(g_ref[r0 // 2:(r0 + n) // 2, :]).astype(f32)
        out_ref[r0:r0 + n, :] = (x_ref[r0:r0 + n, :].astype(f32) + _rb(_rb(sacc) * g)).astype(bf16)
        last_copies[c].start()
    for b in range(NB - 1):
        out_copy(b).wait()
    for c in last_copies:
        c.wait()

@jax.jit
def pallas_recurrent_scan__sliding_block_cached__moe_arch_mod__prompt_kernel(
    A_x, A_k_cache, A_v_cache, A_wq, A_wo, B_x, B_w_r, B_w_gate, B_w_up, B_w_down,
):
    kt = jnp.swapaxes(A_k_cache, 2, 3)
    vt = jnp.swapaxes(A_v_cache, 2, 3)
    any_spec = pl.BlockSpec(memory_space=pl.ANY)
    return pl.pallas_call(
        _kernel,
        in_specs=[any_spec] * 9,
        out_specs=any_spec,
        out_shape=jax.ShapeDtypeStruct(A_x.shape, A_x.dtype),
        scratch_shapes=[
            pltpu.VMEM((S, D), bf16),
            pltpu.VMEM((S // 2, D), u32),
            pltpu.VMEM((S, D), f32),
            pltpu.VMEM((NP, D, PW), bf16),
            pltpu.VMEM((H * DH, D), bf16),
            pltpu.VMEM((H, DH, W), bf16),
            pltpu.VMEM((H, DH, W), bf16),
            pltpu.VMEM((2, 2, W // 2, KP), u32),
            pltpu.VMEM((2, 2, DH // 2, W), u32),
            pltpu.VMEM((TQ // 2, PW), u32),
            pltpu.VMEM((TQ // 2, PW), u32),
            pltpu.VMEM((2 * NJ, W, 128), f32),
            pltpu.VMEM((2 * NJ, 8, 128), f32),
            pltpu.VMEM((S // 2, D), u32),
            pltpu.VMEM((2, 2, GR // 2, 128), i32),
            pltpu.VMEM((D,), bf16),
            pltpu.VMEM((D, F), bf16),
            pltpu.VMEM((D, F), bf16),
            pltpu.VMEM((F, D), bf16),
            pltpu.VMEM((S, D), bf16),
            pltpu.SemaphoreType.DMA((4 + NB - 1,)),
            pltpu.SemaphoreType.DMA((4,)),
            pltpu.SemaphoreType.DMA((4,)),
            pltpu.SemaphoreType.DMA((4,)),
            pltpu.SemaphoreType.DMA((4,)),
            pltpu.SemaphoreType.DMA((3,)),
            pltpu.SemaphoreType.DMA((NB - 1 + NLAST,)),
        ],
        compiler_params=pltpu.CompilerParams(
            vmem_limit_bytes=128 * 1024 * 1024,
            disable_bounds_checks=True,
        ),
    )(A_x, kt, vt, A_wq, A_wo, B_w_r, B_w_gate, B_w_up, B_w_down)
```

```python
import math

import jax
import jax.numpy as jnp
import jax.experimental.pallas as pl
import jax.experimental.pallas.tpu as pltpu

S, D = 2048, 640
H, DH, W = 32, 192, 512
F = 1536
NP = H // 2
PW = 2 * DH
TQ = 512
NB = S // TQ
NJ = TQ // 128
NIT = NP * NB
KP = 256
GR = S // NIT
ROUTER_LEAD = 4
NLAST = 4
KEY_MIN = -2 ** 31
NT_DIMS = (((1,), (1,)), ((), ()))
QSCALE = (DH ** -0.5) * math.log2(math.e)
LOG2E = math.log2(math.e)
EPS_BF16 = 1.0013580322265625e-05

bf16 = jnp.bfloat16
f32 = jnp.float32
u32 = jnp.uint32
i32 = jnp.int32


def _rb(t):
    return t.astype(bf16).astype(f32)


def _sigmoid(t):
    return 0.5 * jnp.tanh(0.5 * t) + 0.5


def _recip(t):
    r = pl.reciprocal(t, approx=True)
    return r * (2.0 - t * r)


def _pack(t):
    return pltpu.bitcast(t, u32)


def _unpack(t):
    return pltpu.bitcast(t, bf16)


def _even_odd(u):
    return (pltpu.unpack_elementwise(u, index=0, packed_dtype=bf16, unpacked_dtype=f32),
            pltpu.unpack_elementwise(u, index=1, packed_dtype=bf16, unpacked_dtype=f32))


def _pack2(e, o):
    return pltpu.pack_elementwise([e, o], packed_dtype=bf16)


def _dot(a, b):
    return jnp.dot(a, b, preferred_element_type=f32)


def _dot_nt(a, b):
    return jax.lax.dot_general(a, b, NT_DIMS, preferred_element_type=f32)


def _span(i, n):
    if isinstance(i, int):
        return pl.ds(i * n, n)
    return pl.ds(pl.multiple_of(i * n, n), n)


def _kernel(x_hbm, kt_hbm, vt_hbm, wq_hbm, wo_hbm, wr_hbm, wg_hbm, wu_hbm, wd_hbm,
            out_hbm,
            x_ref, xn_ref, acc_ref, wq_ref, wo_ref, kt_ref, vt_ref, kb_ref, vb_ref,
            q_ref, o_ref, s_ref, m_ref, g_ref, top_ref,
            wr_ref, wg_ref, wu_ref, wd_ref, out_ref,
            sem_x, sem_g0, sem_ga, sem_gb, sem_gc, sem_moe, sem_out):
    sk = kt_hbm.shape[-1]

    win = pl.ds(sk - W, W)

    def x_copy(r0, n, sem):
        rows = pl.ds(r0, n)
        return pltpu.make_async_copy(x_hbm.at[0, rows, :], x_ref.at[rows, :], sem)

    def wq_copies(p0, n, sem):
        return [pltpu.make_async_copy(wq_hbm.at[:, pl.ds(p * PW, PW)], wq_ref.at[p], sem)
                for p in range(p0, p0 + n)]

    def wo_copy(p0, n, sem):
        rows = pl.ds(p0 * PW, n * PW)
        return pltpu.make_async_copy(wo_hbm.at[rows, :], wo_ref.at[rows, :], sem)

    def kv_copy(src, dst, p0, n, sem):
        heads = pl.ds(2 * p0, 2 * n)
        return pltpu.make_async_copy(src.at[0, heads, :, win], dst.at[heads], sem)

    def group_copies(p0, n, sems, n_wo=None):
        return [kv_copy(kt_hbm, kt_ref, p0 + 1, n, sems.at[0]),
                kv_copy(vt_hbm, vt_ref, p0 + 1, n, sems.at[1]),
                wo_copy(p0, n if n_wo is None else n_wo, sems.at[3])] + wq_copies(p0 + 1, n, sems.at[2])

    x0_copies = [x_copy(c * 128, 128, sem_x.at[c]) for c in range(4)]
    x_copies = [None] + [x_copy(b * TQ, TQ, sem_x.at[3 + b]) for b in range(1, NB)]
    wq0_copy, = wq_copies(0, 1, sem_g0.at[0])
    kt0_copy = kv_copy(kt_hbm, kt_ref, 0, 1, sem_g0.at[1])
    vt0_copy = kv_copy(vt_hbm, vt_ref, 0, 1, sem_g0.at[2])
    wr_copy = pltpu.make_async_copy(wr_hbm, wr_ref, sem_g0.at[3])
    ga = group_copies(0, 1, sem_ga)
    gb = group_copies(1, 2, sem_gb)
    gc = group_copies(3, NP - 4, sem_gc, n_wo=NP - 3)
    moe_copies = [pltpu.make_async_copy(wg_hbm, wg_ref, sem_moe.at[0]),
                  pltpu.make_async_copy(wu_hbm, wu_ref, sem_moe.at[1]),
                  pltpu.make_async_copy(wd_hbm, wd_ref, sem_moe.at[2])]

    def out_copy(b):
        rows = pl.ds(b * TQ, TQ)
        return pltpu.make_async_copy(out_ref.at[rows, :], out_hbm.at[0, rows, :], sem_out.at[b])

    last_copies = [
        pltpu.make_async_copy(out_ref.at[pl.ds((NB - 1) * TQ + c * (TQ // NLAST), TQ // NLAST), :],
                              out_hbm.at[0, pl.ds((NB - 1) * TQ + c * (TQ // NLAST), TQ // NLAST), :],
                              sem_out.at[NB - 1 + c]) for c in range(NLAST)]

    def layer_norm_rows(r0):
        outs = []
        for xf in _even_odd(_pack(x_ref[r0:r0 + 128, :])):
            mean = jnp.sum(xf, axis=-1, keepdims=True) * (1.0 / D)
            xc = xf - mean
            var = jnp.sum(xc * xc, axis=-1, keepdims=True) * (1.0 / D)
            d = _rb(xf - _rb(mean))
            ve = _rb(_rb(var) + EPS_BF16)
            den = _rb(ve * jax.lax.rsqrt(ve))
            outs.append(d * _recip(den))
        xn_ref[r0 // 2:r0 // 2 + 64, :] = _pack2(*outs)

    def layer_norm(b):
        for c in range(TQ // 128):
            layer_norm_rows(b * TQ + c * 128)

    def gate_router(c):
        valid = c < NIT
        c = jnp.minimum(c, NIT - 1)
        prow = _span(c, GR // 2)
        wr = wr_ref[...].astype(f32).reshape(1, D)
        gs = []
        row = jax.lax.broadcasted_iota(i32, (GR // 2, 128), 0)
        for par, xn in enumerate(_even_odd(xn_ref[prow, :])):
            gs.append(xn * _rb(_sigmoid(xn)))
            r = _rb(jnp.sum(xn * wr, axis=-1, keepdims=True)) + 0.0
            bits = pltpu.bitcast(jnp.broadcast_to(r, (GR // 2, 128)), i32)
            key = jnp.where(bits < 0, bits ^ jnp.int32(0x7FFF0000), bits)
            key = key | (0xFFFF - (c * GR + par + 2 * row))
            key = jnp.where(valid, key, KEY_MIN)
            k1 = top_ref[par, 0]
            top_ref[par, 0] = jnp.maximum(k1, key)
            top_ref[par, 1] = jnp.maximum(top_ref[par, 1], jnp.minimum(k1, key))
        g_ref[prow, :] = _pack2(*gs)

    def q_stage(p, b, half=None):
        if half is None:
            src, dst = _span(b, TQ // 2), pl.ds(0, TQ // 2)
        else:
            src, dst = _span(2 * b + half, TQ // 4), _span(half, TQ // 4)
        q = _dot(_unpack(xn_ref[src, :]), wq_ref[p])
        q_ref[dst, :] = _pack((q * QSCALE).astype(bf16))

    def _quarter(t):
        if isinstance(t, int):
            return pl.ds(t * 128, 128), pl.ds(t * 64, 64)
        return (pl.ds(pl.multiple_of(t * 128, 128), 128), pl.ds(pl.multiple_of(t * 64, 64), 64))

    def k_prep(p, t, dst=None):
        dst = p if dst is None else dst
        cols, prow = _quarter(t)
        zpad = jnp.zeros((KP - DH, 128), bf16)
        for h in range(2):
            kt = kt_ref[2 * p + h, :, cols]
            kt = jnp.concatenate([kt, zpad] if h == 0 else [zpad, kt], axis=0)
            ke, ko = _even_odd(_pack(kt.T))
            kb_ref[dst % 2, h, prow, :] = _pack(jnp.concatenate([ke, ko], axis=0).astype(bf16))

    def v_prep(p, t, dst=None):
        dst = p if dst is None else dst
        cols, _ = _quarter(t)
        for h in range(2):
            vb_ref[dst % 2, h, 0:DH // 2, cols] = _pack(vt_ref[2 * p + h, :, cols])

    def s_stage(p):
        slot = p % 2
        for j in range(NJ):
            for h in range(2):
                qh = _unpack(q_ref[64 * j:64 * (j + 1), 128 * h:128 * h + 256])
                st = _dot_nt(_unpack(kb_ref[slot, h, 0:W // 2, :]), qh)
                s_ref[2 * j + h] = st
                m_ref[2 * j + h] = jnp.max(st.reshape(W // 8, 8, 128), axis=0)

    def c_stage():
        ls = []
        ps = []
        for u in range(2 * NJ):
            m = jnp.max(m_ref[u], axis=0, keepdims=True)
            pt = jnp.exp2(s_ref[u] - m)
            ls.append(jnp.sum(pt, axis=0, keepdims=True))
            ps.append(jnp.concatenate(
                [_pack2(pt[128 * c:128 * c + 64], pt[128 * c + 64:128 * c + 128])
                 for c in range(W // 128)], axis=0))
        return ls, ps

    def p_stage(p, ls, ps):
        slot = p % 2
        os_ = []
        for j in range(NJ):
            ots = []
            for h in range(2):
                ot = _dot(_unpack(vb_ref[slot, h, 0:DH // 2, :]), _unpack(ps[2 * j + h]))
                ots.append(ot * (1.0 / ls[2 * j + h]))
            os_.append(jnp.concatenate(ots, axis=0).T)
        o_ref[...] = _pack(jnp.concatenate(os_, axis=0).astype(bf16))

    def o_dot(p):
        return _dot(_unpack(o_ref[...]), wo_ref[_span(p, PW), :])

    def rows_of(b):
        if isinstance(b, int):
            return pl.ds(b * TQ, TQ)
        return pl.ds(pl.multiple_of(b * TQ, TQ), TQ)

    def finish(b, s):
        rows = rows_of(b)
        if isinstance(b, int):
            prow = pl.ds(b * (TQ // 2), TQ // 2)
        else:
            prow = pl.ds(pl.multiple_of(b * (TQ // 2), TQ // 2), TQ // 2)
        g = _unpack(g_ref[prow, :]).astype(f32)
        out_ref[rows, :] = (x_ref[rows, :].astype(f32) + _rb(_rb(s) * g)).astype(bf16)

    for c in x0_copies:
        c.start()
    wq0_copy.start()
    for par in range(2):
        for j in range(2):
            top_ref[par, j] = jnp.full((GR // 2, 128), KEY_MIN, i32)

    for c in range(4):
        x0_copies[c].wait()
        if c == 0:
            kt0_copy.start()
        if c == 3:
            x_copies[1].start()
        layer_norm_rows(c * 128)

    wq0_copy.wait()
    q_stage(0, 0, 0)
    kt0_copy.wait()
    wr_copy.start()
    vt0_copy.start()
    x_copies[2].start()
    x_copies[3].start()
    for t in range(4):
        k_prep(0, t)
    q_stage(0, 0, 1)

    x_copies[1].wait()
    layer_norm(1)
    s_stage(0)

    wr_copy.wait()
    vt0_copy.wait()
    x_copies[2].wait()
    x_copies[3].wait()
    for c in ga:
        c.start()
    for t in range(4):
        v_prep(0, t)
    ls, ps = c_stage()
    q_stage(0, 1)
    p_stage(0, ls, ps)
    s_stage(0)
    layer_norm(2)
    layer_norm(3)
    for c in range(ROUTER_LEAD + 1):
        gate_router(c)
    for c in ga:
        c.wait()
    for c in gb:
        c.start()

    def step(p, b, first):
        pn, bn = (p, b + 1) if b + 1 < NB else (p + 1, 0)
        pp, bp = (p, b - 1) if b > 0 else (p - 1, NB - 1)
        ls, ps = c_stage()
        q_stage(pn, bn)
        rows = rows_of(bp)
        acc_ref[rows, :] = jnp.where(first, 0.0, acc_ref[rows, :]) + o_dot(pp)
        p_stage(p, ls, ps)
        s_stage(pn)

    def quad(p, carry):
        first = p == 0
        for t in range(NB):
            k_prep(p + 1, t)
            v_prep(p + 1, t)
        for b in range(1, NB + 1):
            gate_router(p * NB + b + ROUTER_LEAD)
        for b in range(1, NB):
            step(p, b, first)
        step(p + 1, 0, first)
        return carry

    def segment(sgm, carry):
        @pl.when(sgm == 1)
        def _():
            for c in gb:
                c.wait()
            for c in gc:
                c.start()

        @pl.when(sgm == 2)
        def _():
            for c in gc:
                c.wait()
            for c in moe_copies:
                c.start()

        lo = jnp.where(sgm == 0, 0, jnp.where(sgm == 1, 1, 3))
        hi = jnp.where(sgm == 0, 1, jnp.where(sgm == 1, 3, NP - 1))
        jax.lax.fori_loop(lo, hi, quad, 0)
        return carry

    jax.lax.fori_loop(0, 3, segment, 0)

    keys = jnp.concatenate([top_ref[0, 0], top_ref[1, 0], top_ref[0, 1], top_ref[1, 1]], axis=0)
    top1 = jnp.max(keys, axis=0, keepdims=True)
    top2 = jnp.max(jnp.where(keys == top1, KEY_MIN, keys), axis=0, keepdims=True)
    key1 = top1[0, 0]
    key2 = top2[0, 0]

    def decode(key):
        idx = jnp.clip(0xFFFF - (key & 0xFFFF), 0, S - 1)
        hi = key & jnp.int32(-65536)
        bits = jnp.where(hi < 0, hi ^ jnp.int32(0x7FFF0000), hi)
        return idx, bits

    i1, b1 = decode(key1)
    i2, b2 = decode(key2)

    for c in moe_copies:
        c.wait()
    row16 = jax.lax.broadcasted_iota(i32, (16, D), 0)
    xrows = []
    for idx in (i1, i2):
        e, o = _even_odd(xn_ref[pl.ds(idx // 2, 1), :])
        xrows.append(jnp.where(idx % 2 == 0, e, o))
    xs = jnp.where(row16 == 0, xrows[0], jnp.where(row16 == 1, xrows[1], 0.0)).astype(bf16)
    hg = _rb(_dot(xs, wg_ref[...]))
    hg = _rb(hg * _rb(_sigmoid(hg)))
    hu = _rb(_dot(xs, wu_ref[...]))
    y = _rb(_dot((hg * hu).astype(bf16), wd_ref[...]))
    rs = pltpu.bitcast(jnp.where(row16 == 0, b1, b2), f32)
    y = _rb(y * _rb(_sigmoid(rs)))
    for j, idx in enumerate((i1, i2)):
        gin = _rb(xrows[j] + y[j:j + 1, :])
        gbits = pltpu.bitcast(_rb(gin * _rb(_sigmoid(gin))), u32)
        word = pl.ds(idx // 2, 1)
        old = g_ref[word, :]
        g_ref[word, :] = jnp.where(idx % 2 == 0,
                                   (old & jnp.uint32(0xFFFF0000)) | (gbits >> 16),
                                   (old & jnp.uint32(0x0000FFFF)) | gbits)

    for b in range(1, NB):
        ls, ps = c_stage()
        if b + 1 < NB:
            q_stage(NP - 1, b + 1)
        finish(b - 1, acc_ref[rows_of(b - 1), :] + o_dot(NP - 1))
        p_stage(NP - 1, ls, ps)
        if b + 1 < NB:
            s_stage(NP - 1)
        out_copy(b - 1).start()
    for c in range(NLAST):
        n = TQ // NLAST
        r0 = (NB - 1) * TQ + c * n
        o = _unpack(o_ref[c * n // 2:(c + 1) * n // 2, :])
        sacc = acc_ref[r0:r0 + n, :] + _dot(o, wo_ref[_span(NP - 1, PW), :])
        g = _unpack(g_ref[r0 // 2:(r0 + n) // 2, :]).astype(f32)
        out_ref[r0:r0 + n, :] = (x_ref[r0:r0 + n, :].astype(f32) + _rb(_rb(sacc) * g)).astype(bf16)
        last_copies[c].start()
    for b in range(NB - 1):
        out_copy(b).wait()
    for c in last_copies:
        c.wait()

@jax.jit
def pallas_recurrent_scan__sliding_block_cached__moe_arch_mod__prompt_kernel(
    A_x, A_k_cache, A_v_cache, A_wq, A_wo, B_x, B_w_r, B_w_gate, B_w_up, B_w_down,
):
    kt = jnp.swapaxes(A_k_cache, 2, 3)
    vt = jnp.swapaxes(A_v_cache, 2, 3)
    any_spec = pl.BlockSpec(memory_space=pl.ANY)
    return pl.pallas_call(
        _kernel,
        in_specs=[any_spec] * 9,
        out_specs=any_spec,
        out_shape=jax.ShapeDtypeStruct(A_x.shape, A_x.dtype),
        scratch_shapes=[
            pltpu.VMEM((S, D), bf16),
            pltpu.VMEM((S // 2, D), u32),
            pltpu.VMEM((S, D), f32),
            pltpu.VMEM((NP, D, PW), bf16),
            pltpu.VMEM((H * DH, D), bf16),
            pltpu.VMEM((H, DH, W), bf16),
            pltpu.VMEM((H, DH, W), bf16),
            pltpu.VMEM((2, 2, W // 2 + 8, KP), u32),
            pltpu.VMEM((2, 2, DH // 2 + 8, W), u32),
            pltpu.VMEM((TQ // 2, PW), u32),
            pltpu.VMEM((TQ // 2, PW), u32),
            pltpu.VMEM((2 * NJ, W, 128), f32),
            pltpu.VMEM((2 * NJ, 8, 128), f32),
            pltpu.VMEM((S // 2, D), u32),
            pltpu.VMEM((2, 2, GR // 2, 128), i32),
            pltpu.VMEM((D,), bf16),
            pltpu.VMEM((D, F), bf16),
            pltpu.VMEM((D, F), bf16),
            pltpu.VMEM((F, D), bf16),
            pltpu.VMEM((S, D), bf16),
            pltpu.SemaphoreType.DMA((4 + NB - 1,)),
            pltpu.SemaphoreType.DMA((4,)),
            pltpu.SemaphoreType.DMA((4,)),
            pltpu.SemaphoreType.DMA((4,)),
            pltpu.SemaphoreType.DMA((4,)),
            pltpu.SemaphoreType.DMA((3,)),
            pltpu.SemaphoreType.DMA((NB - 1 + NLAST,)),
        ],
        compiler_params=pltpu.CompilerParams(
            vmem_limit_bytes=128 * 1024 * 1024,
            disable_bounds_checks=True,
        ),
    )(A_x, kt, vt, A_wq, A_wo, B_w_r, B_w_gate, B_w_up, B_w_down)
```

```python
import math

import jax
import jax.numpy as jnp
import jax.experimental.pallas as pl
import jax.experimental.pallas.tpu as pltpu

S, D = 2048, 640
H, DH, W = 32, 192, 512
F = 1536
NP = H // 2
PW = 2 * DH
TQ = 512
NB = S // TQ
NJ = TQ // 128
NIT = NP * NB
KP = 256
GR = S // NIT
ROUTER_LEAD = 4
NLAST = 4
KEY_MIN = -2 ** 31
NT_DIMS = (((1,), (1,)), ((), ()))
QSCALE = (DH ** -0.5) * math.log2(math.e)
LOG2E = math.log2(math.e)
EPS_BF16 = 1.0013580322265625e-05

bf16 = jnp.bfloat16
f32 = jnp.float32
u32 = jnp.uint32
i32 = jnp.int32


def _rb(t):
    return t.astype(bf16).astype(f32)


def _sigmoid(t):
    return 0.5 * jnp.tanh(0.5 * t) + 0.5


def _recip(t):
    r = pl.reciprocal(t, approx=True)
    return r * (2.0 - t * r)


def _pack(t):
    return pltpu.bitcast(t, u32)


def _unpack(t):
    return pltpu.bitcast(t, bf16)


def _even_odd(u):
    return (pltpu.unpack_elementwise(u, index=0, packed_dtype=bf16, unpacked_dtype=f32),
            pltpu.unpack_elementwise(u, index=1, packed_dtype=bf16, unpacked_dtype=f32))


def _pack2(e, o):
    return pltpu.pack_elementwise([e, o], packed_dtype=bf16)


def _dot(a, b):
    return jnp.dot(a, b, preferred_element_type=f32)


def _dot_nt(a, b):
    return jax.lax.dot_general(a, b, NT_DIMS, preferred_element_type=f32)


def _span(i, n):
    if isinstance(i, int):
        return pl.ds(i * n, n)
    return pl.ds(pl.multiple_of(i * n, n), n)


def _kernel(x_hbm, kt_hbm, vt_hbm, wq_hbm, wo_hbm, wr_hbm, wg_hbm, wu_hbm, wd_hbm,
            out_hbm,
            x_ref, xn_ref, acc_ref, wq_ref, wo_ref, kt_ref, vt_ref, kb_ref, vb_ref,
            wqp_ref, wop_ref, q_ref, o_ref, s_ref, m_ref, g_ref, top_ref,
            wr_ref, wg_ref, wu_ref, wd_ref, out_ref,
            sem_x, sem_g0, sem_ga, sem_gb, sem_gc, sem_moe, sem_out):
    sk = kt_hbm.shape[-1]

    win = pl.ds(sk - W, W)

    def x_copy(r0, n, sem):
        rows = pl.ds(r0, n)
        return pltpu.make_async_copy(x_hbm.at[0, rows, :], x_ref.at[rows, :], sem)

    def wq_copies(p0, n, sem):
        return [pltpu.make_async_copy(wq_hbm.at[:, pl.ds(p * PW, PW)], wq_ref.at[p], sem)
                for p in range(p0, p0 + n)]

    def wo_copy(p0, n, sem):
        rows = pl.ds(p0 * PW, n * PW)
        return pltpu.make_async_copy(wo_hbm.at[rows, :], wo_ref.at[rows, :], sem)

    def kv_copy(src, dst, p0, n, sem):
        heads = pl.ds(2 * p0, 2 * n)
        return pltpu.make_async_copy(src.at[0, heads, :, win], dst.at[heads], sem)

    def group_copies(p0, n, sems, n_wo=None):
        return [kv_copy(kt_hbm, kt_ref, p0 + 1, n, sems.at[0]),
                kv_copy(vt_hbm, vt_ref, p0 + 1, n, sems.at[1]),
                wo_copy(p0, n if n_wo is None else n_wo, sems.at[3])] + wq_copies(p0 + 1, n, sems.at[2])

    x0_copies = [x_copy(c * 128, 128, sem_x.at[c]) for c in range(4)]
    x_copies = [None] + [x_copy(b * TQ, TQ, sem_x.at[3 + b]) for b in range(1, NB)]
    wq0_copy, = wq_copies(0, 1, sem_g0.at[0])
    kt0_copy = kv_copy(kt_hbm, kt_ref, 0, 1, sem_g0.at[1])
    vt0_copy = kv_copy(vt_hbm, vt_ref, 0, 1, sem_g0.at[2])
    wr_copy = pltpu.make_async_copy(wr_hbm, wr_ref, sem_g0.at[3])
    ga = group_copies(0, 1, sem_ga)
    gb = group_copies(1, 2, sem_gb)
    gc = group_copies(3, NP - 4, sem_gc, n_wo=NP - 3)
    moe_copies = [pltpu.make_async_copy(wg_hbm, wg_ref, sem_moe.at[0]),
                  pltpu.make_async_copy(wu_hbm, wu_ref, sem_moe.at[1]),
                  pltpu.make_async_copy(wd_hbm, wd_ref, sem_moe.at[2])]

    def out_copy(b):
        rows = pl.ds(b * TQ, TQ)
        return pltpu.make_async_copy(out_ref.at[rows, :], out_hbm.at[0, rows, :], sem_out.at[b])

    last_copies = [
        pltpu.make_async_copy(out_ref.at[pl.ds((NB - 1) * TQ + c * (TQ // NLAST), TQ // NLAST), :],
                              out_hbm.at[0, pl.ds((NB - 1) * TQ + c * (TQ // NLAST), TQ // NLAST), :],
                              sem_out.at[NB - 1 + c]) for c in range(NLAST)]

    def layer_norm_rows(r0):
        outs = []
        for xf in _even_odd(_pack(x_ref[r0:r0 + 128, :])):
            mean = jnp.sum(xf, axis=-1, keepdims=True) * (1.0 / D)
            xc = xf - mean
            var = jnp.sum(xc * xc, axis=-1, keepdims=True) * (1.0 / D)
            d = _rb(xf - _rb(mean))
            ve = _rb(_rb(var) + EPS_BF16)
            den = _rb(ve * jax.lax.rsqrt(ve))
            outs.append(d * _recip(den))
        xn_ref[r0 // 2:r0 // 2 + 64, :] = _pack2(*outs)

    def layer_norm(b):
        for c in range(TQ // 128):
            layer_norm_rows(b * TQ + c * 128)

    def gate_router(c):
        valid = c < NIT
        c = jnp.minimum(c, NIT - 1)
        prow = _span(c, GR // 2)
        wr = wr_ref[...].astype(f32).reshape(1, D)
        gs = []
        row = jax.lax.broadcasted_iota(i32, (GR // 2, 128), 0)
        for par, xn in enumerate(_even_odd(xn_ref[prow, :])):
            gs.append(xn * _rb(_sigmoid(xn)))
            r = _rb(jnp.sum(xn * wr, axis=-1, keepdims=True)) + 0.0
            bits = pltpu.bitcast(jnp.broadcast_to(r, (GR // 2, 128)), i32)
            key = jnp.where(bits < 0, bits ^ jnp.int32(0x7FFF0000), bits)
            key = key | (0xFFFF - (c * GR + par + 2 * row))
            key = jnp.where(valid, key, KEY_MIN)
            k1 = top_ref[par, 0]
            top_ref[par, 0] = jnp.maximum(k1, key)
            top_ref[par, 1] = jnp.maximum(top_ref[par, 1], jnp.minimum(k1, key))
        g_ref[prow, :] = _pack2(*gs)

    def q_stage(p, b, half=None, packed=True):
        if half is None:
            src, dst = _span(b, TQ // 2), pl.ds(0, TQ // 2)
        else:
            src, dst = _span(2 * b + half, TQ // 4), _span(half, TQ // 4)
        w = _unpack(wqp_ref[p % 2]) if packed else wq_ref[p]
        q = _dot(_unpack(xn_ref[src, :]), w)
        q_ref[dst, :] = _pack((q * QSCALE).astype(bf16))

    def wq_prep(p):
        wqp_ref[p % 2] = _pack(wq_ref[p])

    def wo_prep(p):
        wop_ref[...] = _pack(wo_ref[_span(p, PW), :])

    def _quarter(t):
        if isinstance(t, int):
            return pl.ds(t * 128, 128), pl.ds(t * 64, 64)
        return (pl.ds(pl.multiple_of(t * 128, 128), 128), pl.ds(pl.multiple_of(t * 64, 64), 64))

    def k_prep(p, t, dst=None):
        dst = p if dst is None else dst
        cols, prow = _quarter(t)
        zpad = jnp.zeros((KP - DH, 128), bf16)
        for h in range(2):
            kt = kt_ref[2 * p + h, :, cols]
            kt = jnp.concatenate([kt, zpad] if h == 0 else [zpad, kt], axis=0)
            ke, ko = _even_odd(_pack(kt.T))
            kb_ref[dst % 2, h, prow, :] = _pack(jnp.concatenate([ke, ko], axis=0).astype(bf16))

    def v_prep(p, t, dst=None):
        dst = p if dst is None else dst
        cols, _ = _quarter(t)
        for h in range(2):
            vb_ref[dst % 2, h, 0:DH // 2, cols] = _pack(vt_ref[2 * p + h, :, cols])

    def s_stage(p):
        slot = p % 2
        for j in range(NJ):
            for h in range(2):
                qh = _unpack(q_ref[64 * j:64 * (j + 1), 128 * h:128 * h + 256])
                st = _dot_nt(_unpack(kb_ref[slot, h, 0:W // 2, :]), qh)
                s_ref[2 * j + h] = st
                m_ref[2 * j + h] = jnp.max(st.reshape(W // 8, 8, 128), axis=0)

    def c_stage():
        ls = []
        ps = []
        for u in range(2 * NJ):
            m = jnp.max(m_ref[u], axis=0, keepdims=True)
            pt = jnp.exp2(s_ref[u] - m)
            ls.append(jnp.sum(pt, axis=0, keepdims=True))
            ps.append(jnp.concatenate(
                [_pack2(pt[128 * c:128 * c + 64], pt[128 * c + 64:128 * c + 128])
                 for c in range(W // 128)], axis=0))
        return ls, ps

    def p_stage(p, ls, ps):
        slot = p % 2
        os_ = []
        for j in range(NJ):
            ots = []
            for h in range(2):
                ot = _dot(_unpack(vb_ref[slot, h, 0:DH // 2, :]), _unpack(ps[2 * j + h]))
                ots.append(ot * (1.0 / ls[2 * j + h]))
            os_.append(jnp.concatenate(ots, axis=0).T)
        o_ref[...] = _pack(jnp.concatenate(os_, axis=0).astype(bf16))

    def o_dot():
        return _dot(_unpack(o_ref[...]), _unpack(wop_ref[...]))

    def rows_of(b):
        if isinstance(b, int):
            return pl.ds(b * TQ, TQ)
        return pl.ds(pl.multiple_of(b * TQ, TQ), TQ)

    def finish(b, s):
        rows = rows_of(b)
        if isinstance(b, int):
            prow = pl.ds(b * (TQ // 2), TQ // 2)
        else:
            prow = pl.ds(pl.multiple_of(b * (TQ // 2), TQ // 2), TQ // 2)
        g = _unpack(g_ref[prow, :]).astype(f32)
        out_ref[rows, :] = (x_ref[rows, :].astype(f32) + _rb(_rb(s) * g)).astype(bf16)

    for c in x0_copies:
        c.start()
    wq0_copy.start()
    for par in range(2):
        for j in range(2):
            top_ref[par, j] = jnp.full((GR // 2, 128), KEY_MIN, i32)

    for c in range(4):
        x0_copies[c].wait()
        if c == 0:
            kt0_copy.start()
        if c == 3:
            x_copies[1].start()
        layer_norm_rows(c * 128)

    wq0_copy.wait()
    q_stage(0, 0, 0, packed=False)
    kt0_copy.wait()
    wr_copy.start()
    vt0_copy.start()
    x_copies[2].start()
    x_copies[3].start()
    for t in range(4):
        k_prep(0, t)
    q_stage(0, 0, 1, packed=False)

    x_copies[1].wait()
    layer_norm(1)
    s_stage(0)

    wr_copy.wait()
    vt0_copy.wait()
    x_copies[2].wait()
    x_copies[3].wait()
    for c in ga:
        c.start()
    for t in range(4):
        v_prep(0, t)
    wq_prep(0)
    ls, ps = c_stage()
    q_stage(0, 1, packed=False)
    p_stage(0, ls, ps)
    s_stage(0)
    layer_norm(2)
    layer_norm(3)
    for c in range(ROUTER_LEAD + 1):
        gate_router(c)
    for c in ga:
        c.wait()
    for c in gb:
        c.start()

    def step(p, b, first):
        pn, bn = (p, b + 1) if b + 1 < NB else (p + 1, 0)
        pp, bp = (p, b - 1) if b > 0 else (p - 1, NB - 1)
        ls, ps = c_stage()
        q_stage(pn, bn)
        rows = rows_of(bp)
        acc_ref[rows, :] = jnp.where(first, 0.0, acc_ref[rows, :]) + o_dot()
        p_stage(p, ls, ps)
        s_stage(pn)

    def quad(p, carry):
        first = p == 0
        wo_prep(p)
        for t in range(NB):
            k_prep(p + 1, t)
            v_prep(p + 1, t)
        for b in range(1, NB + 1):
            gate_router(p * NB + b + ROUTER_LEAD)
        for b in range(1, NB):
            if b == NB - 1:
                wq_prep(p + 1)
            step(p, b, first)
        step(p + 1, 0, first)
        return carry

    def segment(sgm, carry):
        @pl.when(sgm == 1)
        def _():
            for c in gb:
                c.wait()
            for c in gc:
                c.start()

        @pl.when(sgm == 2)
        def _():
            for c in gc:
                c.wait()
            for c in moe_copies:
                c.start()

        lo = jnp.where(sgm == 0, 0, jnp.where(sgm == 1, 1, 3))
        hi = jnp.where(sgm == 0, 1, jnp.where(sgm == 1, 3, NP - 1))
        jax.lax.fori_loop(lo, hi, quad, 0)
        return carry

    jax.lax.fori_loop(0, 3, segment, 0)

    keys = jnp.concatenate([top_ref[0, 0], top_ref[1, 0], top_ref[0, 1], top_ref[1, 1]], axis=0)
    top1 = jnp.max(keys, axis=0, keepdims=True)
    top2 = jnp.max(jnp.where(keys == top1, KEY_MIN, keys), axis=0, keepdims=True)
    key1 = top1[0, 0]
    key2 = top2[0, 0]

    def decode(key):
        idx = jnp.clip(0xFFFF - (key & 0xFFFF), 0, S - 1)
        hi = key & jnp.int32(-65536)
        bits = jnp.where(hi < 0, hi ^ jnp.int32(0x7FFF0000), hi)
        return idx, bits

    i1, b1 = decode(key1)
    i2, b2 = decode(key2)

    for c in moe_copies:
        c.wait()
    row16 = jax.lax.broadcasted_iota(i32, (16, D), 0)
    xrows = []
    for idx in (i1, i2):
        e, o = _even_odd(xn_ref[pl.ds(idx // 2, 1), :])
        xrows.append(jnp.where(idx % 2 == 0, e, o))
    xs = jnp.where(row16 == 0, xrows[0], jnp.where(row16 == 1, xrows[1], 0.0)).astype(bf16)
    hg = _rb(_dot(xs, wg_ref[...]))
    hg = _rb(hg * _rb(_sigmoid(hg)))
    hu = _rb(_dot(xs, wu_ref[...]))
    y = _rb(_dot((hg * hu).astype(bf16), wd_ref[...]))
    rs = pltpu.bitcast(jnp.where(row16 == 0, b1, b2), f32)
    y = _rb(y * _rb(_sigmoid(rs)))
    for j, idx in enumerate((i1, i2)):
        gin = _rb(xrows[j] + y[j:j + 1, :])
        gbits = pltpu.bitcast(_rb(gin * _rb(_sigmoid(gin))), u32)
        word = pl.ds(idx // 2, 1)
        old = g_ref[word, :]
        g_ref[word, :] = jnp.where(idx % 2 == 0,
                                   (old & jnp.uint32(0xFFFF0000)) | (gbits >> 16),
                                   (old & jnp.uint32(0x0000FFFF)) | gbits)

    wo_prep(NP - 1)
    for b in range(1, NB):
        ls, ps = c_stage()
        if b + 1 < NB:
            q_stage(NP - 1, b + 1)
        finish(b - 1, acc_ref[rows_of(b - 1), :] + o_dot())
        p_stage(NP - 1, ls, ps)
        if b + 1 < NB:
            s_stage(NP - 1)
        out_copy(b - 1).start()
    for c in range(NLAST):
        n = TQ // NLAST
        r0 = (NB - 1) * TQ + c * n
        o = _unpack(o_ref[c * n // 2:(c + 1) * n // 2, :])
        sacc = acc_ref[r0:r0 + n, :] + _dot(o, _unpack(wop_ref[...]))
        g = _unpack(g_ref[r0 // 2:(r0 + n) // 2, :]).astype(f32)
        out_ref[r0:r0 + n, :] = (x_ref[r0:r0 + n, :].astype(f32) + _rb(_rb(sacc) * g)).astype(bf16)
        last_copies[c].start()
    for b in range(NB - 1):
        out_copy(b).wait()
    for c in last_copies:
        c.wait()

@jax.jit
def pallas_recurrent_scan__sliding_block_cached__moe_arch_mod__prompt_kernel(
    A_x, A_k_cache, A_v_cache, A_wq, A_wo, B_x, B_w_r, B_w_gate, B_w_up, B_w_down,
):
    kt = jnp.swapaxes(A_k_cache, 2, 3)
    vt = jnp.swapaxes(A_v_cache, 2, 3)
    any_spec = pl.BlockSpec(memory_space=pl.ANY)
    return pl.pallas_call(
        _kernel,
        in_specs=[any_spec] * 9,
        out_specs=any_spec,
        out_shape=jax.ShapeDtypeStruct(A_x.shape, A_x.dtype),
        scratch_shapes=[
            pltpu.VMEM((S, D), bf16),
            pltpu.VMEM((S // 2, D), u32),
            pltpu.VMEM((S, D), f32),
            pltpu.VMEM((NP, D, PW), bf16),
            pltpu.VMEM((H * DH, D), bf16),
            pltpu.VMEM((H, DH, W), bf16),
            pltpu.VMEM((H, DH, W), bf16),
            pltpu.VMEM((2, 2, W // 2 + 8, KP), u32),
            pltpu.VMEM((2, 2, DH // 2 + 8, W), u32),
            pltpu.VMEM((2, D // 2, PW), u32),
            pltpu.VMEM((PW // 2, D), u32),
            pltpu.VMEM((TQ // 2, PW), u32),
            pltpu.VMEM((TQ // 2, PW), u32),
            pltpu.VMEM((2 * NJ, W, 128), f32),
            pltpu.VMEM((2 * NJ, 8, 128), f32),
            pltpu.VMEM((S // 2, D), u32),
            pltpu.VMEM((2, 2, GR // 2, 128), i32),
            pltpu.VMEM((D,), bf16),
            pltpu.VMEM((D, F), bf16),
            pltpu.VMEM((D, F), bf16),
            pltpu.VMEM((F, D), bf16),
            pltpu.VMEM((S, D), bf16),
            pltpu.SemaphoreType.DMA((4 + NB - 1,)),
            pltpu.SemaphoreType.DMA((4,)),
            pltpu.SemaphoreType.DMA((4,)),
            pltpu.SemaphoreType.DMA((4,)),
            pltpu.SemaphoreType.DMA((4,)),
            pltpu.SemaphoreType.DMA((3,)),
            pltpu.SemaphoreType.DMA((NB - 1 + NLAST,)),
        ],
        compiler_params=pltpu.CompilerParams(
            vmem_limit_bytes=128 * 1024 * 1024,
            disable_bounds_checks=True,
        ),
    )(A_x, kt, vt, A_wq, A_wo, B_w_r, B_w_gate, B_w_up, B_w_down)
```

```python
import math

import jax
import jax.numpy as jnp
import jax.experimental.pallas as pl
import jax.experimental.pallas.tpu as pltpu

S, D = 2048, 640
H, DH, W = 32, 192, 512
F = 1536
NP = H // 2
PW = 2 * DH
TQ = 512
NB = S // TQ
NJ = TQ // 128
NIT = NP * NB
KP = 256
GR = S // NIT
ROUTER_LEAD = 4
NLAST = 4
KEY_MIN = -2 ** 31
NT_DIMS = (((1,), (1,)), ((), ()))
QSCALE = (DH ** -0.5) * math.log2(math.e)
LOG2E = math.log2(math.e)
EPS_BF16 = 1.0013580322265625e-05

bf16 = jnp.bfloat16
f32 = jnp.float32
u32 = jnp.uint32
i32 = jnp.int32


def _rb(t):
    return t.astype(bf16).astype(f32)


def _sigmoid(t):
    return 0.5 * jnp.tanh(0.5 * t) + 0.5


def _recip(t):
    r = pl.reciprocal(t, approx=True)
    return r * (2.0 - t * r)


def _pack(t):
    return pltpu.bitcast(t, u32)


def _unpack(t):
    return pltpu.bitcast(t, bf16)


def _even_odd(u):
    return (pltpu.unpack_elementwise(u, index=0, packed_dtype=bf16, unpacked_dtype=f32),
            pltpu.unpack_elementwise(u, index=1, packed_dtype=bf16, unpacked_dtype=f32))


def _pack2(e, o):
    return pltpu.pack_elementwise([e, o], packed_dtype=bf16)


def _dot(a, b):
    return jnp.dot(a, b, preferred_element_type=f32)


def _dot_nt(a, b):
    return jax.lax.dot_general(a, b, NT_DIMS, preferred_element_type=f32)


def _span(i, n):
    if isinstance(i, int):
        return pl.ds(i * n, n)
    return pl.ds(pl.multiple_of(i * n, n), n)


def _kernel(x_hbm, kt_hbm, vt_hbm, wq_hbm, wo_hbm, wr_hbm, wg_hbm, wu_hbm, wd_hbm,
            out_hbm,
            x_ref, xn_ref, acc_ref, wq_ref, wo_ref, kt_ref, vt_ref, kb_ref, vb_ref,
            wqp_ref, wop_ref, q_ref, o_ref, s_ref, m_ref, g_ref, top_ref,
            wr_ref, wg_ref, wu_ref, wd_ref, out_ref,
            sem_x, sem_g0, sem_ga, sem_gb, sem_gc, sem_moe, sem_out):
    sk = kt_hbm.shape[-1]

    win = pl.ds(sk - W, W)

    def x_copy(r0, n, sem):
        rows = pl.ds(r0, n)
        return pltpu.make_async_copy(x_hbm.at[0, rows, :], x_ref.at[rows, :], sem)

    def wq_copies(p0, n, sem):
        return [pltpu.make_async_copy(wq_hbm.at[:, pl.ds(p * PW, PW)], wq_ref.at[p], sem)
                for p in range(p0, p0 + n)]

    def wo_copy(p0, n, sem):
        rows = pl.ds(p0 * PW, n * PW)
        return pltpu.make_async_copy(wo_hbm.at[rows, :], wo_ref.at[rows, :], sem)

    def kv_copy(src, dst, p0, n, sem):
        heads = pl.ds(2 * p0, 2 * n)
        return pltpu.make_async_copy(src.at[0, heads, :, win], dst.at[heads], sem)

    def group_copies(p0, n, sems, n_wo=None):
        return [kv_copy(kt_hbm, kt_ref, p0 + 1, n, sems.at[0]),
                kv_copy(vt_hbm, vt_ref, p0 + 1, n, sems.at[1]),
                wo_copy(p0, n if n_wo is None else n_wo, sems.at[3])] + wq_copies(p0 + 1, n, sems.at[2])

    x0_copies = [x_copy(c * 128, 128, sem_x.at[c]) for c in range(4)]
    x_copies = [None] + [x_copy(b * TQ, TQ, sem_x.at[3 + b]) for b in range(1, NB)]
    wq0_copy, = wq_copies(0, 1, sem_g0.at[0])
    kt0_copy = kv_copy(kt_hbm, kt_ref, 0, 1, sem_g0.at[1])
    vt0_copy = kv_copy(vt_hbm, vt_ref, 0, 1, sem_g0.at[2])
    wr_copy = pltpu.make_async_copy(wr_hbm, wr_ref, sem_g0.at[3])
    ga = group_copies(0, 1, sem_ga)
    gb = group_copies(1, 2, sem_gb)
    gc = group_copies(3, NP - 4, sem_gc, n_wo=NP - 3)
    moe_copies = [pltpu.make_async_copy(wg_hbm, wg_ref, sem_moe.at[0]),
                  pltpu.make_async_copy(wu_hbm, wu_ref, sem_moe.at[1]),
                  pltpu.make_async_copy(wd_hbm, wd_ref, sem_moe.at[2])]

    def out_copy(b):
        rows = pl.ds(b * TQ, TQ)
        return pltpu.make_async_copy(out_ref.at[rows, :], out_hbm.at[0, rows, :], sem_out.at[b])

    last_copies = [
        pltpu.make_async_copy(out_ref.at[pl.ds((NB - 1) * TQ + c * (TQ // NLAST), TQ // NLAST), :],
                              out_hbm.at[0, pl.ds((NB - 1) * TQ + c * (TQ // NLAST), TQ // NLAST), :],
                              sem_out.at[NB - 1 + c]) for c in range(NLAST)]

    def layer_norm_rows(r0):
        outs = []
        for xf in _even_odd(_pack(x_ref[r0:r0 + 128, :])):
            mean = jnp.sum(xf, axis=-1, keepdims=True) * (1.0 / D)
            xc = xf - mean
            var = jnp.sum(xc * xc, axis=-1, keepdims=True) * (1.0 / D)
            d = _rb(xf - _rb(mean))
            ve = _rb(_rb(var) + EPS_BF16)
            den = _rb(ve * jax.lax.rsqrt(ve))
            outs.append(d * _recip(den))
        xn_ref[r0 // 2:r0 // 2 + 64, :] = _pack2(*outs)

    def layer_norm(b):
        for c in range(TQ // 128):
            layer_norm_rows(b * TQ + c * 128)

    def gate_router(c):
        valid = c < NIT
        c = jnp.minimum(c, NIT - 1)
        prow = _span(c, GR // 2)
        wr = wr_ref[...].astype(f32).reshape(1, D)
        gs = []
        row = jax.lax.broadcasted_iota(i32, (GR // 2, 128), 0)
        for par, xn in enumerate(_even_odd(xn_ref[prow, :])):
            gs.append(xn * _rb(_sigmoid(xn)))
            r = _rb(jnp.sum(xn * wr, axis=-1, keepdims=True)) + 0.0
            bits = pltpu.bitcast(jnp.broadcast_to(r, (GR // 2, 128)), i32)
            key = jnp.where(bits < 0, bits ^ jnp.int32(0x7FFF0000), bits)
            key = key | (0xFFFF - (c * GR + par + 2 * row))
            key = jnp.where(valid, key, KEY_MIN)
            k1 = top_ref[par, 0]
            top_ref[par, 0] = jnp.maximum(k1, key)
            top_ref[par, 1] = jnp.maximum(top_ref[par, 1], jnp.minimum(k1, key))
        g_ref[prow, :] = _pack2(*gs)

    def q_stage(p, b, half=None, packed=True):
        if half is None:
            src, dst = _span(b, TQ // 2), pl.ds(0, TQ // 2)
        else:
            src, dst = _span(2 * b + half, TQ // 4), _span(half, TQ // 4)
        w = _unpack(wqp_ref[...]) if packed else wq_ref[p]
        q = _dot(_unpack(xn_ref[src, :]), w)
        q_ref[dst, :] = _pack((q * QSCALE).astype(bf16))

    def wq_prep(p):
        wqp_ref[...] = _pack(wq_ref[p])

    def wo_prep(p):
        wop_ref[...] = _pack(wo_ref[_span(p, PW), :])

    def _quarter(t):
        if isinstance(t, int):
            return pl.ds(t * 128, 128), pl.ds(t * 64, 64)
        return (pl.ds(pl.multiple_of(t * 128, 128), 128), pl.ds(pl.multiple_of(t * 64, 64), 64))

    def k_prep(p, t):
        cols, prow = _quarter(t)
        zpad = jnp.zeros((KP - DH, 128), bf16)
        for h in range(2):
            kt = kt_ref[2 * p + h, :, cols]
            kt = jnp.concatenate([kt, zpad] if h == 0 else [zpad, kt], axis=0)
            ke, ko = _even_odd(_pack(kt.T))
            kb_ref[h, prow, :] = _pack(jnp.concatenate([ke, ko], axis=0).astype(bf16))

    def v_prep(p, t):
        cols, _ = _quarter(t)
        for h in range(2):
            vb_ref[h, 0:DH // 2, cols] = _pack(vt_ref[2 * p + h, :, cols])

    def s_stage():
        for j in range(NJ):
            for h in range(2):
                qh = _unpack(q_ref[64 * j:64 * (j + 1), 128 * h:128 * h + 256])
                st = _dot_nt(_unpack(kb_ref[h, 0:W // 2, :]), qh)
                s_ref[2 * j + h] = st
                m_ref[2 * j + h] = jnp.max(st.reshape(W // 8, 8, 128), axis=0)

    def c_stage():
        ls = []
        ps = []
        for u in range(2 * NJ):
            m = jnp.max(m_ref[u], axis=0, keepdims=True)
            pt = jnp.exp2(s_ref[u] - m)
            ls.append(jnp.sum(pt, axis=0, keepdims=True))
            ps.append(jnp.concatenate(
                [_pack2(pt[128 * c:128 * c + 64], pt[128 * c + 64:128 * c + 128])
                 for c in range(W // 128)], axis=0))
        return ls, ps

    def p_stage(ls, ps):
        os_ = []
        for j in range(NJ):
            ots = []
            for h in range(2):
                ot = _dot(_unpack(vb_ref[h, 0:DH // 2, :]), _unpack(ps[2 * j + h]))
                ots.append(ot * (1.0 / ls[2 * j + h]))
            os_.append(jnp.concatenate(ots, axis=0).T)
        o_ref[...] = _pack(jnp.concatenate(os_, axis=0).astype(bf16))

    def o_dot():
        return _dot(_unpack(o_ref[...]), _unpack(wop_ref[...]))

    def rows_of(b):
        if isinstance(b, int):
            return pl.ds(b * TQ, TQ)
        return pl.ds(pl.multiple_of(b * TQ, TQ), TQ)

    def finish(b, s):
        rows = rows_of(b)
        if isinstance(b, int):
            prow = pl.ds(b * (TQ // 2), TQ // 2)
        else:
            prow = pl.ds(pl.multiple_of(b * (TQ // 2), TQ // 2), TQ // 2)
        g = _unpack(g_ref[prow, :]).astype(f32)
        out_ref[rows, :] = (x_ref[rows, :].astype(f32) + _rb(_rb(s) * g)).astype(bf16)

    for c in x0_copies:
        c.start()
    wq0_copy.start()
    for par in range(2):
        for j in range(2):
            top_ref[par, j] = jnp.full((GR // 2, 128), KEY_MIN, i32)

    for c in range(4):
        x0_copies[c].wait()
        if c == 0:
            kt0_copy.start()
        if c == 3:
            x_copies[1].start()
            wr_copy.start()
        layer_norm_rows(c * 128)

    wq0_copy.wait()
    q_stage(0, 0, 0, packed=False)
    wq_prep(0)
    kt0_copy.wait()
    vt0_copy.start()
    x_copies[2].start()
    x_copies[3].start()
    for t in range(4):
        k_prep(0, t)
    q_stage(0, 0, 1, packed=False)

    x_copies[1].wait()
    wr_copy.wait()
    for c in range(ROUTER_LEAD + 1):
        gate_router(c)
    layer_norm(1)
    s_stage()

    vt0_copy.wait()
    x_copies[2].wait()
    x_copies[3].wait()
    for c in ga:
        c.start()
    for t in range(4):
        v_prep(0, t)
    ls, ps = c_stage()
    q_stage(0, 1)
    p_stage(ls, ps)
    s_stage()
    layer_norm(2)
    layer_norm(3)
    for c in ga:
        c.wait()
    for c in gb:
        c.start()

    def step(p, b, first):
        pn, bn = (p, b + 1) if b + 1 < NB else (p + 1, 0)
        pp, bp = (p, b - 1) if b > 0 else (p - 1, NB - 1)
        ls, ps = c_stage()
        q_stage(pn, bn)
        rows = rows_of(bp)
        acc_ref[rows, :] = jnp.where(first, 0.0, acc_ref[rows, :]) + o_dot()
        p_stage(ls, ps)
        s_stage()

    def quad(p, carry):
        first = p == 0
        wo_prep(p)
        for b in range(1, NB + 1):
            gate_router(p * NB + b + ROUTER_LEAD)
        for b in range(1, NB - 1):
            step(p, b, first)
        wq_prep(p + 1)
        for t in range(NB):
            k_prep(p + 1, t)
        step(p, NB - 1, first)
        for t in range(NB):
            v_prep(p + 1, t)
        step(p + 1, 0, first)
        return carry

    def segment(sgm, carry):
        @pl.when(sgm == 1)
        def _():
            for c in gb:
                c.wait()
            for c in gc:
                c.start()

        @pl.when(sgm == 2)
        def _():
            for c in gc:
                c.wait()
            for c in moe_copies:
                c.start()

        lo = jnp.where(sgm == 0, 0, jnp.where(sgm == 1, 1, 3))
        hi = jnp.where(sgm == 0, 1, jnp.where(sgm == 1, 3, NP - 1))
        jax.lax.fori_loop(lo, hi, quad, 0)
        return carry

    jax.lax.fori_loop(0, 3, segment, 0)

    keys = jnp.concatenate([top_ref[0, 0], top_ref[1, 0], top_ref[0, 1], top_ref[1, 1]], axis=0)
    top1 = jnp.max(keys, axis=0, keepdims=True)
    top2 = jnp.max(jnp.where(keys == top1, KEY_MIN, keys), axis=0, keepdims=True)
    key1 = top1[0, 0]
    key2 = top2[0, 0]

    def decode(key):
        idx = jnp.clip(0xFFFF - (key & 0xFFFF), 0, S - 1)
        hi = key & jnp.int32(-65536)
        bits = jnp.where(hi < 0, hi ^ jnp.int32(0x7FFF0000), hi)
        return idx, bits

    i1, b1 = decode(key1)
    i2, b2 = decode(key2)

    for c in moe_copies:
        c.wait()
    row16 = jax.lax.broadcasted_iota(i32, (16, D), 0)
    xrows = []
    for idx in (i1, i2):
        e, o = _even_odd(xn_ref[pl.ds(idx // 2, 1), :])
        xrows.append(jnp.where(idx % 2 == 0, e, o))
    xs = jnp.where(row16 == 0, xrows[0], jnp.where(row16 == 1, xrows[1], 0.0)).astype(bf16)
    hg = _rb(_dot(xs, wg_ref[...]))
    hg = _rb(hg * _rb(_sigmoid(hg)))
    hu = _rb(_dot(xs, wu_ref[...]))
    y = _rb(_dot((hg * hu).astype(bf16), wd_ref[...]))
    rs = pltpu.bitcast(jnp.where(row16 == 0, b1, b2), f32)
    y = _rb(y * _rb(_sigmoid(rs)))
    for j, idx in enumerate((i1, i2)):
        gin = _rb(xrows[j] + y[j:j + 1, :])
        gbits = pltpu.bitcast(_rb(gin * _rb(_sigmoid(gin))), u32)
        word = pl.ds(idx // 2, 1)
        old = g_ref[word, :]
        g_ref[word, :] = jnp.where(idx % 2 == 0,
                                   (old & jnp.uint32(0xFFFF0000)) | (gbits >> 16),
                                   (old & jnp.uint32(0x0000FFFF)) | gbits)

    wo_prep(NP - 1)
    for b in range(1, NB):
        ls, ps = c_stage()
        if b + 1 < NB:
            q_stage(NP - 1, b + 1)
        finish(b - 1, acc_ref[rows_of(b - 1), :] + o_dot())
        p_stage(ls, ps)
        if b + 1 < NB:
            s_stage()
        out_copy(b - 1).start()
    for c in range(NLAST):
        n = TQ // NLAST
        r0 = (NB - 1) * TQ + c * n
        o = _unpack(o_ref[c * n // 2:(c + 1) * n // 2, :])
        sacc = acc_ref[r0:r0 + n, :] + _dot(o, _unpack(wop_ref[...]))
        g = _unpack(g_ref[r0 // 2:(r0 + n) // 2, :]).astype(f32)
        out_ref[r0:r0 + n, :] = (x_ref[r0:r0 + n, :].astype(f32) + _rb(_rb(sacc) * g)).astype(bf16)
        last_copies[c].start()
    for b in range(NB - 1):
        out_copy(b).wait()
    for c in last_copies:
        c.wait()

@jax.jit
def pallas_recurrent_scan__sliding_block_cached__moe_arch_mod__prompt_kernel(
    A_x, A_k_cache, A_v_cache, A_wq, A_wo, B_x, B_w_r, B_w_gate, B_w_up, B_w_down,
):
    kt = jnp.swapaxes(A_k_cache, 2, 3)
    vt = jnp.swapaxes(A_v_cache, 2, 3)
    any_spec = pl.BlockSpec(memory_space=pl.ANY)
    return pl.pallas_call(
        _kernel,
        in_specs=[any_spec] * 9,
        out_specs=any_spec,
        out_shape=jax.ShapeDtypeStruct(A_x.shape, A_x.dtype),
        scratch_shapes=[
            pltpu.VMEM((S, D), bf16),
            pltpu.VMEM((S // 2, D), u32),
            pltpu.VMEM((S, D), f32),
            pltpu.VMEM((NP, D, PW), bf16),
            pltpu.VMEM((H * DH, D), bf16),
            pltpu.VMEM((H, DH, W), bf16),
            pltpu.VMEM((H, DH, W), bf16),
            pltpu.VMEM((2, W // 2 + 8, KP), u32),
            pltpu.VMEM((2, DH // 2 + 8, W), u32),
            pltpu.VMEM((D // 2, PW), u32),
            pltpu.VMEM((PW // 2, D), u32),
            pltpu.VMEM((TQ // 2, PW), u32),
            pltpu.VMEM((TQ // 2, PW), u32),
            pltpu.VMEM((2 * NJ, W, 128), f32),
            pltpu.VMEM((2 * NJ, 8, 128), f32),
            pltpu.VMEM((S // 2, D), u32),
            pltpu.VMEM((2, 2, GR // 2, 128), i32),
            pltpu.VMEM((D,), bf16),
            pltpu.VMEM((D, F), bf16),
            pltpu.VMEM((D, F), bf16),
            pltpu.VMEM((F, D), bf16),
            pltpu.VMEM((S, D), bf16),
            pltpu.SemaphoreType.DMA((4 + NB - 1,)),
            pltpu.SemaphoreType.DMA((4,)),
            pltpu.SemaphoreType.DMA((4,)),
            pltpu.SemaphoreType.DMA((4,)),
            pltpu.SemaphoreType.DMA((4,)),
            pltpu.SemaphoreType.DMA((3,)),
            pltpu.SemaphoreType.DMA((NB - 1 + NLAST,)),
        ],
        compiler_params=pltpu.CompilerParams(
            vmem_limit_bytes=128 * 1024 * 1024,
            disable_bounds_checks=True,
        ),
    )(A_x, kt, vt, A_wq, A_wo, B_w_r, B_w_gate, B_w_up, B_w_down)
```

```python
import math

import jax
import jax.numpy as jnp
import jax.experimental.pallas as pl
import jax.experimental.pallas.tpu as pltpu

S, D = 2048, 640
H, DH, W = 32, 192, 512
F = 1536
NP = H // 2
PW = 2 * DH
TQ = 512
NB = S // TQ
NJ = TQ // 128
NIT = NP * NB
KP = 256
GR = S // NIT
ROUTER_LEAD = 4
NLAST = 4
KEY_MIN = -2 ** 31
NT_DIMS = (((1,), (1,)), ((), ()))
QSCALE = (DH ** -0.5) * math.log2(math.e)
EPS_BF16 = 1.0013580322265625e-05

bf16 = jnp.bfloat16
f32 = jnp.float32
u32 = jnp.uint32
i32 = jnp.int32


def _rb(t):
    return t.astype(bf16).astype(f32)


def _sigmoid(t):
    return 0.5 * jnp.tanh(0.5 * t) + 0.5


def _recip(t):
    r = pl.reciprocal(t, approx=True)
    return r * (2.0 - t * r)


def _pack(t):
    return pltpu.bitcast(t, u32)


def _unpack(t):
    return pltpu.bitcast(t, bf16)


def _even_odd(u):
    return (pltpu.unpack_elementwise(u, index=0, packed_dtype=bf16, unpacked_dtype=f32),
            pltpu.unpack_elementwise(u, index=1, packed_dtype=bf16, unpacked_dtype=f32))


def _pack2(e, o):
    return pltpu.pack_elementwise([e, o], packed_dtype=bf16)


def _dot(a, b):
    return jnp.dot(a, b, preferred_element_type=f32)


def _dot_nt(a, b):
    return jax.lax.dot_general(a, b, NT_DIMS, preferred_element_type=f32)


def _span(i, n):
    if isinstance(i, int):
        return pl.ds(i * n, n)
    return pl.ds(pl.multiple_of(i * n, n), n)


def _kernel(x_hbm, kt_hbm, vt_hbm, wq_hbm, wo_hbm, wr_hbm, wg_hbm, wu_hbm, wd_hbm,
            out_hbm,
            x_ref, xn_ref, acc_ref, wq_ref, wo_ref, kt_ref, vt_ref, kb_ref, vb_ref,
            wqp_ref, wop_ref, q_ref, o_ref, s_ref, m_ref, g_ref, top_ref,
            wr_ref, wg_ref, wu_ref, wd_ref, out_ref,
            sem_x, sem_g0, sem_ga, sem_gb, sem_gc, sem_moe, sem_out):
    sk = kt_hbm.shape[-1]

    win = pl.ds(sk - W, W)

    def x_copy(r0, n, sem):
        rows = pl.ds(r0, n)
        return pltpu.make_async_copy(x_hbm.at[0, rows, :], x_ref.at[rows, :], sem)

    def wq_copies(p0, n, sem):
        return [pltpu.make_async_copy(wq_hbm.at[:, pl.ds(p * PW, PW)], wq_ref.at[p], sem)
                for p in range(p0, p0 + n)]

    def wo_copy(p0, n, sem):
        rows = pl.ds(p0 * PW, n * PW)
        return pltpu.make_async_copy(wo_hbm.at[rows, :], wo_ref.at[rows, :], sem)

    def kv_copy(src, dst, p0, n, sem):
        heads = pl.ds(2 * p0, 2 * n)
        return pltpu.make_async_copy(src.at[0, heads, :, win], dst.at[heads], sem)

    def group_copies(p0, n, sems, n_wo=None):
        return [kv_copy(kt_hbm, kt_ref, p0 + 1, n, sems.at[0]),
                kv_copy(vt_hbm, vt_ref, p0 + 1, n, sems.at[1]),
                wo_copy(p0, n if n_wo is None else n_wo, sems.at[3])] + wq_copies(p0 + 1, n, sems.at[2])

    x0_copies = [x_copy(c * 128, 128, sem_x.at[c]) for c in range(4)]
    x_copies = [None] + [x_copy(b * TQ, TQ, sem_x.at[3 + b]) for b in range(1, NB)]
    wq0_copy, = wq_copies(0, 1, sem_g0.at[0])
    kt0_copy = kv_copy(kt_hbm, kt_ref, 0, 1, sem_g0.at[1])
    vt0_copy = kv_copy(vt_hbm, vt_ref, 0, 1, sem_g0.at[2])
    wr_copy = pltpu.make_async_copy(wr_hbm, wr_ref, sem_g0.at[3])
    ga = group_copies(0, 1, sem_ga)
    gb = group_copies(1, 2, sem_gb)
    gc = group_copies(3, NP - 4, sem_gc, n_wo=NP - 3)
    moe_copies = [pltpu.make_async_copy(wg_hbm, wg_ref, sem_moe.at[0]),
                  pltpu.make_async_copy(wu_hbm, wu_ref, sem_moe.at[1]),
                  pltpu.make_async_copy(wd_hbm, wd_ref, sem_moe.at[2])]

    def out_copy(b):
        rows = pl.ds(b * TQ, TQ)
        return pltpu.make_async_copy(out_ref.at[rows, :], out_hbm.at[0, rows, :], sem_out.at[b])

    last_copies = [
        pltpu.make_async_copy(out_ref.at[pl.ds((NB - 1) * TQ + c * (TQ // NLAST), TQ // NLAST), :],
                              out_hbm.at[0, pl.ds((NB - 1) * TQ + c * (TQ // NLAST), TQ // NLAST), :],
                              sem_out.at[NB - 1 + c]) for c in range(NLAST)]

    def layer_norm_rows(r0):
        outs = []
        for xf in _even_odd(_pack(x_ref[r0:r0 + 128, :])):
            mean = jnp.sum(xf, axis=-1, keepdims=True) * (1.0 / D)
            xc = xf - mean
            var = jnp.sum(xc * xc, axis=-1, keepdims=True) * (1.0 / D)
            d = _rb(xf - _rb(mean))
            ve = _rb(_rb(var) + EPS_BF16)
            den = _rb(ve * jax.lax.rsqrt(ve))
            outs.append(d * _recip(den))
        xn_ref[r0 // 2:r0 // 2 + 64, :] = _pack2(*outs)

    def layer_norm(b):
        for c in range(TQ // 128):
            layer_norm_rows(b * TQ + c * 128)

    def gate_router(c):
        valid = c < NIT
        c = jnp.minimum(c, NIT - 1)
        prow = _span(c, GR // 2)
        wr = wr_ref[...].astype(f32).reshape(1, D)
        gs = []
        row = jax.lax.broadcasted_iota(i32, (GR // 2, 128), 0)
        for par, xn in enumerate(_even_odd(xn_ref[prow, :])):
            gs.append(xn * _rb(_sigmoid(xn)))
            r = _rb(jnp.sum(xn * wr, axis=-1, keepdims=True)) + 0.0
            bits = pltpu.bitcast(jnp.broadcast_to(r, (GR // 2, 128)), i32)
            key = jnp.where(bits < 0, bits ^ jnp.int32(0x7FFF0000), bits)
            key = key | (0xFFFF - (c * GR + par + 2 * row))
            key = jnp.where(valid, key, KEY_MIN)
            k1 = top_ref[par, 0]
            top_ref[par, 0] = jnp.maximum(k1, key)
            top_ref[par, 1] = jnp.maximum(top_ref[par, 1], jnp.minimum(k1, key))
        g_ref[prow, :] = _pack2(*gs)

    def q_stage(p, b, half=None, packed=True):
        if half is None:
            src, dst = _span(b, TQ // 2), pl.ds(0, TQ // 2)
        else:
            src, dst = _span(2 * b + half, TQ // 4), _span(half, TQ // 4)
        w = _unpack(wqp_ref[...]) if packed else wq_ref[p]
        q = _dot(_unpack(xn_ref[src, :]), w)
        q_ref[dst, :] = _pack((q * QSCALE).astype(bf16))

    def wq_prep(p):
        wqp_ref[...] = _pack(wq_ref[p])

    def wo_prep(p):
        wop_ref[...] = _pack(wo_ref[_span(p, PW), :])

    def k_prep(p, t):
        cols, prow = _span(t, 128), _span(t, 64)
        zpad = jnp.zeros((KP - DH, 128), bf16)
        for h in range(2):
            kt = kt_ref[2 * p + h, :, cols]
            kt = jnp.concatenate([kt, zpad] if h == 0 else [zpad, kt], axis=0)
            ke, ko = _even_odd(_pack(kt.T))
            kb_ref[h, prow, :] = _pack(jnp.concatenate([ke, ko], axis=0).astype(bf16))

    def v_prep(p, t):
        cols = _span(t, 128)
        for h in range(2):
            vb_ref[h, 0:DH // 2, cols] = _pack(vt_ref[2 * p + h, :, cols])

    def s_stage():
        for j in range(NJ):
            for h in range(2):
                qh = _unpack(q_ref[64 * j:64 * (j + 1), 128 * h:128 * h + 256])
                st = _dot_nt(_unpack(kb_ref[h, 0:W // 2, :]), qh)
                s_ref[2 * j + h] = st
                m_ref[2 * j + h] = jnp.max(st.reshape(W // 8, 8, 128), axis=0)

    def c_stage():
        ls = []
        ps = []
        for u in range(2 * NJ):
            m = jnp.max(m_ref[u], axis=0, keepdims=True)
            pt = jnp.exp2(s_ref[u] - m)
            ls.append(jnp.sum(pt, axis=0, keepdims=True))
            ps.append(jnp.concatenate(
                [_pack2(pt[128 * c:128 * c + 64], pt[128 * c + 64:128 * c + 128])
                 for c in range(W // 128)], axis=0))
        return ls, ps

    def p_stage(ls, ps):
        os_ = []
        for j in range(NJ):
            ots = []
            for h in range(2):
                ot = _dot(_unpack(vb_ref[h, 0:DH // 2, :]), _unpack(ps[2 * j + h]))
                ots.append(ot * (1.0 / ls[2 * j + h]))
            os_.append(jnp.concatenate(ots, axis=0).T)
        o_ref[...] = _pack(jnp.concatenate(os_, axis=0).astype(bf16))

    def o_dot():
        return _dot(_unpack(o_ref[...]), _unpack(wop_ref[...]))

    def rows_of(b):
        return _span(b, TQ)

    def finish(b, s):
        rows = rows_of(b)
        g = _unpack(g_ref[_span(b, TQ // 2), :]).astype(f32)
        out_ref[rows, :] = (x_ref[rows, :].astype(f32) + _rb(_rb(s) * g)).astype(bf16)

    for c in x0_copies:
        c.start()
    wq0_copy.start()
    for par in range(2):
        for j in range(2):
            top_ref[par, j] = jnp.full((GR // 2, 128), KEY_MIN, i32)

    for c in range(4):
        x0_copies[c].wait()
        if c == 0:
            kt0_copy.start()
        if c == 3:
            x_copies[1].start()
            wr_copy.start()
        layer_norm_rows(c * 128)

    wq0_copy.wait()
    q_stage(0, 0, 0, packed=False)
    wq_prep(0)
    kt0_copy.wait()
    vt0_copy.start()
    x_copies[2].start()
    x_copies[3].start()
    for t in range(4):
        k_prep(0, t)
    q_stage(0, 0, 1, packed=False)

    x_copies[1].wait()
    wr_copy.wait()
    for c in range(ROUTER_LEAD + 1):
        gate_router(c)
    layer_norm(1)
    s_stage()

    vt0_copy.wait()
    x_copies[2].wait()
    x_copies[3].wait()
    for c in ga:
        c.start()
    for t in range(4):
        v_prep(0, t)
    ls, ps = c_stage()
    q_stage(0, 1)
    p_stage(ls, ps)
    s_stage()
    layer_norm(2)
    layer_norm(3)
    for c in ga:
        c.wait()
    for c in gb:
        c.start()

    def step(p, b, first):
        pn, bn = (p, b + 1) if b + 1 < NB else (p + 1, 0)
        ls, ps = c_stage()
        q_stage(pn, bn)
        rows = rows_of((b - 1) % NB)
        acc_ref[rows, :] = jnp.where(first, 0.0, acc_ref[rows, :]) + o_dot()
        p_stage(ls, ps)
        s_stage()

    def quad(p, carry):
        first = p == 0
        wo_prep(p)
        for b in range(1, NB + 1):
            gate_router(p * NB + b + ROUTER_LEAD)
        for b in range(1, NB - 1):
            step(p, b, first)
        wq_prep(p + 1)
        for t in range(NB):
            k_prep(p + 1, t)
        step(p, NB - 1, first)
        for t in range(NB):
            v_prep(p + 1, t)
        step(p + 1, 0, first)
        return carry

    def segment(sgm, carry):
        @pl.when(sgm == 1)
        def _():
            for c in gb:
                c.wait()
            for c in gc:
                c.start()

        @pl.when(sgm == 2)
        def _():
            for c in gc:
                c.wait()
            for c in moe_copies:
                c.start()

        lo = jnp.where(sgm == 0, 0, jnp.where(sgm == 1, 1, 3))
        hi = jnp.where(sgm == 0, 1, jnp.where(sgm == 1, 3, NP - 1))
        jax.lax.fori_loop(lo, hi, quad, 0)
        return carry

    jax.lax.fori_loop(0, 3, segment, 0)

    keys = jnp.concatenate([top_ref[0, 0], top_ref[1, 0], top_ref[0, 1], top_ref[1, 1]], axis=0)
    top1 = jnp.max(keys, axis=0, keepdims=True)
    top2 = jnp.max(jnp.where(keys == top1, KEY_MIN, keys), axis=0, keepdims=True)
    key1 = top1[0, 0]
    key2 = top2[0, 0]

    def decode(key):
        idx = jnp.clip(0xFFFF - (key & 0xFFFF), 0, S - 1)
        hi = key & jnp.int32(-65536)
        bits = jnp.where(hi < 0, hi ^ jnp.int32(0x7FFF0000), hi)
        return idx, bits

    i1, b1 = decode(key1)
    i2, b2 = decode(key2)

    for c in moe_copies:
        c.wait()
    row16 = jax.lax.broadcasted_iota(i32, (16, D), 0)
    xrows = []
    for idx in (i1, i2):
        e, o = _even_odd(xn_ref[pl.ds(idx // 2, 1), :])
        xrows.append(jnp.where(idx % 2 == 0, e, o))
    xs = jnp.where(row16 == 0, xrows[0], jnp.where(row16 == 1, xrows[1], 0.0)).astype(bf16)
    hg = _rb(_dot(xs, wg_ref[...]))
    hg = _rb(hg * _rb(_sigmoid(hg)))
    hu = _rb(_dot(xs, wu_ref[...]))
    y = _rb(_dot((hg * hu).astype(bf16), wd_ref[...]))
    rs = pltpu.bitcast(jnp.where(row16 == 0, b1, b2), f32)
    y = _rb(y * _rb(_sigmoid(rs)))
    for j, idx in enumerate((i1, i2)):
        gin = _rb(xrows[j] + y[j:j + 1, :])
        gbits = pltpu.bitcast(_rb(gin * _rb(_sigmoid(gin))), u32)
        word = pl.ds(idx // 2, 1)
        old = g_ref[word, :]
        g_ref[word, :] = jnp.where(idx % 2 == 0,
                                   (old & jnp.uint32(0xFFFF0000)) | (gbits >> 16),
                                   (old & jnp.uint32(0x0000FFFF)) | gbits)

    wo_prep(NP - 1)
    for b in range(1, NB):
        ls, ps = c_stage()
        if b + 1 < NB:
            q_stage(NP - 1, b + 1)
        finish(b - 1, acc_ref[rows_of(b - 1), :] + o_dot())
        p_stage(ls, ps)
        if b + 1 < NB:
            s_stage()
        out_copy(b - 1).start()
    for c in range(NLAST):
        n = TQ // NLAST
        r0 = (NB - 1) * TQ + c * n
        o = _unpack(o_ref[c * n // 2:(c + 1) * n // 2, :])
        sacc = acc_ref[r0:r0 + n, :] + _dot(o, _unpack(wop_ref[...]))
        g = _unpack(g_ref[r0 // 2:(r0 + n) // 2, :]).astype(f32)
        out_ref[r0:r0 + n, :] = (x_ref[r0:r0 + n, :].astype(f32) + _rb(_rb(sacc) * g)).astype(bf16)
        last_copies[c].start()
    for b in range(NB - 1):
        out_copy(b).wait()
    for c in last_copies:
        c.wait()


@jax.jit
def pallas_recurrent_scan__sliding_block_cached__moe_arch_mod__prompt_kernel(
    A_x, A_k_cache, A_v_cache, A_wq, A_wo, B_x, B_w_r, B_w_gate, B_w_up, B_w_down,
):
    kt = jnp.swapaxes(A_k_cache, 2, 3)
    vt = jnp.swapaxes(A_v_cache, 2, 3)
    any_spec = pl.BlockSpec(memory_space=pl.ANY)
    return pl.pallas_call(
        _kernel,
        in_specs=[any_spec] * 9,
        out_specs=any_spec,
        out_shape=jax.ShapeDtypeStruct(A_x.shape, A_x.dtype),
        scratch_shapes=[
            pltpu.VMEM((S, D), bf16),
            pltpu.VMEM((S // 2, D), u32),
            pltpu.VMEM((S, D), f32),
            pltpu.VMEM((NP, D, PW), bf16),
            pltpu.VMEM((H * DH, D), bf16),
            pltpu.VMEM((H, DH, W), bf16),
            pltpu.VMEM((H, DH, W), bf16),
            pltpu.VMEM((2, W // 2 + 8, KP), u32),
            pltpu.VMEM((2, DH // 2 + 8, W), u32),
            pltpu.VMEM((D // 2, PW), u32),
            pltpu.VMEM((PW // 2, D), u32),
            pltpu.VMEM((TQ // 2, PW), u32),
            pltpu.VMEM((TQ // 2, PW), u32),
            pltpu.VMEM((2 * NJ, W, 128), f32),
            pltpu.VMEM((2 * NJ, 8, 128), f32),
            pltpu.VMEM((S // 2, D), u32),
            pltpu.VMEM((2, 2, GR // 2, 128), i32),
            pltpu.VMEM((D,), bf16),
            pltpu.VMEM((D, F), bf16),
            pltpu.VMEM((D, F), bf16),
            pltpu.VMEM((F, D), bf16),
            pltpu.VMEM((S, D), bf16),
            pltpu.SemaphoreType.DMA((4 + NB - 1,)),
            pltpu.SemaphoreType.DMA((4,)),
            pltpu.SemaphoreType.DMA((4,)),
            pltpu.SemaphoreType.DMA((4,)),
            pltpu.SemaphoreType.DMA((4,)),
            pltpu.SemaphoreType.DMA((3,)),
            pltpu.SemaphoreType.DMA((NB - 1 + NLAST,)),
        ],
        compiler_params=pltpu.CompilerParams(
            vmem_limit_bytes=128 * 1024 * 1024,
            disable_bounds_checks=True,
        ),
    )(A_x, kt, vt, A_wq, A_wo, B_w_r, B_w_gate, B_w_up, B_w_down)
```
